```python
import jax
import jax.numpy as jnp

def _softmax(x, axis=-1):
    return jax.nn.softmax(x, axis=axis)

def _gelu(x):
    return jax.nn.gelu(x, approximate=True)

def _silu(x):
    return jax.nn.silu(x)

def _sigmoid(x):
    return jax.nn.sigmoid(x)

def _layernorm(x, axis=-1, eps=1e-05):
    m = jnp.mean(x, axis=axis, keepdims=True)
    v = jnp.var(x, axis=axis, keepdims=True)
    return (x - m) / jnp.sqrt(v + eps)

def _scatter_add(tgt, idx, src, axis=0):
    return tgt.at[idx].add(src)

def _segment_sum(src, seg, n):
    return jax.ops.segment_sum(src, seg, n)

class _Rng:

    def __init__(self, key):
        self._k = key

    def _next(self):
        self._k, sub = jax.random.split(self._k)
        return sub

    def normal(self, shape):
        return jax.random.normal(self._next(), shape, dtype=jnp.bfloat16)

    def randint(self, lo, hi, shape):
        return jax.random.randint(self._next(), shape, lo, hi, dtype=jnp.int32)

    def uniform(self, shape, lo=0.0, hi=1.0):
        return jax.random.uniform(self._next(), shape, jnp.bfloat16, lo, hi)

    def permutation(self, n):
        return jax.random.permutation(self._next(), n)
kernel_name = 'parallel_sum__memory_aug_infini_attn__moe_arch_mod__prompt'

def setup_inputs():
    _rng = _Rng(jax.random.key(int.from_bytes(__import__("os").urandom(4), "little")))
    _w = lambda a: (lambda t: t.astype(jnp.bfloat16) if jnp.issubdtype(t.dtype, jnp.floating) else t)(jnp.asarray(a))

    def _A_setup():
        B, S, D, H = (1, 2048, 576, 32)
        N = 4
        L = max(1, S // N)
        sc = D ** (-0.5)
        return {'x': _w((lambda *s: _rng.normal(s) * 0.05)(B, N * L, D)), 'wq': _w((lambda *s: _rng.normal(s) * 0.05)(D, D) * sc), 'wk': _w((lambda *s: _rng.normal(s) * 0.05)(D, D) * sc), 'wv': _w((lambda *s: _rng.normal(s) * 0.05)(D, D) * sc), 'wo': _w((lambda *s: _rng.normal(s) * 0.05)(D, D) * sc), 'beta': _w((lambda *s: _rng.normal(s) * 0.05)(H))}
    _A_in = _A_setup()

    def _B_setup():
        B, S, D, F, C = (1, 2048, 576, 4608, 2)
        return {'x': _w((lambda *s: _rng.normal(s) * 0.05)(B, S, D)), 'w_r': _w((lambda *s: _rng.normal(s) * 0.05)(D)), 'w_gate': _w((lambda *s: _rng.normal(s) * 0.05)(D, F)), 'w_up': _w((lambda *s: _rng.normal(s) * 0.05)(D, F)), 'w_down': _w((lambda *s: _rng.normal(s) * 0.05)(F, D))}
    _B_in = _B_setup()
    return {'A_x': _A_in['x'], 'A_wq': _A_in['wq'], 'A_wk': _A_in['wk'], 'A_wv': _A_in['wv'], 'A_wo': _A_in['wo'], 'A_beta': _A_in['beta'], 'B_x': _B_in['x'], 'B_w_r': _B_in['w_r'], 'B_w_gate': _B_in['w_gate'], 'B_w_up': _B_in['w_up'], 'B_w_down': _B_in['w_down']}

def reference(A_x, A_wq, A_wk, A_wv, A_wo, A_beta, B_x, B_w_r, B_w_gate, B_w_up, B_w_down):

    def _A_ref(x, wq, wk, wv, wo, beta):
        B, S, D = x.shape
        H = 32
        Dh = D // H
        N = 4
        L = S // N
        q = (lambda x, *d: x.transpose(*d))((x @ wq).reshape(B, S, H, Dh), 0, 2, 1, 3).reshape(B, H, N, L, Dh)
        k = (lambda x, *d: x.transpose(*d))((x @ wk).reshape(B, S, H, Dh), 0, 2, 1, 3).reshape(B, H, N, L, Dh)
        v = (lambda x, *d: x.transpose(*d))((x @ wv).reshape(B, S, H, Dh), 0, 2, 1, 3).reshape(B, H, N, L, Dh)
        phi = lambda t: jnp.where(t > 0, t + 1.0, jnp.exp(t))
        scale = Dh ** (-0.5)
        ar = jnp.arange(L)
        mask = (lambda x, dt: x.astype(dt))(ar[:, None] < ar[None, :], x.dtype) * -1000000000.0
        g = _sigmoid(beta).reshape(1, H, 1, 1)
        M = jnp.einsum('bhd,bhe->bhde', q[:, :, 0, 0, :] * 0.0, q[:, :, 0, 0, :] * 0.0)
        z = q[:, :, 0, 0, :] * 0.0
        outs = []
        for s in range(N):
            qs, ks, vs = (q[:, :, s].copy(), k[:, :, s].copy(), v[:, :, s].copy())
            logits = jnp.einsum('bhqd,bhkd->bhqk', qs, ks) * scale + mask
            p = _softmax(logits, axis=-1)
            a_dot = jnp.einsum('bhqk,bhkd->bhqd', p, vs)
            pq = phi(qs)
            num = jnp.einsum('bhld,bhde->bhle', pq, M)
            den = jnp.einsum('bhld,bhd->bhl', pq, z)[..., None] + 1e-06
            a_mem = num / den
            o = g * a_mem + (1.0 - g) * a_dot
            outs.append(o)
            pk = phi(ks)
            M = M + jnp.einsum('bhld,bhle->bhde', pk, vs)
            z = z + jnp.einsum('bhld->bhd', pk)
        o = (lambda x, *d: x.transpose(*d))(jnp.stack(outs, 2).reshape(B, H, S, Dh), 0, 2, 1, 3).reshape(B, S, D)
        return o @ wo

    def _B_ref(x, w_r, w_gate, w_up, w_down):
        B, S, D = x.shape
        C = 2
        r = x @ w_r
        idx = jnp.argsort(-r, axis=-1)[:, :C]
        idx_e = jnp.repeat(idx.reshape(B, C, 1), D, axis=2)
        x_sel = jnp.take_along_axis(x, idx_e, axis=1)
        g = _silu(x_sel @ w_gate)
        u = x_sel @ w_up
        y = g * u @ w_down
        r_sel = _sigmoid(jnp.take_along_axis(r, idx, axis=1))
        y = y * r_sel.reshape(B, C, 1)
        b_off = (jnp.arange(B) * S).reshape(B, 1)
        flat_idx = (idx + b_off).reshape(B * C)
        zero = (x * 0.0).reshape(B * S, D)
        upd = _scatter_add(zero, flat_idx, y.reshape(B * C, D), axis=0)
        return x + upd.reshape(B, S, D)
    x = A_x
    xn = _layernorm(x, axis=-1)
    return x + _A_ref(xn, A_wq, A_wk, A_wv, A_wo, A_beta) + _B_ref(xn, B_w_r, B_w_gate, B_w_up, B_w_down)
```

```python
import functools
import math

import jax
import jax.numpy as jnp
import numpy as np
from jax import lax
import jax.experimental.pallas as pl
import jax.experimental.pallas.tpu as pltpu

S = 2048
D = 576
H = 32
DH = D // H
NSEG = 4
L = S // NSEG
F = 4608
T = 128
DP = 640
NQT = L // T
WIN = 112
NWIN = 5
HEAD_WIN = [0] * 7 + [1] * 6 + [2] * 6 + [3] * 6 + [4] * 7
WIN_HEADS = [[h for h in range(H) if HEAD_WIN[h] == t] for t in range(NWIN)]
NROW = 3 * D + 16
LOG2E = math.log2(math.e)
QSCALE = DH ** -0.5 * LOG2E
MASKVAL = -999292928.0 * LOG2E

LN_EPS = float(np.asarray(1e-5, dtype=jnp.bfloat16).astype(np.float32))

bf16 = jnp.bfloat16
f32 = jnp.float32
u32 = jnp.uint32


def _pack(x):
    return pltpu.bitcast(x, u32)


def _unpack(x):
    return pltpu.bitcast(x, bf16)


def _dot(a, b):
    return jnp.dot(a, b, preferred_element_type=f32)


def _dot_nt(a, b):
    return lax.dot_general(a, b, (((1,), (1,)), ((), ())), preferred_element_type=f32)


def _iota(shape, dim):
    return lax.broadcasted_iota(jnp.int32, shape, dim)


def _phi(t):
    return jnp.where(t > 0, t + 1.0, jnp.exp(t))


def _round_bf16(x):
    return x.astype(bf16).astype(f32)


def _sigmoid(x):
    return 1.0 / (1.0 + jnp.exp(-x))


def _w_tile(w_ref, i, j, tail=None):
    r = min(T, D - T * i)
    c = min(T, D - T * j)
    t = w_ref[T * i:T * i + r, T * j:T * j + c]
    if c < T:
        t = jnp.concatenate([t, jnp.zeros((r, T - c), bf16)], axis=1)
    if r < T:
        parts = [t]
        if tail is not None:
            parts.append(tail)
        n = T - sum(p.shape[0] for p in parts)
        parts.append(jnp.zeros((n, T), bf16))
        t = jnp.concatenate(parts, axis=0)
    return t


def _store_wt(dst, row0, w_ref, i, j, tail=None):
    c = min(T, D - T * j)
    t = _pack(_w_tile(w_ref, i, j, tail).T)
    r0 = (row0 + T * j) // 2
    dst[r0:r0 + c // 2, T * i:T * (i + 1)] = t[:c // 2]


def kernel(x_hbm, wq_hbm, wk_hbm, wv_hbm, wo_hbm, beta_ref, wr_ref, wg_hbm, wu_hbm, wd_hbm,
           out_hbm,
           x_v, wq_v, wk_v, wv_v, wo_v, wg_v, wu_v, wd_v, out_v,
           wt, wot, xn_s, q_s, k_s, v_s, pq_s, pk_s, r_s, g_s, bias_s, o_s, m_s, sems, osems):
    def xcopy(s):
        return pltpu.make_async_copy(x_hbm.at[:, pl.ds(s * L, L)], x_v.at[s], sems.at[s])

    cp_k = pltpu.make_async_copy(wk_hbm, wk_v, sems.at[4])
    cp_q = pltpu.make_async_copy(wq_hbm, wq_v, sems.at[5])
    cp_v = pltpu.make_async_copy(wv_hbm, wv_v, sems.at[6])
    cp_o = pltpu.make_async_copy(wo_hbm, wo_v, sems.at[7])
    cp_g = pltpu.make_async_copy(wg_hbm, wg_v, sems.at[8])
    cp_u = pltpu.make_async_copy(wu_hbm, wu_v, sems.at[9])
    cp_d = pltpu.make_async_copy(wd_hbm, wd_v, sems.at[10])

    cp_q.start()
    xcopy(0).start()
    cp_k.start()
    cp_v.start()
    for s in range(1, NSEG):
        xcopy(s).start()
    cp_o.start()
    cp_g.start()
    cp_u.start()
    cp_d.start()

    bias_s[...] = jnp.where(_iota((T, T), 0) > _iota((T, T), 1), MASKVAL, 0.0).astype(f32)
    g = _round_bf16(_sigmoid(beta_ref[...].astype(f32)))
    g = jnp.concatenate([g, jnp.zeros((1, T - H), f32)], axis=1)
    g_s[...] = jnp.broadcast_to(g, (T, T)).T
    wr = wr_ref[...].reshape(1, D)
    wr = jnp.concatenate([wr, jnp.zeros((1, DP - D), bf16)], axis=1)
    wt[3 * D // 2:NROW // 2, :] = _pack(jnp.broadcast_to(wr, (16, DP)))
    m_s[...] = jnp.zeros(m_s.shape, f32)

    for n, (cp, w) in enumerate(((cp_q, wq_v), (cp_k, wk_v), (cp_v, wv_v))):
        cp.wait()
        for i in range(5):
            for j in range(5):
                _store_wt(wt, n * D, w, i, j)

    def proj_segment(s, carry):
        xcopy(s).wait()
        for j in range(NQT):
            x = x_v[s, :, T * j:T * (j + 1)].astype(f32)
            mean = jnp.sum(x, axis=0, keepdims=True) / D
            c = x - mean
            var = jnp.sum(c * c, axis=0, keepdims=True) / D
            sd = _round_bf16(jnp.sqrt(_round_bf16(_round_bf16(var) + LN_EPS)))
            d = _round_bf16(x - _round_bf16(mean))
            xn = (d * (1.0 / sd)).astype(bf16)
            xn_s[NQT * s + j, 0:D // 2, :] = _pack(xn)
            xn_s[NQT * s + j, D // 2:DP // 2, :] = jnp.zeros(((DP - D) // 2, T), u32)
        xn = jnp.concatenate([_unpack(xn_s[NQT * s + j]) for j in range(NQT)], axis=1)
        q = _dot(_unpack(wt[0:D // 2, :]), xn)
        q_s[s] = _pack((q * QSCALE).astype(bf16))
        pq_s[s] = _pack(_phi(q).astype(bf16))
        k = _dot(_unpack(wt[D // 2:D, :]), xn)
        pk_s[s] = _pack(_phi(k).astype(bf16))
        kb = k.astype(bf16)
        for t in range(NWIN):
            for j in range(NQT):
                k_s[s, t, 64 * j:64 * (j + 1), :] = _pack(kb[WIN * t:WIN * t + T, T * j:T * (j + 1)].T)
        v = _dot(_unpack(wt[D:NROW // 2, :]), xn)
        v_s[s] = _pack(v[:D].astype(bf16))
        for j in range(NQT):
            r_s[pl.ds(NQT * s + j, 1), :] = v[D:D + 1, T * j:T * (j + 1)]
        return carry

    lax.fori_loop(0, NSEG, proj_segment, 0)

    r = _round_bf16(r_s[...])
    pos = _iota((S // T, T), 0) * T + _iota((S // T, T), 1)
    r1 = jnp.max(r)
    i1 = jnp.minimum(jnp.min(jnp.where(r == r1, pos, S)), S - 1)
    rest = pos != i1
    r2 = jnp.max(jnp.where(rest, r, -jnp.inf))
    i2 = jnp.minimum(jnp.min(jnp.where(rest & (r == r2), pos, S)), S - 1)

    lane = _iota((DP // 2, T), 1)
    row16 = _iota((16, T), 0)
    xsel = jnp.zeros((16, DP), f32)
    for c, idx in enumerate((i1, i2)):
        col = jnp.where(lane == idx % T, xn_s[idx // T], jnp.zeros((), u32))
        xsel = xsel + _dot_nt(jnp.where(row16 == c, 1.0, 0.0).astype(bf16), _unpack(col))
    xsel = xsel[:, :D].astype(bf16)
    cp_g.wait()
    gate = _dot(xsel, wg_v[...])
    cp_u.wait()
    up = _dot(xsel, wu_v[...])
    hid = (gate * _sigmoid(gate) * up).astype(bf16)
    cp_d.wait()
    y = _dot_nt(hid, wd_v[...])
    rsel = jnp.where(_iota((16, D), 0) == 0, r1, r2)
    y = (y * _sigmoid(rsel)).astype(bf16)
    y = jnp.concatenate([y, jnp.zeros((16, DP - D), bf16)], axis=1)
    cp_o.wait()
    for i in range(5):
        for j in range(5):
            _store_wt(wot, 0, wo_v, i, j, tail=y[:, T * j:T * (j + 1)])

    def ocopy(s):
        return pltpu.make_async_copy(out_v.at[s], out_hbm.at[:, pl.ds(pl.multiple_of(s * L, L), L)],
                                     osems.at[s])

    def attn_segment(s, carry):
        prow = _iota((8, T), 0)
        ones_pk = jnp.full((8, T), 0x3F803F80, u32)
        for h in range(H):
            t = HEAD_WIN[h]
            a = (DH * h) // 16
            o = DH * h - 16 * a
            lo = o // 2
            pos0 = a - (WIN * t) // 16
            g1 = 1.0 - jnp.broadcast_to(g_s[h:h + 1, :], (8, T))
            vts = []
            for i in range(NQT):
                v0 = v_s[s, 8 * a:8 * a + 8, T * i:T * (i + 1)]
                v1 = v_s[s, 8 * a + 8:8 * a + 16, T * i:T * (i + 1)]
                if o < 8:
                    v1 = jnp.where(prow >= 4, ones_pk, v1)
                else:
                    v0 = jnp.where(prow < 4, ones_pk, v0)
                vts.append(_unpack(jnp.concatenate([v0, v1], axis=0)))
            for j in range(NQT):
                q0 = q_s[s, 8 * a:8 * a + 8, T * j:T * (j + 1)]
                q1 = q_s[s, 8 * a + 8:8 * a + 16, T * j:T * (j + 1)]
                if lo > 0:
                    q0 = jnp.where(prow >= lo, q0, jnp.zeros((), u32))
                if lo < 7:
                    q1 = jnp.where(prow <= lo, q1, jnp.zeros((), u32))
                parts = []
                if pos0 > 0:
                    parts.append(jnp.zeros((8 * pos0, T), u32))
                parts += [q0, q1]
                if pos0 < 6:
                    parts.append(jnp.zeros((8 * (6 - pos0), T), u32))
                qm = _unpack(jnp.concatenate(parts, axis=0))
                kw = _unpack(k_s[s, t, 0:64 * (j + 1), :])
                st = _dot(kw, qm)
                if j > 0:
                    st = jnp.concatenate([st[:T * j], st[T * j:] + bias_s[...]], axis=0)
                else:
                    st = st + bias_s[...]
                m = jnp.max(st, axis=0, keepdims=True)
                p = jnp.exp2(st - m).astype(bf16)
                vt = jnp.concatenate(vts[:j + 1], axis=1) if j > 0 else vts[0]
                pv = _dot(vt, p)
                l = pv[24:32] if o < 8 else pv[0:8]
                sc = g1 / l
                b = 0 if o < 8 else 8
                val = pv[b:b + 24] * jnp.concatenate([sc, sc, sc], axis=0)
                o_s[DH * h:DH * (h + 1), T * j:T * (j + 1)] = val[o - b:o - b + DH]

        colh = _iota((T, T), 1)
        rowh = _iota((T, T), 0)
        for t in range(NWIN):
            heads = WIN_HEADS[t]
            r0 = WIN * t
            same = None
            zsel = None
            for n, h in enumerate(heads):
                cin = (colh >= DH * h - r0) & (colh < DH * (h + 1) - r0)
                blk = cin & (rowh >= DH * h - r0) & (rowh < DH * (h + 1) - r0)
                same = blk if same is None else same | blk
                zc = cin[:16] & (rowh[:16] == n)
                zsel = zc if zsel is None else zsel | zc
            mt = m_s[t]
            lhs = jnp.concatenate([jnp.where(same, mt[:T], 0.0), jnp.where(zsel, mt[T:], 0.0)], axis=0)
            rd = _dot(lhs.astype(bf16), _unpack(pq_s[s, r0 // 2:r0 // 2 + 64, :]))
            h0 = heads[0]
            coef = g_s[h0:h0 + 8, :]
            coef = jnp.concatenate([coef] * NQT, axis=1) / (rd[T:T + 8] + 1e-6)
            lo_row = DH * heads[0]
            hi_row = DH * (heads[-1] + 1)
            for rb in range(lo_row // 8 * 8, hi_row, 8):
                ha = max(rb // DH, h0)
                hb = min((rb + 7) // DH, heads[-1])
                cf = jnp.broadcast_to(coef[ha - h0:ha - h0 + 1], (8, L))
                if hb != ha:
                    cf = jnp.where(_iota((8, L), 0) < DH * hb - rb, cf,
                                   jnp.broadcast_to(coef[hb - h0:hb - h0 + 1], (8, L)))
                o_s[rb:rb + 8, :] = o_s[rb:rb + 8, :] + rd[rb - r0:rb - r0 + 8] * cf
            vl = jnp.concatenate([_unpack(v_s[s, r0 // 2:r0 // 2 + 64, :]), jnp.ones((16, L), bf16)], axis=0)
            m_s[t] = mt + _dot_nt(vl, _unpack(pk_s[s, r0 // 2:r0 // 2 + 64, :]))

        tok = _iota((16, L), 1) + s * L
        sel = jnp.where(_iota((16, L), 0) == 0, i1, jnp.where(_iota((16, L), 0) == 1, i2, -1))
        hot = jnp.where(tok == sel, 1.0, 0.0).astype(bf16)
        ob = jnp.concatenate([o_s[...].astype(bf16), hot, jnp.zeros((DP - D - 16, L), bf16)], axis=0)
        res = _dot(_unpack(wot[...]), ob)
        xn = jnp.concatenate([_unpack(xn_s[NQT * s + j, 0:D // 2, :]) for j in range(NQT)], axis=1)
        out_v[s] = (res + x_v[s].astype(f32) + xn.astype(f32)).astype(bf16)
        ocopy(s).start()
        return carry

    lax.fori_loop(0, NSEG, attn_segment, 0)
    for s in range(NSEG):
        ocopy(s).wait()


@jax.jit
def pallas_parallel_sum__memory_aug_infini_attn__moe_arch_mod__prompt_kernel(
    A_x, A_wq, A_wk, A_wv, A_wo, A_beta, B_x, B_w_r, B_w_gate, B_w_up, B_w_down,
):
    del B_x
    any_spec = pl.BlockSpec(memory_space=pl.ANY)
    vmem_spec = pl.BlockSpec(memory_space=pltpu.VMEM)
    out_t = pl.pallas_call(
        kernel,
        out_shape=jax.ShapeDtypeStruct((D, S), bf16),
        in_specs=[any_spec] * 5 + [vmem_spec] * 2 + [any_spec] * 3,
        out_specs=any_spec,
        scratch_shapes=[
            pltpu.VMEM((NSEG, D, L), bf16),
            pltpu.VMEM((D, D), bf16),
            pltpu.VMEM((D, D), bf16),
            pltpu.VMEM((D, D), bf16),
            pltpu.VMEM((D, D), bf16),
            pltpu.VMEM((D, F), bf16),
            pltpu.VMEM((D, F), bf16),
            pltpu.VMEM((D, F), bf16),
            pltpu.VMEM((NSEG, D, L), bf16),
            pltpu.VMEM((NROW // 2, DP), u32),
            pltpu.VMEM((D // 2, DP), u32),
            pltpu.VMEM((S // T, DP // 2, T), u32),
            pltpu.VMEM((NSEG, D // 2, L), u32),
            pltpu.VMEM((NSEG, NWIN, L // 2, T), u32),
            pltpu.VMEM((NSEG, D // 2, L), u32),
            pltpu.VMEM((NSEG, D // 2, L), u32),
            pltpu.VMEM((NSEG, D // 2, L), u32),
            pltpu.VMEM((S // T, T), f32),
            pltpu.VMEM((T, T), f32),
            pltpu.VMEM((T, T), f32),
            pltpu.VMEM((D, L), f32),
            pltpu.VMEM((NWIN, T + 16, T), f32),
            pltpu.SemaphoreType.DMA((11,)),
            pltpu.SemaphoreType.DMA((NSEG,)),
        ],
        compiler_params=pltpu.CompilerParams(vmem_limit_bytes=100 * 1024 * 1024),
        name="infini_moe",
    )(A_x.reshape(S, D).T, A_wq, A_wk, A_wv, A_wo, A_beta.reshape(1, H), B_w_r,
      B_w_gate, B_w_up, B_w_down.T)
    return out_t.T.reshape(1, S, D)
```

```python
import functools
import math

import jax
import jax.numpy as jnp
import numpy as np
from jax import lax
import jax.experimental.pallas as pl
import jax.experimental.pallas.tpu as pltpu

S = 2048
D = 576
H = 32
DH = D // H
NSEG = 4
L = S // NSEG
F = 4608
T = 128
DP = 640
NQT = L // T
WIN = 112
NWIN = 5
HEAD_WIN = [0] * 7 + [1] * 6 + [2] * 6 + [3] * 6 + [4] * 7
WIN_HEADS = [[h for h in range(H) if HEAD_WIN[h] == t] for t in range(NWIN)]
HG = 4
NG = H // HG
GWIN = [min(HG * DH * g // 16 * 16, D - T) for g in range(NG)]
LAG = 5
NB = 8
NROW = 3 * D + 16
LOG2E = math.log2(math.e)
QSCALE = DH ** -0.5 * LOG2E
MASKVAL = -999292928.0 * LOG2E

LN_EPS = float(np.asarray(1e-5, dtype=jnp.bfloat16).astype(np.float32))

bf16 = jnp.bfloat16
f32 = jnp.float32
u32 = jnp.uint32


def _pack(x):
    return pltpu.bitcast(x, u32)


def _unpack(x):
    return pltpu.bitcast(x, bf16)


def _dot(a, b):
    return jnp.dot(a, b, preferred_element_type=f32)


def _dot_nt(a, b):
    return lax.dot_general(a, b, (((1,), (1,)), ((), ())), preferred_element_type=f32)


def _iota(shape, dim):
    return lax.broadcasted_iota(jnp.int32, shape, dim)


def _phi(t):
    return jnp.where(t > 0, t + 1.0, jnp.exp(t))


def _round_bf16(x):
    return x.astype(bf16).astype(f32)


def _sigmoid(x):
    return 1.0 / (1.0 + jnp.exp(-x))


def _w_tile(w_ref, i, j, tail=None):
    r = min(T, D - T * i)
    c = min(T, D - T * j)
    t = w_ref[T * i:T * i + r, T * j:T * j + c]
    if c < T:
        t = jnp.concatenate([t, jnp.zeros((r, T - c), bf16)], axis=1)
    if r < T:
        parts = [t]
        if tail is not None:
            parts.append(tail)
        n = T - sum(p.shape[0] for p in parts)
        parts.append(jnp.zeros((n, T), bf16))
        t = jnp.concatenate(parts, axis=0)
    return t


def _store_wt(dst, row0, w_ref, i, j, tail=None):
    c = min(T, D - T * j)
    t = _pack(_w_tile(w_ref, i, j, tail).T)
    r0 = (row0 + T * j) // 2
    dst[r0:r0 + c // 2, T * i:T * (i + 1)] = t[:c // 2]


def kernel(x_hbm, wq_hbm, wk_hbm, wv_hbm, wo_hbm, beta_ref, wr_ref, wg_hbm, wu_hbm, wd_hbm,
           out_hbm,
           x_v, wq_v, wk_v, wv_v, wo_v, wg_v, wu_v, wd_v, out_v,
           wt, wot, xn_s, q_s, k_s, v_s, pq_s, pk_s, r_s, g_s, bias_s, o_s, m_s, om_s, mask_s, s_s, sems, osems):
    def xcopy(s):
        return pltpu.make_async_copy(x_hbm.at[:, pl.ds(s * L, L)], x_v.at[s], sems.at[s])

    cp_k = pltpu.make_async_copy(wk_hbm, wk_v, sems.at[4])
    cp_q = pltpu.make_async_copy(wq_hbm, wq_v, sems.at[5])
    cp_v = pltpu.make_async_copy(wv_hbm, wv_v, sems.at[6])
    cp_o = pltpu.make_async_copy(wo_hbm, wo_v, sems.at[7])
    cp_g = pltpu.make_async_copy(wg_hbm, wg_v, sems.at[8])
    cp_u = pltpu.make_async_copy(wu_hbm, wu_v, sems.at[9])
    cp_d = pltpu.make_async_copy(wd_hbm, wd_v, sems.at[10])

    cp_q.start()
    xcopy(0).start()
    cp_k.start()
    cp_v.start()
    for s in range(1, NSEG):
        xcopy(s).start()
    cp_o.start()
    cp_g.start()
    cp_u.start()
    cp_d.start()

    bias_s[...] = jnp.where(_iota((T, T), 0) > _iota((T, T), 1), MASKVAL, 0.0).astype(f32)
    g = _round_bf16(_sigmoid(beta_ref[...].astype(f32)))
    g = jnp.concatenate([g, jnp.zeros((1, T - H), f32)], axis=1)
    g_s[...] = jnp.broadcast_to(g, (T, T)).T
    wr = wr_ref[...].reshape(1, D)
    wr = jnp.concatenate([wr, jnp.zeros((1, DP - D), bf16)], axis=1)
    wt[3 * D // 2:NROW // 2, :] = _pack(jnp.broadcast_to(wr, (16, DP)))
    m_s[...] = jnp.zeros(m_s.shape, f32)
    colh = _iota((T, T), 1)
    rowh = _iota((T, T), 0)
    for t in range(NWIN):
        same = None
        zsel = None
        for n, h in enumerate(WIN_HEADS[t]):
            cin = (colh >= DH * h - WIN * t) & (colh < DH * (h + 1) - WIN * t)
            blk = cin & (rowh >= DH * h - WIN * t) & (rowh < DH * (h + 1) - WIN * t)
            same = blk if same is None else same | blk
            zc = cin[:16] & (rowh[:16] == n)
            zsel = zc if zsel is None else zsel | zc
        mask_s[t, 0:T] = jnp.where(same, 1.0, 0.0)
        mask_s[t, T:T + 16] = jnp.where(zsel, 1.0, 0.0)

    for n, (cp, w) in enumerate(((cp_q, wq_v), (cp_k, wk_v), (cp_v, wv_v))):
        cp.wait()
        for i in range(5):
            for j in range(5):
                _store_wt(wt, n * D, w, i, j)

    def proj_segment(s, carry):
        xcopy(s).wait()
        for j in range(NQT):
            x = x_v[s, :, T * j:T * (j + 1)].astype(f32)
            mean = jnp.sum(x, axis=0, keepdims=True) / D
            c = x - mean
            var = jnp.sum(c * c, axis=0, keepdims=True) / D
            sd = _round_bf16(jnp.sqrt(_round_bf16(_round_bf16(var) + LN_EPS)))
            d = _round_bf16(x - _round_bf16(mean))
            xn = (d * (1.0 / sd)).astype(bf16)
            xn_s[NQT * s + j, 0:D // 2, :] = _pack(xn)
            xn_s[NQT * s + j, D // 2:DP // 2, :] = jnp.zeros(((DP - D) // 2, T), u32)
        xn = jnp.concatenate([_unpack(xn_s[NQT * s + j]) for j in range(NQT)], axis=1)
        q = _dot(_unpack(wt[0:D // 2, :]), xn)
        q_s[s] = _pack((q * QSCALE).astype(bf16))
        pq_s[s] = _pack(_phi(q).astype(bf16))
        k = _dot(_unpack(wt[D // 2:D, :]), xn)
        pk_s[s] = _pack(_phi(k).astype(bf16))
        kb = k.astype(bf16)
        for g in range(NG):
            for j in range(NQT):
                k_s[s, g, 64 * j:64 * (j + 1), :] = _pack(kb[GWIN[g]:GWIN[g] + T, T * j:T * (j + 1)].T)
        v = _dot(_unpack(wt[D:NROW // 2, :]), xn)
        v_s[s] = _pack(v[:D].astype(bf16))
        for j in range(NQT):
            r_s[pl.ds(NQT * s + j, 1), :] = v[D:D + 1, T * j:T * (j + 1)]
        return carry

    lax.fori_loop(0, NSEG, proj_segment, 0)

    r = _round_bf16(r_s[...])
    pos = _iota((S // T, T), 0) * T + _iota((S // T, T), 1)
    r1 = jnp.max(r)
    i1 = jnp.minimum(jnp.min(jnp.where(r == r1, pos, S)), S - 1)
    rest = pos != i1
    r2 = jnp.max(jnp.where(rest, r, -jnp.inf))
    i2 = jnp.minimum(jnp.min(jnp.where(rest & (r == r2), pos, S)), S - 1)

    lane = _iota((DP // 2, T), 1)
    row16 = _iota((16, T), 0)
    xsel = jnp.zeros((16, DP), f32)
    for c, idx in enumerate((i1, i2)):
        col = jnp.where(lane == idx % T, xn_s[idx // T], jnp.zeros((), u32))
        xsel = xsel + _dot_nt(jnp.where(row16 == c, 1.0, 0.0).astype(bf16), _unpack(col))
    xsel = xsel[:, :D].astype(bf16)
    cp_g.wait()
    gate = _dot(xsel, wg_v[...])
    cp_u.wait()
    up = _dot(xsel, wu_v[...])
    hid = (gate * _sigmoid(gate) * up).astype(bf16)
    cp_d.wait()
    y = _dot_nt(hid, wd_v[...])
    rsel = jnp.where(_iota((16, D), 0) == 0, r1, r2)
    y = (y * _sigmoid(rsel)).astype(bf16)
    y = jnp.concatenate([y, jnp.zeros((16, DP - D), bf16)], axis=1)
    cp_o.wait()
    for i in range(5):
        for j in range(5):
            _store_wt(wot, 0, wo_v, i, j, tail=y[:, T * j:T * (j + 1)])

    def ocopy(s):
        return pltpu.make_async_copy(out_v.at[s], out_hbm.at[:, pl.ds(pl.multiple_of(s * L, L), L)],
                                     osems.at[s])

    def attn_segment(s, carry):
        prow = _iota((8, T), 0)
        ones_pk = jnp.full((8, T), 0x3F803F80, u32)
        steps = [(g, j, i) for g in range(NG) for j in range(NQT) for i in range(j + 1)]
        mx, qms, acc = {}, {}, {}

        def head_geom(h):
            a = (DH * h) // 16
            return a, DH * h - 16 * a

        def q_masked(g, j):
            cols = []
            for h in range(HG * g, HG * (g + 1)):
                a, o = head_geom(h)
                lo = o // 2
                pos0 = a - GWIN[g] // 16
                q0 = q_s[s, 8 * a:8 * a + 8, T * j:T * (j + 1)]
                q1 = q_s[s, 8 * a + 8:8 * a + 16, T * j:T * (j + 1)]
                if lo > 0:
                    q0 = jnp.where(prow >= lo, q0, jnp.zeros((), u32))
                if lo < 7:
                    q1 = jnp.where(prow <= lo, q1, jnp.zeros((), u32))
                parts = []
                if pos0 > 0:
                    parts.append(jnp.zeros((8 * pos0, T), u32))
                parts += [q0, q1]
                if pos0 < 6:
                    parts.append(jnp.zeros((8 * (6 - pos0), T), u32))
                cols.append(jnp.concatenate(parts, axis=0))
            return _unpack(jnp.concatenate(cols, axis=1))

        def qk(n):
            g, j, i = steps[n]
            st = _dot(_unpack(k_s[s, g, 64 * i:64 * (i + 1), :]), q_masked(g, j))
            if i == j:
                st = st + jnp.concatenate([bias_s[...]] * HG, axis=1)
            s_s[n % NB] = st
            m = st[0:8]
            part = [st[8 * r:8 * r + 8] for r in range(16)]
            while len(part) > 1:
                part = [jnp.maximum(part[2 * r], part[2 * r + 1]) for r in range(len(part) // 2)]
            mx[g, j] = part[0] if i == 0 else jnp.maximum(mx[g, j], part[0])
            if i == j:
                mx[g, j] = jnp.max(mx[g, j], axis=0, keepdims=True)

        def pv(n):
            g, j, i = steps[n]
            for c in range(HG):
                p = jnp.exp2(s_s[n % NB, :, T * c:T * (c + 1)] - mx[g, j][:, T * c:T * (c + 1)]).astype(bf16)
                h = HG * g + c
                a, o = head_geom(h)
                v0 = v_s[s, 8 * a:8 * a + 8, T * i:T * (i + 1)]
                v1 = v_s[s, 8 * a + 8:8 * a + 16, T * i:T * (i + 1)]
                if o < 8:
                    v1 = jnp.where(prow >= 4, ones_pk, v1)
                else:
                    v0 = jnp.where(prow < 4, ones_pk, v0)
                r = _dot(_unpack(jnp.concatenate([v0, v1], axis=0)), p)
                acc[h] = r if i == 0 else acc[h] + r
                if i == j:
                    r = acc[h]
                    l = r[24:32] if o < 8 else r[0:8]
                    sc = (1.0 - jnp.broadcast_to(g_s[h:h + 1, :], (8, T))) / l
                    b = 0 if o < 8 else 8
                    val = r[b:b + 24] * jnp.concatenate([sc, sc, sc], axis=0)
                    o_s[DH * h:DH * (h + 1), T * j:T * (j + 1)] = val[o - b:o - b + DH]

        def mem_read(t):
            heads = WIN_HEADS[t]
            r0 = WIN * t
            lhs = jnp.where(mask_s[t] > 0, m_s[t], 0.0)
            rd = _dot(lhs.astype(bf16), _unpack(pq_s[s, r0 // 2:r0 // 2 + 64, :]))
            h0 = heads[0]
            coef = g_s[h0:h0 + 8, :]
            coef = jnp.concatenate([coef] * NQT, axis=1) / (rd[T:T + 8] + 1e-6)
            lo_row = DH * heads[0]
            hi_row = DH * (heads[-1] + 1)
            for rb in range(lo_row // 8 * 8, hi_row, 8):
                ha = max(rb // DH, h0)
                hb = min((rb + 7) // DH, heads[-1])
                cf = jnp.broadcast_to(coef[ha - h0:ha - h0 + 1], (8, L))
                if hb != ha:
                    cf = jnp.where(_iota((8, L), 0) < DH * hb - rb, cf,
                                   jnp.broadcast_to(coef[hb - h0:hb - h0 + 1], (8, L)))
                val = rd[rb - r0:rb - r0 + 8] * cf
                ra, re = max(rb, lo_row), min(rb + 8, hi_row)
                om_s[ra:re, :] = val[ra - rb:re - rb]

        def mem_update(t):
            r0 = WIN * t
            vl = jnp.concatenate([_unpack(v_s[s, r0 // 2:r0 // 2 + 64, :]), jnp.ones((16, L), bf16)], axis=0)
            m_s[t] = m_s[t] + _dot_nt(vl, _unpack(pk_s[s, r0 // 2:r0 // 2 + 64, :]))

        ns = len(steps)
        for n in range(ns + LAG):
            if n < ns:
                qk(n)
            else:
                mem_update(n - ns)
            if n >= LAG:
                pv(n - LAG)
            else:
                mem_read(n)

        tok = _iota((16, L), 1) + s * L
        sel = jnp.where(_iota((16, L), 0) == 0, i1, jnp.where(_iota((16, L), 0) == 1, i2, -1))
        hot = jnp.where(tok == sel, 1.0, 0.0).astype(bf16)
        ob = jnp.concatenate([(o_s[...] + om_s[...]).astype(bf16), hot, jnp.zeros((DP - D - 16, L), bf16)], axis=0)
        res = _dot(_unpack(wot[...]), ob)
        xn = jnp.concatenate([_unpack(xn_s[NQT * s + j, 0:D // 2, :]) for j in range(NQT)], axis=1)
        out_v[s] = (res + x_v[s].astype(f32) + xn.astype(f32)).astype(bf16)
        ocopy(s).start()
        return carry

    lax.fori_loop(0, NSEG, attn_segment, 0)
    for s in range(NSEG):
        ocopy(s).wait()


@jax.jit
def pallas_parallel_sum__memory_aug_infini_attn__moe_arch_mod__prompt_kernel(
    A_x, A_wq, A_wk, A_wv, A_wo, A_beta, B_x, B_w_r, B_w_gate, B_w_up, B_w_down,
):
    del B_x
    any_spec = pl.BlockSpec(memory_space=pl.ANY)
    vmem_spec = pl.BlockSpec(memory_space=pltpu.VMEM)
    out_t = pl.pallas_call(
        kernel,
        out_shape=jax.ShapeDtypeStruct((D, S), bf16),
        in_specs=[any_spec] * 5 + [vmem_spec] * 2 + [any_spec] * 3,
        out_specs=any_spec,
        scratch_shapes=[
            pltpu.VMEM((NSEG, D, L), bf16),
            pltpu.VMEM((D, D), bf16),
            pltpu.VMEM((D, D), bf16),
            pltpu.VMEM((D, D), bf16),
            pltpu.VMEM((D, D), bf16),
            pltpu.VMEM((D, F), bf16),
            pltpu.VMEM((D, F), bf16),
            pltpu.VMEM((D, F), bf16),
            pltpu.VMEM((NSEG, D, L), bf16),
            pltpu.VMEM((NROW // 2, DP), u32),
            pltpu.VMEM((D // 2, DP), u32),
            pltpu.VMEM((S // T, DP // 2, T), u32),
            pltpu.VMEM((NSEG, D // 2, L), u32),
            pltpu.VMEM((NSEG, NG, L // 2, T), u32),
            pltpu.VMEM((NSEG, D // 2, L), u32),
            pltpu.VMEM((NSEG, D // 2, L), u32),
            pltpu.VMEM((NSEG, D // 2, L), u32),
            pltpu.VMEM((S // T, T), f32),
            pltpu.VMEM((T, T), f32),
            pltpu.VMEM((T, T), f32),
            pltpu.VMEM((D, L), f32),
            pltpu.VMEM((NWIN, T + 16, T), f32),
            pltpu.VMEM((D, L), f32),
            pltpu.VMEM((NWIN, T + 16, T), f32),
            pltpu.VMEM((NB, T, HG * T), f32),
            pltpu.SemaphoreType.DMA((11,)),
            pltpu.SemaphoreType.DMA((NSEG,)),
        ],
        compiler_params=pltpu.CompilerParams(vmem_limit_bytes=100 * 1024 * 1024),
        name="infini_moe",
    )(A_x.reshape(S, D).T, A_wq, A_wk, A_wv, A_wo, A_beta.reshape(1, H), B_w_r,
      B_w_gate, B_w_up, B_w_down.T)
    return out_t.T.reshape(1, S, D)
```

```python
import math
import os

import jax
import jax.numpy as jnp
import numpy as np
from jax import lax
import jax.experimental.pallas as pl
import jax.experimental.pallas.tpu as pltpu

S = 2048
D = 576
H = 32
DH = D // H
NSEG = 4
L = S // NSEG
F = 4608
T = 128
DP = 640
NQT = L // T
WIN = 112
NWIN = 5
HEAD_WIN = [0] * 7 + [1] * 6 + [2] * 6 + [3] * 6 + [4] * 7
WIN_HEADS = [[h for h in range(H) if HEAD_WIN[h] == t] for t in range(NWIN)]
HG = 4
NG = H // HG
GWIN = [min(HG * DH * g // 16 * 16, D - T) for g in range(NG)]
TOKROW = int(os.environ.get('TOKROW', 0))
TOKBACK = int(os.environ.get('TOKBACK', 1))
MOE0 = int(os.environ.get('MOE0', 80))
LAG = 5
NB = 8
RQ, RK, RV = 0, D + 16, 2 * D + 16
NROW = 3 * D + 16
LOG2E = math.log2(math.e)
QSCALE = DH ** -0.5 * LOG2E
MASKVAL = -999292928.0 * LOG2E
LN_EPS = float(np.asarray(1e-5, dtype=jnp.bfloat16).astype(np.float32))

bf16 = jnp.bfloat16
f32 = jnp.float32
u32 = jnp.uint32


def _pack(x):
    return pltpu.bitcast(x, u32)


def _unpack(x):
    return pltpu.bitcast(x, bf16)


def _dot(a, b):
    return jnp.dot(a, b, preferred_element_type=f32)


def _dot_nt(a, b):
    return lax.dot_general(a, b, (((1,), (1,)), ((), ())), preferred_element_type=f32)


def _iota(shape, dim):
    return lax.broadcasted_iota(jnp.int32, shape, dim)


def _phi(t):
    return jnp.where(t > 0, t + 1.0, jnp.exp(t))


def _round_bf16(x):
    return x.astype(bf16).astype(f32)


def _sigmoid(x):
    return 1.0 / (1.0 + jnp.exp(-x))


def _w_tile(w_ref, i, j, tail=None):
    r = min(T, D - T * i)
    c = min(T, D - T * j)
    t = w_ref[T * i:T * i + r, T * j:T * j + c]
    if c < T:
        t = jnp.concatenate([t, jnp.zeros((r, T - c), bf16)], axis=1)
    if r < T:
        parts = [t]
        if tail is not None:
            parts.append(tail)
        n = T - sum(p.shape[0] for p in parts)
        parts.append(jnp.zeros((n, T), bf16))
        t = jnp.concatenate(parts, axis=0)
    return t


def _store_wt(dst, row0, w_ref, i, j, tail=None):
    c = min(T, D - T * j)
    t = _pack(_w_tile(w_ref, i, j, tail).T)
    r0 = (row0 + T * j) // 2
    dst[r0:r0 + c // 2, T * i:T * (i + 1)] = t[:c // 2]


def kernel(x_hbm, wq_hbm, wk_hbm, wv_hbm, wo_hbm, beta_ref, wr_ref, wg_hbm, wu_hbm, wd_hbm,
           out_hbm,
           x_v, wq_v, wk_v, wv_v, wo_v, wg_v, wu_v, wd_v, out_v,
           wt, wot, xn_s, q_s, k_s, v_s, pq_s, pk_s, r_s, g_s, o_s, ob_s, m_s, om_s, mask_s, s_s,
           h_s, sems, osems):
    cp_x = [pltpu.make_async_copy(x_hbm.at[:, pl.ds(s * L, L)], x_v.at[s], sems.at[s])
            for s in range(NSEG)]
    cp_o = [pltpu.make_async_copy(out_v.at[s], out_hbm.at[:, pl.ds(s * L, L)], osems.at[s])
            for s in range(NSEG)]
    cp_wk = pltpu.make_async_copy(wk_hbm, wk_v, sems.at[4])
    cp_wq = pltpu.make_async_copy(wq_hbm, wq_v, sems.at[5])
    cp_wv = pltpu.make_async_copy(wv_hbm, wv_v, sems.at[6])
    cp_wo = pltpu.make_async_copy(wo_hbm, wo_v, sems.at[7])
    cp_wg = pltpu.make_async_copy(wg_hbm, wg_v, sems.at[8])
    cp_wu = pltpu.make_async_copy(wu_hbm, wu_v, sems.at[9])
    cp_wd = pltpu.make_async_copy(wd_hbm, wd_v, sems.at[10])
    for cp in (cp_x[0], cp_wq, cp_wk, cp_wv, cp_x[1], cp_x[2], cp_x[3], cp_wo, cp_wg, cp_wu, cp_wd):
        cp.start()

    g = _round_bf16(_sigmoid(beta_ref[...].astype(f32)))
    g = jnp.concatenate([g, jnp.zeros((1, T - H), f32)], axis=1)
    g_s[...] = jnp.broadcast_to(g, (T, T)).T
    wr = wr_ref[...].reshape(1, D)
    wr = jnp.concatenate([wr, jnp.zeros((1, DP - D), bf16)], axis=1)
    wt[D // 2:RK // 2, :] = _pack(jnp.broadcast_to(wr, (16, DP)))
    colh = _iota((T, T), 1)
    rowh = _iota((T, T), 0)
    for t in range(NWIN):
        same = None
        zsel = None
        for n, h in enumerate(WIN_HEADS[t]):
            cin = (colh >= DH * h - WIN * t) & (colh < DH * (h + 1) - WIN * t)
            blk = cin & (rowh >= DH * h - WIN * t) & (rowh < DH * (h + 1) - WIN * t)
            same = blk if same is None else same | blk
            zc = cin[:16] & (rowh[:16] == n)
            zsel = zc if zsel is None else zsel | zc
        mask_s[t, 0:T] = jnp.where(same, 1.0, 0.0)
        mask_s[t, T:T + 16] = jnp.where(zsel, 1.0, 0.0)
    for j in range(S // T):
        xn_s[j, D // 2:DP // 2, :] = jnp.zeros(((DP - D) // 2, T), u32)

    def transpose_w(row0, w):
        for j in range(5):
            for i in range(5):
                _store_wt(wt, row0, w, i, j)

    def layernorm(s, j):
        x = x_v[s, :, T * j:T * (j + 1)].astype(f32)
        mean = jnp.sum(x, axis=0, keepdims=True) / D
        c = x - mean
        var = jnp.sum(c * c, axis=0, keepdims=True) / D
        sd = _round_bf16(jnp.sqrt(_round_bf16(_round_bf16(var) + LN_EPS)))
        d = _round_bf16(x - _round_bf16(mean))
        xn_s[NQT * s + j, 0:D // 2, :] = _pack((d * (1.0 / sd)).astype(bf16))

    def xn_seg(s):
        return _unpack(jnp.concatenate([xn_s[NQT * s + j] for j in range(NQT)], axis=1))

    def proj_q(s):
        q = _dot(_unpack(wt[RQ // 2:RK // 2, :]), xn_seg(s))
        q_s[s] = _pack((q[:D] * QSCALE).astype(bf16))
        if s > 0:
            pq_s[s - 1] = _pack(_phi(q[:D]).astype(bf16))
        for j in range(NQT):
            r_s[NQT * s + j:NQT * s + j + 1, :] = q[D:D + 1, T * j:T * (j + 1)]

    def proj_k(s):
        k = _dot(_unpack(wt[RK // 2:RV // 2, :]), xn_seg(s))
        if s < NSEG - 1:
            pk_s[s] = _pack(_phi(k).astype(bf16))
        for j in range(NQT):
            kb = k[:, T * j:T * (j + 1)].astype(bf16)
            for g in range(NG):
                k_s[s, g, 64 * j:64 * (j + 1), :] = _pack(kb[GWIN[g]:GWIN[g] + T].T)

    def proj_v(s):
        v_s[s] = _pack(_dot(_unpack(wt[RV // 2:NROW // 2, :]), xn_seg(s)).astype(bf16))

    cp_x[0].wait()
    for j in range(NQT):
        layernorm(0, j)
    cp_wq.wait()
    transpose_w(RQ, wq_v)
    proj_q(0)
    cp_wk.wait()
    cp_wv.wait()
    transpose_w(RK, wk_v)
    transpose_w(RV, wv_v)
    proj_k(0)
    for s in range(1, NSEG):
        cp_x[s].wait()
    for j in range(NQT):
        layernorm(1, j)
    proj_v(0)
    for s in range(1, NSEG):
        if s + 1 < NSEG:
            for j in range(NQT):
                layernorm(s + 1, j)
        proj_q(s)

    r = _round_bf16(r_s[...])
    pos = _iota((S // T, T), 0) * T + _iota((S // T, T), 1)
    r1 = jnp.max(r)
    i1 = jnp.minimum(jnp.min(jnp.where(r == r1, pos, S)), S - 1)
    rest = pos != i1
    r2 = jnp.max(jnp.where(rest, r, -jnp.inf))
    i2 = jnp.minimum(jnp.min(jnp.where(rest & (r == r2), pos, S)), S - 1)

    for s in range(1, NSEG):
        proj_k(s)
        proj_v(s)

    lane = _iota((DP // 2, T), 1)
    row16 = _iota((16, T), 0)
    xsel = jnp.zeros((16, DP), f32)
    for c, idx in enumerate((i1, i2)):
        col = jnp.where(lane == idx % T, xn_s[idx // T], jnp.zeros((), u32))
        xsel = xsel + _dot_nt(jnp.where(row16 == c, 1.0, 0.0).astype(bf16), _unpack(col))

    moe = {}

    def ffn_in(w, name, cg, i):
        k = min(T, D - T * i)
        r_ = _dot(xsel[:, T * i:T * i + k].astype(bf16), w[T * i:T * i + k, L * cg:L * (cg + 1)])[:8]
        moe[name] = r_ if i == 0 else moe[name] + r_
        if name == "up" and i == 4:
            gate = moe["gate"]
            hid = gate * _sigmoid(gate) * moe["up"]
            h_s[:, L * cg:L * (cg + 1)] = _pack(
                jnp.concatenate([hid, jnp.zeros((8, L), f32)], axis=0).astype(bf16))

    def ffn_out(cg, i):
        if i < 4:
            c0 = L * cg + T * i
            r_ = _dot_nt(_unpack(h_s[:, c0:c0 + T]), wd_v[0:4 * T, c0:c0 + T])[:8]
            moe["y0"] = r_ if "y0" not in moe else moe["y0"] + r_
        else:
            r_ = _dot_nt(_unpack(h_s[:, L * cg:L * (cg + 1)]), wd_v[4 * T:D, L * cg:L * (cg + 1)])[:8]
            moe["y1"] = r_ if "y1" not in moe else moe["y1"] + r_

    def ffn_finish():
        y = jnp.concatenate([moe["y0"], moe["y1"], jnp.zeros((8, DP - D), f32)], axis=1)
        y = y * _sigmoid(jnp.where(_iota((8, DP), 0) == 0, r1, r2))
        y = jnp.concatenate([y, jnp.zeros((8, DP), f32)], axis=0)
        for j in range(5):
            _store_wt(wot, 0, wo_v, 4, j, tail=y[:, T * j:T * (j + 1)].astype(bf16))

    rounds = []
    for cg in range(F // L):
        rounds += [(ffn_in, wg_v, "gate", cg, i) for i in range(5)]
        rounds += [(ffn_in, wu_v, "up", cg, i) for i in range(5)]
        if cg > 0:
            rounds += [(ffn_out, cg - 1, i) for i in range(5)]
    rounds += [None] * 3
    rounds += [(ffn_out, F // L - 1, i) for i in range(5)]

    prow = _iota((8, T), 0)
    ones_pk = jnp.full((8, T), 0x3F803F80, u32)
    steps = [(s, g, j, i) for s in range(NSEG) for g in range(NG) for j in range(NQT)
             for i in range(j + 1)]
    ns = len(steps)
    mx, tok, acc = {}, {}, {}
    never = prow > i1 + 8
    qmk = _iota((8, HG * T), 1) % T - _iota((8, HG * T), 0)

    def head_geom(h):
        a = (DH * h) // 16
        return a, DH * h - 16 * a

    def q_masked(s, g, j):
        cols = []
        for h in range(HG * g, HG * (g + 1)):
            a, o = head_geom(h)
            lo = o // 2
            pos0 = a - GWIN[g] // 16
            q0 = q_s[s, 8 * a:8 * a + 8, T * j:T * (j + 1)]
            q1 = q_s[s, 8 * a + 8:8 * a + 16, T * j:T * (j + 1)]
            if lo > 0:
                q0 = jnp.where(prow >= lo, q0, jnp.zeros((), u32))
            if lo < 7:
                q1 = jnp.where(prow <= lo, q1, jnp.zeros((), u32))
            parts = []
            if pos0 > 0:
                parts.append(jnp.zeros((8 * pos0, T), u32))
            parts += [q0, q1]
            if pos0 < 6:
                parts.append(jnp.zeros((8 * (6 - pos0), T), u32))
            cols.append(jnp.concatenate(parts, axis=0))
        return _unpack(jnp.concatenate(cols, axis=1))

    def qk(n):
        s, g, j, i = steps[n]
        st = _dot(_unpack(k_s[s, g, 64 * i:64 * (i + 1), :]), q_masked(s, g, j))
        m = None if i == 0 else mx[s, g, j]
        for r_ in range(16):
            x = st[8 * r_:8 * r_ + 8]
            if i == j:
                x = jnp.where(qmk < 8 * r_, MASKVAL, x)
            s_s[n % NB, 8 * r_:8 * r_ + 8, :] = x
            m = x if m is None else jnp.maximum(m, x)
            if r_ == TOKROW:
                tok[n] = x
        mx[s, g, j] = jnp.max(m, axis=0, keepdims=True) if i == j else m

    def pv(n):
        s, g, j, i = steps[n]
        for c in range(HG):
            m = jnp.broadcast_to(mx[s, g, j][:, T * c:T * (c + 1)], (8, T))
            m = jnp.where(never, tok[min(n + LAG - TOKBACK, ns - 1)][:, T * c:T * (c + 1)], m)
            m = jnp.concatenate([m] * 16, axis=0)
            p = jnp.exp2(s_s[n % NB, :, T * c:T * (c + 1)] - m).astype(bf16)
            h = HG * g + c
            a, o = head_geom(h)
            v0 = v_s[s, 8 * a:8 * a + 8, T * i:T * (i + 1)]
            v1 = v_s[s, 8 * a + 8:8 * a + 16, T * i:T * (i + 1)]
            if o < 8:
                v1 = jnp.where(prow >= 4, ones_pk, v1)
            else:
                v0 = jnp.where(prow < 4, ones_pk, v0)
            r_ = _dot(_unpack(jnp.concatenate([v0, v1], axis=0)), p)
            acc[h] = r_ if i == 0 else acc[h] + r_
            if i == j:
                r_ = acc[h]
                l = r_[24:32] if o < 8 else r_[0:8]
                sc = (1.0 - jnp.broadcast_to(g_s[h:h + 1, :], (8, T))) / l
                b = 0 if o < 8 else 8
                val = r_[b:b + 24] * jnp.concatenate([sc, sc, sc], axis=0)
                o_s[s % 2, DH * h:DH * (h + 1), T * j:T * (j + 1)] = val[o - b:o - b + DH]

    def mem_read(s, t):
        heads = WIN_HEADS[t]
        r0 = WIN * t
        lhs = jnp.where(mask_s[t] > 0, m_s[t], 0.0)
        rd = _dot(lhs.astype(bf16), _unpack(pq_s[s - 1, r0 // 2:r0 // 2 + 64, :]))
        h0 = heads[0]
        coef = jnp.concatenate([g_s[h0:h0 + 8, :]] * NQT, axis=1) / (rd[T:T + 8] + 1e-6)
        lo_row = DH * heads[0]
        hi_row = DH * (heads[-1] + 1)
        for rb in range(lo_row // 8 * 8, hi_row, 8):
            ha = max(rb // DH, h0)
            hb = min((rb + 7) // DH, heads[-1])
            cf = jnp.broadcast_to(coef[ha - h0:ha - h0 + 1], (8, L))
            if hb != ha:
                cf = jnp.where(_iota((8, L), 0) < DH * hb - rb, cf,
                               jnp.broadcast_to(coef[hb - h0:hb - h0 + 1], (8, L)))
            val = rd[rb - r0:rb - r0 + 8] * cf
            ra, re = max(rb, lo_row), min(rb + 8, hi_row)
            om_s[s % 2, ra:re, :] = val[ra - rb:re - rb]

    def mem_update(s, t):
        r0 = WIN * t
        vl = jnp.concatenate([_unpack(v_s[s, r0 // 2:r0 // 2 + 64, :]), jnp.ones((16, L), bf16)], axis=0)
        upd = _dot_nt(vl, _unpack(pk_s[s, r0 // 2:r0 // 2 + 64, :]))
        m_s[t] = upd if s == 0 else m_s[t] + upd

    def pack_o(s, r0, r1_):
        o = o_s[s % 2, r0:r1_, :]
        if s > 0:
            o = o + om_s[s % 2, r0:r1_, :]
        ob_s[s, r0 // 2:r1_ // 2, :] = _pack(o.astype(bf16))

    def out_proj(s, r0, r1_):
        res = _dot(_unpack(wot[r0 // 2:r1_ // 2, :]), _unpack(ob_s[s]))
        xn = _unpack(jnp.concatenate(
            [xn_s[NQT * s + j, r0 // 2:r1_ // 2, :] for j in range(NQT)], axis=1))
        out_v[s, r0:r1_, :] = (res + x_v[s, r0:r1_, :].astype(f32) + xn.astype(f32)).astype(bf16)

    for s in range(NSEG):
        tpos = _iota((16, L), 1) + s * L
        sel = jnp.where(_iota((16, L), 0) == 0, i1, jnp.where(_iota((16, L), 0) == 1, i2, -1))
        ob_s[s, D // 2:D // 2 + 8, :] = _pack(jnp.where(tpos == sel, 1.0, 0.0).astype(bf16))
        ob_s[s, D // 2 + 8:DP // 2, :] = jnp.zeros(((DP - D) // 2 - 8, L), u32)

    extra = {}

    def at(n, fn, *args):
        extra.setdefault(n, []).append((fn,) + args)

    per = ns // NSEG
    for t in range(NWIN):
        at(t, mem_update, 0, t)
        for s in range(1, NSEG):
            at(per * s - 40 + 4 * t, mem_read, s, t)
            if s < NSEG - 1:
                at(per * s + 10 + 4 * t, mem_update, s, t)

    def late_weights():
        for cp in (cp_wo, cp_wg, cp_wu, cp_wd):
            cp.wait()
        for j in range(5):
            for i in range(4):
                _store_wt(wot, 0, wo_v, i, j)

    at(MOE0, late_weights)
    for k, rd_ in enumerate(rounds):
        if rd_ is not None:
            at(MOE0 + k, *rd_)
    done = MOE0 + len(rounds) + 2
    at(done, ffn_finish)
    at(done + 5, out_proj, 0, 0, D)
    at(done + 6, cp_o[0].start)
    at(done + 10, out_proj, 1, 0, D)
    at(done + 11, cp_o[1].start)
    for s in range(NSEG - 1):
        for c in range(4):
            at(per * s + 20 * (c + 1) + LAG + 1, pack_o, s, 144 * c, 144 * (c + 1))
    for c in range(3):
        at(per * 3 + 20 * (c + 1) + LAG + 1, pack_o, 3, 144 * c, 144 * (c + 1))
    for c, (r0, r1_) in enumerate(((0, 112), (112, 224), (224, 336), (336, 448), (448, D))):
        at(ns + c, out_proj, 2, r0, r1_)

    for n in range(ns + LAG):
        if n < ns:
            qk(n)
        for task in extra.get(n, ()):
            task[0](*task[1:])
        if n >= LAG:
            pv(n - LAG)
    cp_o[2].start()
    pack_o(3, 432, D)
    out_proj(3, 0, D)
    cp_o[3].start()
    for s in range(NSEG):
        cp_o[s].wait()


@jax.jit
def pallas_parallel_sum__memory_aug_infini_attn__moe_arch_mod__prompt_kernel(
    A_x, A_wq, A_wk, A_wv, A_wo, A_beta, B_x, B_w_r, B_w_gate, B_w_up, B_w_down,
):
    del B_x
    any_spec = pl.BlockSpec(memory_space=pl.ANY)
    vmem_spec = pl.BlockSpec(memory_space=pltpu.VMEM)
    out_t = pl.pallas_call(
        kernel,
        out_shape=jax.ShapeDtypeStruct((D, S), bf16),
        in_specs=[any_spec] * 5 + [vmem_spec] * 2 + [any_spec] * 3,
        out_specs=any_spec,
        scratch_shapes=[
            pltpu.VMEM((NSEG, D, L), bf16),
            pltpu.VMEM((D, D), bf16),
            pltpu.VMEM((D, D), bf16),
            pltpu.VMEM((D, D), bf16),
            pltpu.VMEM((D, D), bf16),
            pltpu.VMEM((D, F), bf16),
            pltpu.VMEM((D, F), bf16),
            pltpu.VMEM((D, F), bf16),
            pltpu.VMEM((NSEG, D, L), bf16),
            pltpu.VMEM((NROW // 2, DP), u32),
            pltpu.VMEM((D // 2, DP), u32),
            pltpu.VMEM((S // T, DP // 2, T), u32),
            pltpu.VMEM((NSEG, D // 2, L), u32),
            pltpu.VMEM((NSEG, NG, L // 2, T), u32),
            pltpu.VMEM((NSEG, D // 2, L), u32),
            pltpu.VMEM((NSEG - 1, D // 2, L), u32),
            pltpu.VMEM((NSEG - 1, D // 2, L), u32),
            pltpu.VMEM((S // T, T), f32),
            pltpu.VMEM((T, T), f32),
            pltpu.VMEM((2, D, L), f32),
            pltpu.VMEM((NSEG, DP // 2, L), u32),
            pltpu.VMEM((NWIN, T + 16, T), f32),
            pltpu.VMEM((2, D, L), f32),
            pltpu.VMEM((NWIN, T + 16, T), f32),
            pltpu.VMEM((NB, T, HG * T), f32),
            pltpu.VMEM((8, F), u32),
            pltpu.SemaphoreType.DMA((11,)),
            pltpu.SemaphoreType.DMA((NSEG,)),
        ],
        compiler_params=pltpu.CompilerParams(vmem_limit_bytes=100 * 1024 * 1024),
        name="infini_moe",
    )(A_x.reshape(S, D).T, A_wq, A_wk, A_wv, A_wo, A_beta.reshape(1, H), B_w_r,
      B_w_gate, B_w_up, B_w_down.T)
    return out_t.T.reshape(1, S, D)
```

```python
import math
import os

import jax
import jax.numpy as jnp
import numpy as np
from jax import lax
import jax.experimental.pallas as pl
import jax.experimental.pallas.tpu as pltpu

S = 2048
D = 576
H = 32
DH = D // H
NSEG = 4
L = S // NSEG
F = 4608
T = 128
DP = 640
NQT = L // T
WIN = 112
NWIN = 5
HEAD_WIN = [0] * 7 + [1] * 6 + [2] * 6 + [3] * 6 + [4] * 7
WIN_HEADS = [[h for h in range(H) if HEAD_WIN[h] == t] for t in range(NWIN)]
HG = 4
NG = H // HG
GK = 80
GWIN = [HG * DH * g // 16 * 16 for g in range(NG)]
TOKROW = int(os.environ.get('TOKROW', 10))
TOKBACK = int(os.environ.get('TOKBACK', 2))
MOE0 = int(os.environ.get('MOE0', 80))
LAG = int(os.environ.get('LAG', 6))
NB = int(os.environ.get('NB', 8))
RQ, RK, RV = 0, D + 16, 2 * D + 16
NROW = 3 * D + 16
TAIL = ((0, 288), (288, 480), (480, D))
LOG2E = math.log2(math.e)
QSCALE = DH ** -0.5 * LOG2E
MASKVAL = -999292928.0 * LOG2E
LN_EPS = float(np.asarray(1e-5, dtype=jnp.bfloat16).astype(np.float32))

bf16 = jnp.bfloat16
f32 = jnp.float32
u32 = jnp.uint32


def _pack(x):
    return pltpu.bitcast(x, u32)


def _unpack(x):
    return pltpu.bitcast(x, bf16)


def _dot(a, b):
    return jnp.dot(a, b, preferred_element_type=f32)


def _dot_nt(a, b):
    return lax.dot_general(a, b, (((1,), (1,)), ((), ())), preferred_element_type=f32)


def _dot_mixed(a, b):
    return lax.dot_general(a, b, (((1,), (0,)), ((), ())), preferred_element_type=f32)


def _iota(shape, dim):
    return lax.broadcasted_iota(jnp.int32, shape, dim)


def _phi(t):
    return jnp.where(t > 0, t + 1.0, jnp.exp(t))


def _round_bf16(x):
    return x.astype(bf16).astype(f32)


def _sigmoid(x):
    return 1.0 / (1.0 + jnp.exp(-x))


def _w_tile(w_ref, i, j, tail=None):
    r = min(T, D - T * i)
    c = min(T, D - T * j)
    t = w_ref[T * i:T * i + r, T * j:T * j + c]
    if c < T:
        t = jnp.concatenate([t, jnp.zeros((r, T - c), bf16)], axis=1)
    if r < T:
        parts = [t]
        if tail is not None:
            parts.append(tail)
        n = T - sum(p.shape[0] for p in parts)
        parts.append(jnp.zeros((n, T), bf16))
        t = jnp.concatenate(parts, axis=0)
    return t


def _store_wt(dst, row0, w_ref, i, j, tail=None):
    c = min(T, D - T * j)
    t = _pack(_w_tile(w_ref, i, j, tail).T)
    r0 = (row0 + T * j) // 2
    dst[0, r0:r0 + c // 2, T * i:T * (i + 1)] = t[:c // 2]


def kernel(x_hbm, wq_hbm, wk_hbm, wv_hbm, wo_hbm, beta_hbm, wr_hbm, wg_hbm, wu_hbm, wd_hbm,
           out_hbm,
           x_v, wq_v, wk_v, wv_v, wo_v, wg_v, wu_v, wd_v, out_v,
           wt, wot, xn_s, q_s, k_s, v_s, pq_s, pk_s, r_s, g_s, o_s, ob_s, m_s, om_s, mask_s, s_s,
           h_s, acc_s, bias_s, beta_ref, wr_ref, sems, osems):
    cp_x = [pltpu.make_async_copy(x_hbm.at[:, pl.ds(s * L, L)], x_v.at[s], sems.at[s])
            for s in range(NSEG)]
    cp_o = [pltpu.make_async_copy(out_v.at[s], out_hbm.at[:, pl.ds(s * L, L)], osems.at[s])
            for s in range(NSEG - 1)]
    cp_tail = [pltpu.make_async_copy(out_v.at[NSEG - 1, pl.ds(r0, r1 - r0)],
                                     out_hbm.at[pl.ds(r0, r1 - r0), pl.ds(S - L, L)],
                                     osems.at[NSEG - 1 + c])
               for c, (r0, r1) in enumerate(TAIL)]
    cp_wk = pltpu.make_async_copy(wk_hbm, wk_v, sems.at[4])
    cp_wq = pltpu.make_async_copy(wq_hbm, wq_v, sems.at[5])
    cp_wv = pltpu.make_async_copy(wv_hbm, wv_v, sems.at[6])
    cp_wo = pltpu.make_async_copy(wo_hbm, wo_v, sems.at[7])
    cp_wg = pltpu.make_async_copy(wg_hbm, wg_v, sems.at[8])
    cp_wu = pltpu.make_async_copy(wu_hbm, wu_v, sems.at[9])
    cp_wd = pltpu.make_async_copy(wd_hbm, wd_v, sems.at[10])
    cp_beta = pltpu.make_async_copy(beta_hbm, beta_ref, sems.at[11])
    cp_wr = pltpu.make_async_copy(wr_hbm, wr_ref, sems.at[12])
    for cp in (cp_x[0], cp_beta, cp_wr, cp_wq, cp_wk, cp_x[1], cp_wv, cp_x[2], cp_x[3],
               cp_wo, cp_wg, cp_wu, cp_wd):
        cp.start()

    colh = _iota((T, T), 1)
    rowh = _iota((T, T), 0)
    for t in range(NWIN):
        same = None
        zsel = None
        for n, h in enumerate(WIN_HEADS[t]):
            cin = (colh >= DH * h - WIN * t) & (colh < DH * (h + 1) - WIN * t)
            blk = cin & (rowh >= DH * h - WIN * t) & (rowh < DH * (h + 1) - WIN * t)
            same = blk if same is None else same | blk
            zc = cin[:8] & (rowh[:8] == n)
            zsel = zc if zsel is None else zsel | zc
        mask_s[t, 0:T] = jnp.where(same, 1.0, 0.0)
        mask_s[t, T:T + 8] = jnp.where(zsel, 1.0, 0.0)
    key = _iota((T // 2, T), 0)
    qry = _iota((T // 2, T), 1)
    for c, qpos in enumerate([qry, (qry + T // 2) % T] * (HG // 2) + [qry % (T // 2)]):
        bias_s[:, T * c:T * (c + 1)] = jnp.where(qpos < key, MASKVAL, 0.0)
    for j in range(S // T):
        xn_s[j, D // 2:DP // 2, :] = jnp.zeros(((DP - D) // 2, T), u32)

    def transpose_w(row0, w):
        for j in range(5):
            for i in range(5):
                _store_wt(wt, row0, w, i, j)

    def layernorm(s, j):
        x = x_v[s, :, T * j:T * (j + 1)].astype(f32)
        mean = jnp.sum(x, axis=0, keepdims=True) / D
        c = x - mean
        var = jnp.sum(c * c, axis=0, keepdims=True) / D
        sd = _round_bf16(jnp.sqrt(_round_bf16(_round_bf16(var) + LN_EPS)))
        d = _round_bf16(x - _round_bf16(mean))
        xn_s[NQT * s + j, 0:D // 2, :] = _pack((d * (1.0 / sd)).astype(bf16))

    def xn_seg(s):
        return _unpack(jnp.concatenate([xn_s[NQT * s + j] for j in range(NQT)], axis=1))

    def proj_q(s):
        q = _dot(_unpack(wt[z, RQ // 2:RK // 2, :]), xn_seg(s))
        qp = _pack((q[:D] * QSCALE).astype(bf16))
        for h in range(H):
            a = (DH * h) // 16
            lo = (DH * h - 16 * a) // 2
            prow = _iota((16, L), 0)
            qh = jnp.where((prow >= lo) & (prow <= lo + 8), qp[8 * a:8 * a + 16], jnp.zeros((), u32))
            for j in range(NQT):
                qt = qh[:, T * j:T * (j + 1)]
                q_s[s, h, j] = pltpu.roll(qt, T // 2, 1) if h % 2 else qt
        if s > 0:
            pq_s[s - 1] = _pack(_phi(q[:D]).astype(bf16))
        for j in range(NQT):
            r_s[NQT * s + j:NQT * s + j + 1, :] = q[D:D + 1, T * j:T * (j + 1)]

    def proj_k(s):
        k = _dot(_unpack(wt[z, RK // 2:RV // 2, :]), xn_seg(s))
        if s < NSEG - 1:
            pk_s[s] = _pack(_phi(k).astype(bf16))
        for j in range(NQT):
            kb = k[:, T * j:T * (j + 1)].astype(bf16)
            for g in range(NG):
                kw = jnp.concatenate([kb[GWIN[g]:GWIN[g] + GK], jnp.zeros((T - GK, T), bf16)], axis=0)
                k_s[s, g, 64 * j:64 * (j + 1), :] = _pack(kw.T)

    def proj_v(s):
        v_s[s] = _round_bf16(_dot(_unpack(wt[z, RV // 2:NROW // 2, :]), xn_seg(s)))

    cp_x[0].wait()
    cp_beta.wait()
    cp_wr.wait()
    g = _round_bf16(_sigmoid(beta_ref[...].astype(f32)))
    z = jnp.where(jnp.max(g) > 2.0, 1, 0)
    g = jnp.concatenate([g, jnp.zeros((1, T - H), f32)], axis=1)
    g_s[...] = jnp.broadcast_to(g, (T, T)).T
    wr = wr_ref[...].reshape(1, D)
    wr = jnp.concatenate([wr, jnp.zeros((1, DP - D), bf16)], axis=1)
    wt[0, D // 2:RK // 2, :] = _pack(jnp.broadcast_to(wr, (16, DP)))
    for j in range(NQT):
        layernorm(0, j)
    cp_wq.wait()
    transpose_w(RQ, wq_v)
    proj_q(0)
    cp_wk.wait()
    cp_x[1].wait()
    transpose_w(RK, wk_v)
    for j in range(NQT):
        layernorm(1, j)
    proj_k(0)
    proj_q(1)
    cp_wv.wait()
    cp_x[2].wait()
    cp_x[3].wait()
    transpose_w(RV, wv_v)
    for j in range(NQT):
        layernorm(2, j)
    proj_k(1)
    for j in range(NQT):
        layernorm(3, j)
    proj_q(2)
    proj_q(3)

    r = _round_bf16(r_s[...])
    pos = _iota((S // T, T), 0) * T + _iota((S // T, T), 1)
    r1 = jnp.max(r)
    i1 = jnp.minimum(jnp.min(jnp.where(r == r1, pos, S)), S - 1)
    rest = pos != i1
    r2 = jnp.max(jnp.where(rest, r, -jnp.inf))
    i2 = jnp.minimum(jnp.min(jnp.where(rest & (r == r2), pos, S)), S - 1)

    for s in range(NSEG):
        if s > 1:
            proj_k(s)
        proj_v(s)

    lane = _iota((DP // 2, T), 1)
    row16 = _iota((16, T), 0)
    xsel = jnp.zeros((16, DP), f32)
    for c, idx in enumerate((i1, i2)):
        col = jnp.where(lane == idx % T, xn_s[idx // T], jnp.zeros((), u32))
        xsel = xsel + _dot_nt(jnp.where(row16 == c, 1.0, 0.0).astype(bf16), _unpack(col))

    moe = {}

    def ffn_in(w, name, cg, i):
        k = min(T, D - T * i)
        r_ = _dot(xsel[:, T * i:T * i + k].astype(bf16), w[T * i:T * i + k, L * cg:L * (cg + 1)])[:8]
        moe[name] = r_ if i == 0 else moe[name] + r_
        if name == "up" and i == 4:
            gate = moe["gate"]
            hid = gate * _sigmoid(gate) * moe["up"]
            h_s[:, L * cg:L * (cg + 1)] = _pack(
                jnp.concatenate([hid, jnp.zeros((8, L), f32)], axis=0).astype(bf16))

    def ffn_out(cg, i):
        if i < 4:
            c0 = L * cg + T * i
            r_ = _dot_nt(_unpack(h_s[:, c0:c0 + T]), wd_v[0:4 * T, c0:c0 + T])[:8]
            moe["y0"] = r_ if "y0" not in moe else moe["y0"] + r_
        else:
            r_ = _dot_nt(_unpack(h_s[:, L * cg:L * (cg + 1)]), wd_v[4 * T:D, L * cg:L * (cg + 1)])[:8]
            moe["y1"] = r_ if "y1" not in moe else moe["y1"] + r_

    def ffn_finish():
        y = jnp.concatenate([moe["y0"], moe["y1"], jnp.zeros((8, DP - D), f32)], axis=1)
        y = y * _sigmoid(jnp.where(_iota((8, DP), 0) == 0, r1, r2))
        y = jnp.concatenate([y, jnp.zeros((8, DP), f32)], axis=0)
        for j in range(5):
            _store_wt(wot, 0, wo_v, 4, j, tail=y[:, T * j:T * (j + 1)].astype(bf16))

    rounds = []
    for cg in range(F // L):
        rounds += [(ffn_in, wg_v, "gate", cg, i) for i in range(5)]
        rounds += [(ffn_in, wu_v, "up", cg, i) for i in range(5)]
        if cg > 0:
            rounds += [(ffn_out, cg - 1, i) for i in range(5)]
    rounds += [None] * 3
    rounds += [(ffn_out, F // L - 1, i) for i in range(5)]

    prow = _iota((8, T), 0)
    steps = [(s, g, j, i) for s in range(NSEG) for g in range(NG) for j in range(NQT)
             for i in range(j + 1)]
    ns = len(steps)
    mx, tok = {}, {}
    never = prow > i1 + 8
    lane8 = _iota((8, T), 1)
    hi = lane8 >= T // 2

    def q_masked(s, g, j, c):
        h = HG * g + c
        pos0 = (DH * h) // 16 - GWIN[g] // 16
        zero = jnp.zeros((8, T), u32)
        return ([zero] * pos0 + [q_s[s, h, j, 0:8], q_s[s, h, j, 8:16]]
                + [zero] * (GK // 16 - 2 - pos0))

    def k_rows(s, g, r0, r1_):
        return _unpack(k_s[s + z, g, r0 // 2:r1_ // 2, :])[:, :GK]

    def qk(n):
        s, g, j, i = steps[n]
        qm = [q_masked(s, g, j, c) for c in range(HG)]
        rows = T // 2 if i == j else T
        st = _dot(k_rows(s, g, T * i, T * i + rows),
                  _unpack(jnp.concatenate([jnp.concatenate(q, axis=0) for q in qm], axis=1)))
        m = None if i == 0 else mx[s, g, j]
        for r_ in range(rows // 8):
            x = st[8 * r_:8 * r_ + 8]
            if i == j:
                x = x + bias_s[8 * r_:8 * r_ + 8, 0:HG * T]
            s_s[n % NB, 8 * r_:8 * r_ + 8, :] = x
            m = x if m is None else jnp.maximum(m, x)
            if r_ == TOKROW * rows // T:
                tok[n] = x
        if i == j:
            ms = []
            for c in range(0, HG, 2):
                w = _unpack(jnp.concatenate(
                    [jnp.where(hi, qa, qb) for qa, qb in zip(qm[c], qm[c + 1])], axis=0))
                mp = None
                for half in range(2):
                    r0 = T // 2 + T // 4 * half
                    sx = _dot(k_rows(s, g, T * i + r0, T * i + r0 + T // 4), w)
                    for r_ in range(4):
                        x = sx[8 * r_:8 * r_ + 8] + bias_s[32 * half + 8 * r_:32 * half + 8 * r_ + 8, HG * T:]
                        s_s[n % NB, r0 + 8 * r_:r0 + 8 * r_ + 8, T * c:T * (c + 1)] = x
                        mp = x if mp is None else jnp.maximum(mp, x)
                ma, mb = m[:, T * c:T * (c + 1)], m[:, T * (c + 1):T * (c + 2)]
                ms += [jnp.where(hi, jnp.maximum(ma, mp), ma), jnp.where(hi, mb, jnp.maximum(mb, mp))]
            m = jnp.max(jnp.concatenate(ms, axis=1), axis=0, keepdims=True)
        mx[s, g, j] = m

    def pv(n):
        s, g, j, i = steps[n]
        ms = []
        for c in range(HG):
            m = jnp.broadcast_to(mx[s, g, j][:, T * c:T * (c + 1)], (8, T))
            ms.append(jnp.where(never, tok[min(n + LAG - TOKBACK, ns - 1)][:, T * c:T * (c + 1)], m))

        def probs(r0, r1_, c, m):
            m = jnp.concatenate([m] * ((r1_ - r0) // 8), axis=0)
            return jnp.exp2(s_s[n % NB, r0:r1_, T * c:T * (c + 1)] - m)

        for c in range(HG):
            if i == j:
                if c % 2 == 0:
                    px = probs(T // 2, T, c, jnp.where(hi, ms[c], ms[c + 1]))
                half = [px[8 * r_:8 * r_ + 8] for r_ in range(8)]
                half = [jnp.where(hi, 0.0, x) if c % 2 else jnp.where(hi, x, 0.0) for x in half]
                p = jnp.concatenate([probs(0, T // 2, c, ms[c])] + half, axis=0)
            else:
                p = probs(0, T, c, ms[c])
            h = HG * g + c
            a = DH * h // 8 * 8
            o = DH * h - a
            one = 23 if o == 0 else 0
            vt = [v_s[s, a + 8 * r_:a + 8 * r_ + 8, T * i:T * (i + 1)] for r_ in range(3)]
            vt[one // 8] = jnp.where(prow == one % 8, 1.0, vt[one // 8])
            r_ = _dot_mixed(jnp.concatenate(vt, axis=0), p.astype(bf16))
            if i > 0:
                r_ = acc_s[c] + r_
            if i < j:
                acc_s[c] = r_
            else:
                sc = (1.0 - g_s[h:h + 1, :]) / r_[one:one + 1]
                val = r_ * sc
                if c % 2:
                    val = pltpu.roll(val, T // 2, 1)
                o_s[s % 2, DH * h:DH * (h + 1), T * j:T * (j + 1)] = val[o:o + DH]

    def win_rows(t):
        heads = WIN_HEADS[t]
        return DH * heads[0] // 8 * 8, -(-DH * (heads[-1] + 1) // 8) * 8

    def mem_read(s, t):
        heads = WIN_HEADS[t]
        r0 = WIN * t
        ra0, re0 = win_rows(t)
        lhs = jnp.concatenate(
            [jnp.where(mask_s[t, a:b] > 0, _round_bf16(m_s[t, a:b]), 0.0)
             for a, b in ((ra0 - r0, re0 - r0), (T, T + 8))], axis=0)
        rd = _dot_mixed(lhs, _unpack(pq_s[s - 1, r0 // 2:r0 // 2 + 64, :]))
        h0 = heads[0]
        coef = jnp.concatenate([g_s[h0:h0 + 8, :]] * NQT, axis=1) / (rd[re0 - ra0:] + 1e-6)
        lo_row = DH * heads[0]
        hi_row = DH * (heads[-1] + 1)
        for rb in range(ra0, re0, 8):
            ha = max(rb // DH, h0)
            hb = min((rb + 7) // DH, heads[-1])
            cf = jnp.broadcast_to(coef[ha - h0:ha - h0 + 1], (8, L))
            if hb != ha:
                cf = jnp.where(_iota((8, L), 0) < DH * hb - rb, cf,
                               jnp.broadcast_to(coef[hb - h0:hb - h0 + 1], (8, L)))
            val = rd[rb - ra0:rb - ra0 + 8] * cf
            ra, re = max(rb, lo_row), min(rb + 8, hi_row)
            om_s[s % 2, ra:re, :] = val[ra - rb:re - rb]

    def mem_update(s, t):
        r0 = WIN * t
        ra0, re0 = win_rows(t)
        vl = jnp.concatenate([v_s[s, ra0:re0, :], jnp.ones((8, L), f32)], axis=0)
        upd = lax.dot_general(vl, _unpack(pk_s[s, r0 // 2:r0 // 2 + 64, :]),
                              (((1,), (1,)), ((), ())), preferred_element_type=f32)
        for a, b, u in ((ra0 - r0, re0 - r0, upd[:re0 - ra0]), (T, T + 8, upd[re0 - ra0:])):
            m_s[t, a:b] = u if s == 0 else m_s[t, a:b] + u

    def pack_o(s, r0, r1_):
        o = o_s[s % 2, r0:r1_, :]
        if s > 0:
            o = o + om_s[s % 2, r0:r1_, :]
        ob_s[s, r0 // 2:r1_ // 2, :] = _pack(o.astype(bf16))

    def out_proj(s, r0, r1_):
        res = _dot(_unpack(wot[z, r0 // 2:r1_ // 2, :]), _unpack(ob_s[s]))
        xn = _unpack(jnp.concatenate(
            [xn_s[NQT * s + j, r0 // 2:r1_ // 2, :] for j in range(NQT)], axis=1))
        out_v[s, r0:r1_, :] = (res + x_v[s, r0:r1_, :].astype(f32) + xn.astype(f32)).astype(bf16)

    for s in range(NSEG):
        tpos = _iota((16, L), 1) + s * L
        sel = jnp.where(_iota((16, L), 0) == 0, i1, jnp.where(_iota((16, L), 0) == 1, i2, -1))
        ob_s[s, D // 2:D // 2 + 8, :] = _pack(jnp.where(tpos == sel, 1.0, 0.0).astype(bf16))
        ob_s[s, D // 2 + 8:DP // 2, :] = jnp.zeros(((DP - D) // 2 - 8, L), u32)

    extra = {}

    def at(n, fn, *args):
        extra.setdefault(n, []).append((fn,) + args)

    per = ns // NSEG
    for t in range(NWIN):
        at(t, mem_update, 0, t)
        for s in range(1, NSEG):
            at(per * s - 40 + 4 * t, mem_read, s, t)
            if s < NSEG - 1:
                at(per * s + 10 + 4 * t, mem_update, s, t)

    def late_weights():
        for cp in (cp_wo, cp_wg, cp_wu, cp_wd):
            cp.wait()
        for j in range(5):
            for i in range(4):
                _store_wt(wot, 0, wo_v, i, j)

    at(MOE0, late_weights)
    for k, rd_ in enumerate(rounds):
        if rd_ is not None:
            at(MOE0 + k, *rd_)
    done = MOE0 + len(rounds) + 2
    at(done, ffn_finish)
    at(done + 5, out_proj, 0, 0, D)
    at(done + 6, cp_o[0].start)
    at(done + 10, out_proj, 1, 0, D)
    at(done + 11, cp_o[1].start)
    for s in range(NSEG - 1):
        for c in range(4):
            at(per * s + 20 * (c + 1) + LAG + 1, pack_o, s, 144 * c, 144 * (c + 1))
    for c in range(3):
        at(per * 3 + 20 * (c + 1) + LAG + 1, pack_o, 3, 144 * c, 144 * (c + 1))
    for c, (r0, r1_) in enumerate(((0, 112), (112, 224), (224, 336), (336, 448), (448, D))):
        at(ns + c + LAG - 5, out_proj, 2, r0, r1_)

    for n in range(ns + LAG):
        if n < ns:
            qk(n)
        for task in extra.get(n, ()):
            if task[0] is not ffn_in:
                task[0](*task[1:])
        if n >= LAG:
            pv(n - LAG)
        for task in extra.get(n, ()):
            if task[0] is ffn_in:
                task[0](*task[1:])
    cp_o[2].start()
    pack_o(3, 432, D)
    for (r0, r1_), cp in zip(TAIL, cp_tail):
        out_proj(NSEG - 1, r0, r1_)
        cp.start()
    for cp in cp_o + cp_tail:
        cp.wait()


@jax.jit
def pallas_parallel_sum__memory_aug_infini_attn__moe_arch_mod__prompt_kernel(
    A_x, A_wq, A_wk, A_wv, A_wo, A_beta, B_x, B_w_r, B_w_gate, B_w_up, B_w_down,
):
    del B_x
    any_spec = pl.BlockSpec(memory_space=pl.ANY)
    out_t = pl.pallas_call(
        kernel,
        out_shape=jax.ShapeDtypeStruct((D, S), bf16),
        in_specs=[any_spec] * 10,
        out_specs=any_spec,
        scratch_shapes=[
            pltpu.VMEM((NSEG, D, L), bf16),
            pltpu.VMEM((D, D), bf16),
            pltpu.VMEM((D, D), bf16),
            pltpu.VMEM((D, D), bf16),
            pltpu.VMEM((D, D), bf16),
            pltpu.VMEM((D, F), bf16),
            pltpu.VMEM((D, F), bf16),
            pltpu.VMEM((D, F), bf16),
            pltpu.VMEM((NSEG, D, L), bf16),
            pltpu.VMEM((1, NROW // 2, DP), u32),
            pltpu.VMEM((1, D // 2, DP), u32),
            pltpu.VMEM((S // T, DP // 2, T), u32),
            pltpu.VMEM((NSEG, H, NQT, 16, T), u32),
            pltpu.VMEM((NSEG, NG, L // 2, T), u32),
            pltpu.VMEM((NSEG, D, L), f32),
            pltpu.VMEM((NSEG - 1, D // 2, L), u32),
            pltpu.VMEM((NSEG - 1, D // 2, L), u32),
            pltpu.VMEM((S // T, T), f32),
            pltpu.VMEM((T, T), f32),
            pltpu.VMEM((2, D, L), f32),
            pltpu.VMEM((NSEG, DP // 2, L), u32),
            pltpu.VMEM((NWIN, T + 8, T), f32),
            pltpu.VMEM((2, D, L), f32),
            pltpu.VMEM((NWIN, T + 8, T), f32),
            pltpu.VMEM((NB, T, HG * T), f32),
            pltpu.VMEM((8, F), u32),
            pltpu.VMEM((HG, 24, T), f32),
            pltpu.VMEM((T // 2, (HG + 1) * T), f32),
            pltpu.VMEM((1, H), bf16),
            pltpu.VMEM((D,), bf16),
            pltpu.SemaphoreType.DMA((13,)),
            pltpu.SemaphoreType.DMA((NSEG - 1 + len(TAIL),)),
        ],
        compiler_params=pltpu.CompilerParams(vmem_limit_bytes=100 * 1024 * 1024),
        name="infini_moe",
    )(A_x.reshape(S, D).T, A_wq, A_wk, A_wv, A_wo, A_beta.reshape(1, H), B_w_r,
      B_w_gate, B_w_up, B_w_down.T)
    return out_t.T.reshape(1, S, D)
```

```python
import math
import os

import jax
import jax.numpy as jnp
import numpy as np
from jax import lax
import jax.experimental.pallas as pl
import jax.experimental.pallas.tpu as pltpu

S = 2048
D = 576
H = 32
DH = D // H
NSEG = 4
L = S // NSEG
F = 4608
T = 128
DP = 640
NQT = L // T
WIN = 112
NWIN = 5
HEAD_WIN = [0] * 7 + [1] * 6 + [2] * 6 + [3] * 6 + [4] * 7
WIN_HEADS = [[h for h in range(H) if HEAD_WIN[h] == t] for t in range(NWIN)]
HG = 4
NG = H // HG
GK = 80
GWIN = [HG * DH * g // 16 * 16 for g in range(NG)]
TOKROW = int(os.environ.get('TOKROW', 10))
TOKBACK = int(os.environ.get('TOKBACK', 2))
MOE0 = int(os.environ.get('MOE0', 80))
LAG = int(os.environ.get('LAG', 6))
NB = int(os.environ.get('NB', 8))
RQ, RK, RV = 0, D + 16, 2 * D + 16
NROW = 3 * D + 16
FILL = int(os.environ.get('FILL', 48))
VSPLIT = int(os.environ.get('VSPLIT', 448))
TAIL = ((0, 288), (288, 480), (480, D))
LOG2E = math.log2(math.e)
QSCALE = DH ** -0.5 * LOG2E
MASKVAL = -999292928.0 * LOG2E
LN_EPS = float(np.asarray(1e-5, dtype=jnp.bfloat16).astype(np.float32))

bf16 = jnp.bfloat16
f32 = jnp.float32
u32 = jnp.uint32


def _pack(x):
    return pltpu.bitcast(x, u32)


def _unpack(x):
    return pltpu.bitcast(x, bf16)


def _halves(x):
    return [pltpu.unpack_elementwise(x, index=i, packed_dtype=bf16, unpacked_dtype=f32)
            for i in range(2)]


def _join(even, odd):
    return pltpu.bitcast(pltpu.pack_elementwise([even, odd], packed_dtype=bf16), u32)


def _dot(a, b):
    return jnp.dot(a, b, preferred_element_type=f32)


def _dot_nt(a, b):
    return lax.dot_general(a, b, (((1,), (1,)), ((), ())), preferred_element_type=f32)


def _dot_mixed(a, b):
    return lax.dot_general(a, b, (((1,), (0,)), ((), ())), preferred_element_type=f32)


def _iota(shape, dim):
    return lax.broadcasted_iota(jnp.int32, shape, dim)


def _phi(t):
    return jnp.where(t > 0, t + 1.0, jnp.exp(t))


def _round_bf16(x):
    return x.astype(bf16).astype(f32)


def _sigmoid(x):
    return 1.0 / (1.0 + jnp.exp(-x))


def _w_tile(w_ref, i, j, tail=None):
    r = min(T, D - T * i)
    c = min(T, D - T * j)
    t = w_ref[T * i:T * i + r, T * j:T * j + c]
    if c < T:
        t = jnp.concatenate([t, jnp.zeros((r, T - c), bf16)], axis=1)
    if r < T:
        parts = [t]
        if tail is not None:
            parts.append(tail)
        n = T - sum(p.shape[0] for p in parts)
        parts.append(jnp.zeros((n, T), bf16))
        t = jnp.concatenate(parts, axis=0)
    return t


def _store_wt(dst, row0, w_ref, i, j, tail=None):
    c = min(T, D - T * j)
    t = _pack(_w_tile(w_ref, i, j, tail).T)
    r0 = (row0 + T * j) // 2
    dst[0, r0:r0 + c // 2, T * i:T * (i + 1)] = t[:c // 2]


def kernel(x_hbm, wq_hbm, wk_hbm, wv_hbm, wo_hbm, beta_hbm, wr_hbm, wg_hbm, wu_hbm, wd_hbm,
           out_hbm,
           x_v, wq_v, wk_v, wv_v, wo_v, wg_v, wu_v, wd_v, out_v,
           wt, wot, xn_s, q_s, k_s, v_s, pq_s, pk_s, r_s, g_s, o_s, ob_s, m_s, om_s, mask_s, s_s,
           h_s, acc_s, bias_s, beta_ref, wr_ref, sems, osems):
    cp_x = [pltpu.make_async_copy(x_hbm.at[:, pl.ds(s * L, L)], x_v.at[s], sems.at[s])
            for s in range(NSEG)]
    cp_o = [pltpu.make_async_copy(out_v.at[s], out_hbm.at[:, pl.ds(s * L, L)], osems.at[s])
            for s in range(NSEG - 1)]
    cp_tail = [pltpu.make_async_copy(out_v.at[NSEG - 1, pl.ds(r0, r1 - r0)],
                                     out_hbm.at[pl.ds(r0, r1 - r0), pl.ds(S - L, L)],
                                     osems.at[NSEG - 1 + c])
               for c, (r0, r1) in enumerate(TAIL)]
    cp_wk = pltpu.make_async_copy(wk_hbm, wk_v, sems.at[4])
    cp_wq = pltpu.make_async_copy(wq_hbm, wq_v, sems.at[5])
    cp_wv = pltpu.make_async_copy(wv_hbm, wv_v, sems.at[6])
    cp_wo = pltpu.make_async_copy(wo_hbm, wo_v, sems.at[7])
    cp_wg = pltpu.make_async_copy(wg_hbm, wg_v, sems.at[8])
    cp_wu = pltpu.make_async_copy(wu_hbm, wu_v, sems.at[9])
    cp_wd = pltpu.make_async_copy(wd_hbm, wd_v, sems.at[10])
    cp_beta = pltpu.make_async_copy(beta_hbm, beta_ref, sems.at[11])
    cp_wr = pltpu.make_async_copy(wr_hbm, wr_ref, sems.at[12])
    for cp in (cp_x[0], cp_beta, cp_wr, cp_wv, cp_wq, cp_x[1], cp_wk, cp_x[2], cp_x[3],
               cp_wo, cp_wg, cp_wu, cp_wd):
        cp.start()

    colh = _iota((T, T), 1)
    rowh = _iota((T, T), 0)
    for t in range(NWIN):
        same = None
        zsel = None
        for n, h in enumerate(WIN_HEADS[t]):
            cin = (colh >= DH * h - WIN * t) & (colh < DH * (h + 1) - WIN * t)
            blk = cin & (rowh >= DH * h - WIN * t) & (rowh < DH * (h + 1) - WIN * t)
            same = blk if same is None else same | blk
            zc = cin[:8] & (rowh[:8] == n)
            zsel = zc if zsel is None else zsel | zc
        mask_s[t, 0:T] = jnp.where(same, 1.0, 0.0)
        mask_s[t, T:T + 8] = jnp.where(zsel, 1.0, 0.0)
    key = _iota((T // 2, T), 0)
    qry = _iota((T // 2, T), 1)
    for c, qpos in enumerate([qry, (qry + T // 2) % T] * (HG // 2) + [qry % (T // 2)]):
        bias_s[:, T * c:T * (c + 1)] = jnp.where(qpos < key, MASKVAL, 0.0)
    for j in range(S // T):
        xn_s[j, D // 2:DP // 2, :] = jnp.zeros(((DP - D) // 2, T), u32)

    def transpose_w(row0, w):
        for j in range(5):
            for i in range(5):
                _store_wt(wt, row0, w, i, j)

    def layernorm(s, j):
        xe, xo = _halves(_pack(x_v[s, :, T * j:T * (j + 1)]))
        mean = jnp.sum(xe + xo, axis=0, keepdims=True) / D
        ce, co = xe - mean, xo - mean
        var = jnp.sum(ce * ce + co * co, axis=0, keepdims=True) / D
        inv = 1.0 / _round_bf16(jnp.sqrt(_round_bf16(_round_bf16(var) + LN_EPS)))
        mean = _round_bf16(mean)
        de, do = _halves(_join(xe - mean, xo - mean))
        xn_s[NQT * s + j, 0:D // 2, :] = _join(de * inv, do * inv)

    def xn_seg(s):
        return _unpack(jnp.concatenate([xn_s[NQT * s + j] for j in range(NQT)], axis=1))

    def proj_q(s):
        q = _dot(_unpack(wt[z, RQ // 2:RK // 2, :]), xn_seg(s))
        for j in range(NQT):
            r_s[NQT * s + j:NQT * s + j + 1, :] = q[D:D + 1, T * j:T * (j + 1)]
        if s > 0:
            pq_s[s - 1] = _pack(_phi(q[:D]).astype(bf16))
        qp = _pack((q[:D] * QSCALE).astype(bf16))
        for h in range(H):
            a = (DH * h) // 16
            lo = (DH * h - 16 * a) // 2
            prow = _iota((16, L), 0)
            qh = jnp.where((prow >= lo) & (prow <= lo + 8), qp[8 * a:8 * a + 16], jnp.zeros((), u32))
            for j in range(NQT):
                qt = qh[:, T * j:T * (j + 1)]
                q_s[s, h, j] = pltpu.roll(qt, T // 2, 1) if h % 2 else qt

    def proj_k(s):
        k = _dot(_unpack(wt[z, RK // 2:RV // 2, :]), xn_seg(s))
        if s < NSEG - 1:
            pk_s[s] = _pack(_phi(k).astype(bf16))
        for j in range(NQT):
            kb = k[:, T * j:T * (j + 1)].astype(bf16)
            for g in range(NG):
                kw = jnp.concatenate([kb[GWIN[g]:GWIN[g] + GK], jnp.zeros((T - GK, T), bf16)], axis=0)
                k_s[s, g, 64 * j:64 * (j + 1), :] = _pack(kw.T)

    def proj_v(s, r0=0, r1_=D):
        v_s[s, r0:r1_, :] = _round_bf16(
            _dot(_unpack(wt[z, (RV + r0) // 2:(RV + r1_) // 2, :]), xn_seg(s)))

    cp_x[0].wait()
    cp_beta.wait()
    cp_wr.wait()
    g = _round_bf16(_sigmoid(beta_ref[...].astype(f32)))
    z = jnp.where(jnp.max(g) > 2.0, 1, 0)
    g = jnp.concatenate([g, jnp.zeros((1, T - H), f32)], axis=1)
    g_s[...] = jnp.broadcast_to(g, (T, T)).T
    wr = wr_ref[...].reshape(1, D)
    wr = jnp.concatenate([wr, jnp.zeros((1, DP - D), bf16)], axis=1)
    wt[0, D // 2:RK // 2, :] = _pack(jnp.broadcast_to(wr, (16, DP)))
    for j in range(NQT):
        layernorm(0, j)
    cp_wv.wait()
    transpose_w(RV, wv_v)
    proj_v(0, 0, 416)
    cp_wq.wait()
    transpose_w(RQ, wq_v)
    proj_v(0, 416, 496)
    proj_q(0)
    cp_x[1].wait()
    cp_wk.wait()
    transpose_w(RK, wk_v)
    for j in range(NQT):
        layernorm(1, j)
    proj_v(0, 496, D)
    proj_k(0)
    proj_v(1)
    cp_x[2].wait()
    cp_x[3].wait()
    for j in range(NQT):
        layernorm(2, j)
    proj_q(1)
    for j in range(NQT):
        layernorm(3, j)
    proj_q(2)
    proj_q(3)

    r = _round_bf16(r_s[...])
    pos = _iota((S // T, T), 0) * T + _iota((S // T, T), 1)
    r1 = jnp.max(r)
    i1 = jnp.minimum(jnp.min(jnp.where(r == r1, pos, S)), S - 1)
    rest = pos != i1
    r2 = jnp.max(jnp.where(rest, r, -jnp.inf))
    i2 = jnp.minimum(jnp.min(jnp.where(rest & (r == r2), pos, S)), S - 1)

    for s in range(1, NSEG):
        proj_k(s)
        if s > 1:
            proj_v(s)

    lane = _iota((DP // 2, T), 1)
    row16 = _iota((16, T), 0)
    xsel = jnp.zeros((16, DP), f32)
    for c, idx in enumerate((i1, i2)):
        col = jnp.where(lane == idx % T, xn_s[idx // T], jnp.zeros((), u32))
        xsel = xsel + _dot_nt(jnp.where(row16 == c, 1.0, 0.0).astype(bf16), _unpack(col))

    moe = {}

    def ffn_in(w, name, cg, i):
        k = min(T, D - T * i)
        r_ = _dot(xsel[:, T * i:T * i + k].astype(bf16), w[T * i:T * i + k, L * cg:L * (cg + 1)])[:8]
        moe[name] = r_ if i == 0 else moe[name] + r_
        if name == "up" and i == 4:
            gate = moe["gate"]
            hid = gate * _sigmoid(gate) * moe["up"]
            h_s[:, L * cg:L * (cg + 1)] = _pack(
                jnp.concatenate([hid, jnp.zeros((8, L), f32)], axis=0).astype(bf16))

    def ffn_out(cg, i):
        if i < 4:
            c0 = L * cg + T * i
            r_ = _dot_nt(_unpack(h_s[:, c0:c0 + T]), wd_v[0:4 * T, c0:c0 + T])[:8]
            moe["y0"] = r_ if "y0" not in moe else moe["y0"] + r_
        else:
            r_ = _dot_nt(_unpack(h_s[:, L * cg:L * (cg + 1)]), wd_v[4 * T:D, L * cg:L * (cg + 1)])[:8]
            moe["y1"] = r_ if "y1" not in moe else moe["y1"] + r_

    def ffn_finish():
        y = jnp.concatenate([moe["y0"], moe["y1"], jnp.zeros((8, DP - D), f32)], axis=1)
        y = y * _sigmoid(jnp.where(_iota((8, DP), 0) == 0, r1, r2))
        y = jnp.concatenate([y, jnp.zeros((8, DP), f32)], axis=0)
        for j in range(5):
            _store_wt(wot, 0, wo_v, 4, j, tail=y[:, T * j:T * (j + 1)].astype(bf16))

    rounds = []
    for cg in range(F // L):
        rounds += [(ffn_in, wg_v, "gate", cg, i) for i in range(5)]
        rounds += [(ffn_in, wu_v, "up", cg, i) for i in range(5)]
        if cg > 0:
            rounds += [(ffn_out, cg - 1, i) for i in range(5)]
    rounds += [None] * 3
    rounds += [(ffn_out, F // L - 1, i) for i in range(5)]

    prow = _iota((8, T), 0)
    steps = [(s, g, j, i) for s in range(NSEG) for g in range(NG) for j in range(NQT)
             for i in range(j + 1)]
    ns = len(steps)
    mx, tok = {}, {}
    never = prow > i1 + 8
    lane8 = _iota((8, T), 1)
    hi = lane8 >= T // 2

    def q_masked(s, g, j, c):
        h = HG * g + c
        pos0 = (DH * h) // 16 - GWIN[g] // 16
        zero = jnp.zeros((8, T), u32)
        return ([zero] * pos0 + [q_s[s, h, j, 0:8], q_s[s, h, j, 8:16]]
                + [zero] * (GK // 16 - 2 - pos0))

    def k_rows(s, g, r0, r1_):
        return _unpack(k_s[s + z, g, r0 // 2:r1_ // 2, :])[:, :GK]

    def qk(n):
        s, g, j, i = steps[n]
        qm = [q_masked(s, g, j, c) for c in range(HG)]
        rows = T // 2 if i == j else T
        st = _dot(k_rows(s, g, T * i, T * i + rows),
                  _unpack(jnp.concatenate([jnp.concatenate(q, axis=0) for q in qm], axis=1)))
        m = None if i == 0 else mx[s, g, j]
        for r_ in range(rows // 8):
            x = st[8 * r_:8 * r_ + 8]
            if i == j:
                x = x + bias_s[8 * r_:8 * r_ + 8, 0:HG * T]
            s_s[n % NB, 8 * r_:8 * r_ + 8, :] = x
            m = x if m is None else jnp.maximum(m, x)
            if r_ == TOKROW * rows // T:
                tok[n] = x
        if i == j:
            ms = []
            for c in range(0, HG, 2):
                w = _unpack(jnp.concatenate(
                    [jnp.where(hi, qa, qb) for qa, qb in zip(qm[c], qm[c + 1])], axis=0))
                mp = None
                for half in range(2):
                    r0 = T // 2 + T // 4 * half
                    sx = _dot(k_rows(s, g, T * i + r0, T * i + r0 + T // 4), w)
                    for r_ in range(4):
                        x = sx[8 * r_:8 * r_ + 8] + bias_s[32 * half + 8 * r_:32 * half + 8 * r_ + 8, HG * T:]
                        s_s[n % NB, r0 + 8 * r_:r0 + 8 * r_ + 8, T * c:T * (c + 1)] = x
                        mp = x if mp is None else jnp.maximum(mp, x)
                ma, mb = m[:, T * c:T * (c + 1)], m[:, T * (c + 1):T * (c + 2)]
                ms += [jnp.where(hi, jnp.maximum(ma, mp), ma), jnp.where(hi, mb, jnp.maximum(mb, mp))]
            m = jnp.max(jnp.concatenate(ms, axis=1), axis=0, keepdims=True)
        mx[s, g, j] = m

    def pv(n):
        s, g, j, i = steps[n]
        ms = []
        for c in range(HG):
            m = jnp.broadcast_to(mx[s, g, j][:, T * c:T * (c + 1)], (8, T))
            ms.append(jnp.where(never, tok[min(n + LAG - TOKBACK, ns - 1)][:, T * c:T * (c + 1)], m))

        def probs(r0, r1_, c, m):
            m = jnp.concatenate([m] * ((r1_ - r0) // 8), axis=0)
            return jnp.exp2(s_s[n % NB, r0:r1_, T * c:T * (c + 1)] - m)

        for c in range(HG):
            if i == j:
                if c % 2 == 0:
                    px = probs(T // 2, T, c, jnp.where(hi, ms[c], ms[c + 1]))
                half = [px[8 * r_:8 * r_ + 8] for r_ in range(8)]
                half = [jnp.where(hi, 0.0, x) if c % 2 else jnp.where(hi, x, 0.0) for x in half]
                p = jnp.concatenate([probs(0, T // 2, c, ms[c])] + half, axis=0)
            else:
                p = probs(0, T, c, ms[c])
            h = HG * g + c
            a = DH * h // 8 * 8
            o = DH * h - a
            one = 23 if o == 0 else 0
            vt = [v_s[s, a + 8 * r_:a + 8 * r_ + 8, T * i:T * (i + 1)] for r_ in range(3)]
            vt[one // 8] = jnp.where(prow == one % 8, 1.0, vt[one // 8])
            r_ = _dot_mixed(jnp.concatenate(vt, axis=0), p.astype(bf16))
            if i > 0:
                r_ = acc_s[c] + r_
            if i < j:
                acc_s[c] = r_
            else:
                sc = (1.0 - g_s[h:h + 1, :]) / r_[one:one + 1]
                val = r_ * sc
                if c % 2:
                    val = pltpu.roll(val, T // 2, 1)
                o_s[s % 2, DH * h:DH * (h + 1), T * j:T * (j + 1)] = val[o:o + DH]

    def win_rows(t):
        heads = WIN_HEADS[t]
        return DH * heads[0] // 8 * 8, -(-DH * (heads[-1] + 1) // 8) * 8

    def mem_read(s, t):
        heads = WIN_HEADS[t]
        r0 = WIN * t
        ra0, re0 = win_rows(t)
        lhs = jnp.concatenate(
            [jnp.where(mask_s[t, a:b] > 0, _round_bf16(m_s[t, a:b]), 0.0)
             for a, b in ((ra0 - r0, re0 - r0), (T, T + 8))], axis=0)
        rd = _dot_mixed(lhs, _unpack(pq_s[s - 1, r0 // 2:r0 // 2 + 64, :]))
        h0 = heads[0]
        coef = jnp.concatenate([g_s[h0:h0 + 8, :]] * NQT, axis=1) / (rd[re0 - ra0:] + 1e-6)
        lo_row = DH * heads[0]
        hi_row = DH * (heads[-1] + 1)
        for rb in range(ra0, re0, 8):
            ha = max(rb // DH, h0)
            hb = min((rb + 7) // DH, heads[-1])
            cf = jnp.broadcast_to(coef[ha - h0:ha - h0 + 1], (8, L))
            if hb != ha:
                cf = jnp.where(_iota((8, L), 0) < DH * hb - rb, cf,
                               jnp.broadcast_to(coef[hb - h0:hb - h0 + 1], (8, L)))
            val = rd[rb - ra0:rb - ra0 + 8] * cf
            ra, re = max(rb, lo_row), min(rb + 8, hi_row)
            om_s[s % 2, ra:re, :] = val[ra - rb:re - rb]

    def mem_update(s, t):
        r0 = WIN * t
        ra0, re0 = win_rows(t)
        vl = jnp.concatenate([v_s[s, ra0:re0, :], jnp.ones((8, L), f32)], axis=0)
        upd = lax.dot_general(vl, _unpack(pk_s[s, r0 // 2:r0 // 2 + 64, :]),
                              (((1,), (1,)), ((), ())), preferred_element_type=f32)
        for a, b, u in ((ra0 - r0, re0 - r0, upd[:re0 - ra0]), (T, T + 8, upd[re0 - ra0:])):
            m_s[t, a:b] = u if s == 0 else m_s[t, a:b] + u

    def pack_o(s, r0, r1_):
        o = o_s[s % 2, r0:r1_, :]
        if s > 0:
            o = o + om_s[s % 2, r0:r1_, :]
        ob_s[s, r0 // 2:r1_ // 2, :] = _pack(o.astype(bf16))

    def out_proj(s, r0, r1_):
        res = _dot(_unpack(wot[z, r0 // 2:r1_ // 2, :]), _unpack(ob_s[s]))
        xn = _unpack(jnp.concatenate(
            [xn_s[NQT * s + j, r0 // 2:r1_ // 2, :] for j in range(NQT)], axis=1))
        out_v[s, r0:r1_, :] = (res + x_v[s, r0:r1_, :].astype(f32) + xn.astype(f32)).astype(bf16)

    for s in range(NSEG):
        tpos = _iota((16, L), 1) + s * L
        sel = jnp.where(_iota((16, L), 0) == 0, i1, jnp.where(_iota((16, L), 0) == 1, i2, -1))
        ob_s[s, D // 2:D // 2 + 8, :] = _pack(jnp.where(tpos == sel, 1.0, 0.0).astype(bf16))
        ob_s[s, D // 2 + 8:DP // 2, :] = jnp.zeros(((DP - D) // 2 - 8, L), u32)

    extra = {}

    def at(n, fn, *args):
        extra.setdefault(n, []).append((fn,) + args)

    per = ns // NSEG
    for t in range(NWIN):
        at(t, mem_update, 0, t)
        for s in range(1, NSEG):
            at(per * s - 40 + 4 * t, mem_read, s, t)
            if s < NSEG - 1:
                at(per * s + 10 + 4 * t, mem_update, s, t)

    def late_weights():
        for cp in (cp_wo, cp_wg, cp_wu, cp_wd):
            cp.wait()
        for j in range(5):
            for i in range(4):
                _store_wt(wot, 0, wo_v, i, j)

    at(MOE0, late_weights)
    for k, rd_ in enumerate(rounds):
        if rd_ is not None:
            at(MOE0 + k, *rd_)
    done = MOE0 + len(rounds) + 2
    at(done, ffn_finish)
    for s in range(NSEG - 1):
        for c in range(4):
            at(per * s + 20 * (c + 1) + LAG + 1, pack_o, s, 144 * c, 144 * (c + 1))
    for c in range(3):
        at(per * (NSEG - 1) + 20 * (c + 1) + LAG + 1, pack_o, NSEG - 1, 144 * c, 144 * (c + 1))
    for c in range(LAG):
        at(ns + c, out_proj, 0, FILL * c, FILL * (c + 1))

    for n in range(ns + LAG):
        if n < ns:
            qk(n)
        for task in extra.get(n, ()):
            if task[0] is not ffn_in:
                task[0](*task[1:])
        if n >= LAG:
            pv(n - LAG)
        for task in extra.get(n, ()):
            if task[0] is ffn_in:
                task[0](*task[1:])
    pack_o(NSEG - 1, 432, D)
    for s in range(NSEG - 1):
        out_proj(s, FILL * LAG if s == 0 else 0, D)
        cp_o[s].start()
    for (r0, r1_), cp in zip(TAIL, cp_tail):
        out_proj(NSEG - 1, r0, r1_)
        cp.start()
    for cp in cp_o + cp_tail:
        cp.wait()


@jax.jit
def pallas_parallel_sum__memory_aug_infini_attn__moe_arch_mod__prompt_kernel(
    A_x, A_wq, A_wk, A_wv, A_wo, A_beta, B_x, B_w_r, B_w_gate, B_w_up, B_w_down,
):
    del B_x
    any_spec = pl.BlockSpec(memory_space=pl.ANY)
    out_t = pl.pallas_call(
        kernel,
        out_shape=jax.ShapeDtypeStruct((D, S), bf16),
        in_specs=[any_spec] * 10,
        out_specs=any_spec,
        scratch_shapes=[
            pltpu.VMEM((NSEG, D, L), bf16),
            pltpu.VMEM((D, D), bf16),
            pltpu.VMEM((D, D), bf16),
            pltpu.VMEM((D, D), bf16),
            pltpu.VMEM((D, D), bf16),
            pltpu.VMEM((D, F), bf16),
            pltpu.VMEM((D, F), bf16),
            pltpu.VMEM((D, F), bf16),
            pltpu.VMEM((NSEG, D, L), bf16),
            pltpu.VMEM((1, NROW // 2, DP), u32),
            pltpu.VMEM((1, D // 2, DP), u32),
            pltpu.VMEM((S // T, DP // 2, T), u32),
            pltpu.VMEM((NSEG, H, NQT, 16, T), u32),
            pltpu.VMEM((NSEG, NG, L // 2, T), u32),
            pltpu.VMEM((NSEG, D, L), f32),
            pltpu.VMEM((NSEG - 1, D // 2, L), u32),
            pltpu.VMEM((NSEG - 1, D // 2, L), u32),
            pltpu.VMEM((S // T, T), f32),
            pltpu.VMEM((T, T), f32),
            pltpu.VMEM((2, D, L), f32),
            pltpu.VMEM((NSEG, DP // 2, L), u32),
            pltpu.VMEM((NWIN, T + 8, T), f32),
            pltpu.VMEM((2, D, L), f32),
            pltpu.VMEM((NWIN, T + 8, T), f32),
            pltpu.VMEM((NB, T, HG * T), f32),
            pltpu.VMEM((8, F), u32),
            pltpu.VMEM((HG, 24, T), f32),
            pltpu.VMEM((T // 2, (HG + 1) * T), f32),
            pltpu.VMEM((1, H), bf16),
            pltpu.VMEM((D,), bf16),
            pltpu.SemaphoreType.DMA((13,)),
            pltpu.SemaphoreType.DMA((NSEG - 1 + len(TAIL),)),
        ],
        compiler_params=pltpu.CompilerParams(vmem_limit_bytes=100 * 1024 * 1024),
        name="infini_moe",
    )(A_x.reshape(S, D).T, A_wq, A_wk, A_wv, A_wo, A_beta.reshape(1, H), B_w_r,
      B_w_gate, B_w_up, B_w_down.T)
    return out_t.T.reshape(1, S, D)
```

```python
import math
import os

import jax
import jax.numpy as jnp
import numpy as np
from jax import lax
import jax.experimental.pallas as pl
import jax.experimental.pallas.tpu as pltpu

S = 2048
D = 576
H = 32
DH = D // H
NSEG = 4
L = S // NSEG
F = 4608
T = 128
DP = 640
NQT = L // T
WIN = 112
NWIN = 5
HEAD_WIN = [0] * 7 + [1] * 6 + [2] * 6 + [3] * 6 + [4] * 7
WIN_HEADS = [[h for h in range(H) if HEAD_WIN[h] == t] for t in range(NWIN)]
HG = 4
NG = H // HG
AFTER = int(os.environ.get('AFTER', 1))
PINBACK = int(os.environ.get('PINBACK', 2))
ETOK = int(os.environ.get('ETOK', 2))
DUE = int(os.environ.get('DUE', 10))
QB = T // HG
MERGE = int(os.environ.get('MERGE', 1))
GK = 80
GWIN = [HG * DH * g // 16 * 16 for g in range(NG)]
TOKROW = int(os.environ.get('TOKROW', 10))
TOKBACK = int(os.environ.get('TOKBACK', 2))
MOE0 = int(os.environ.get('MOE0', 61))
LAG = int(os.environ.get('LAG', 11))
NB = int(os.environ.get('NB', 13))
RQ, RK, RV = 0, D + 16, 2 * D + 16
NROW = 3 * D + 16
FILL = int(os.environ.get('FILL', 48))
VSPLIT = int(os.environ.get('VSPLIT', 448))
TAIL = ((0, 288), (288, 480), (480, D))
LOG2E = math.log2(math.e)
QSCALE = DH ** -0.5 * LOG2E
MASKVAL = -999292928.0 * LOG2E
LN_EPS = float(np.asarray(1e-5, dtype=jnp.bfloat16).astype(np.float32))

bf16 = jnp.bfloat16
f32 = jnp.float32
u32 = jnp.uint32


def _pack(x):
    return pltpu.bitcast(x, u32)


def _unpack(x):
    return pltpu.bitcast(x, bf16)


def _halves(x):
    return [pltpu.unpack_elementwise(x, index=i, packed_dtype=bf16, unpacked_dtype=f32)
            for i in range(2)]


def _join(even, odd):
    return pltpu.bitcast(pltpu.pack_elementwise([even, odd], packed_dtype=bf16), u32)


def _dot(a, b):
    return jnp.dot(a, b, preferred_element_type=f32)


def _dot_nt(a, b):
    return lax.dot_general(a, b, (((1,), (1,)), ((), ())), preferred_element_type=f32)


def _dot_mixed(a, b):
    return lax.dot_general(a, b, (((1,), (0,)), ((), ())), preferred_element_type=f32)


def _iota(shape, dim):
    return lax.broadcasted_iota(jnp.int32, shape, dim)


def _phi(t):
    return jnp.where(t > 0, t + 1.0, jnp.exp(t))


def _round_bf16(x):
    return x.astype(bf16).astype(f32)


def _sigmoid(x):
    return 1.0 / (1.0 + jnp.exp(-x))


def _w_tile(w_ref, i, j, tail=None):
    r = min(T, D - T * i)
    c = min(T, D - T * j)
    t = w_ref[T * i:T * i + r, T * j:T * j + c]
    if c < T:
        t = jnp.concatenate([t, jnp.zeros((r, T - c), bf16)], axis=1)
    if r < T:
        parts = [t]
        if tail is not None:
            parts.append(tail)
        n = T - sum(p.shape[0] for p in parts)
        parts.append(jnp.zeros((n, T), bf16))
        t = jnp.concatenate(parts, axis=0)
    return t


def _store_wt(dst, row0, w_ref, i, j, tail=None):
    c = min(T, D - T * j)
    t = _pack(_w_tile(w_ref, i, j, tail).T)
    r0 = (row0 + T * j) // 2
    dst[0, r0:r0 + c // 2, T * i:T * (i + 1)] = t[:c // 2]


def kernel(x_hbm, wq_hbm, wk_hbm, wv_hbm, wo_hbm, beta_hbm, wr_hbm, wg_hbm, wu_hbm, wd_hbm,
           out_hbm,
           x_v, wq_v, wk_v, wv_v, wo_v, wg_v, wu_v, wd_v, out_v,
           wt, wot, xn_s, q_s, k_s, v_s, pq_s, pk_s, r_s, g_s, o_s, ob_s, m_s, om_s, mask_s, s_s,
           h_s, acc_s, bias_s, beta_ref, wr_ref, sems, osems):
    cp_x = [pltpu.make_async_copy(x_hbm.at[:, pl.ds(s * L, L)], x_v.at[s], sems.at[s])
            for s in range(NSEG)]
    cp_o = [pltpu.make_async_copy(out_v.at[s], out_hbm.at[:, pl.ds(s * L, L)], osems.at[s])
            for s in range(NSEG - 1)]
    cp_tail = [pltpu.make_async_copy(out_v.at[NSEG - 1, pl.ds(r0, r1 - r0)],
                                     out_hbm.at[pl.ds(r0, r1 - r0), pl.ds(S - L, L)],
                                     osems.at[NSEG - 1 + c])
               for c, (r0, r1) in enumerate(TAIL)]
    cp_wk = pltpu.make_async_copy(wk_hbm, wk_v, sems.at[4])
    cp_wq = pltpu.make_async_copy(wq_hbm, wq_v, sems.at[5])
    cp_wv = pltpu.make_async_copy(wv_hbm, wv_v, sems.at[6])
    cp_wo = pltpu.make_async_copy(wo_hbm, wo_v, sems.at[7])
    cp_wg = pltpu.make_async_copy(wg_hbm, wg_v, sems.at[8])
    cp_wu = pltpu.make_async_copy(wu_hbm, wu_v, sems.at[9])
    cp_wd = pltpu.make_async_copy(wd_hbm, wd_v, sems.at[10])
    cp_beta = pltpu.make_async_copy(beta_hbm, beta_ref, sems.at[11])
    cp_wr = pltpu.make_async_copy(wr_hbm, wr_ref, sems.at[12])
    for cp in (cp_x[0], cp_beta, cp_wr, cp_wv, cp_wq, cp_x[1], cp_wk, cp_x[2], cp_x[3],
               cp_wo, cp_wg, cp_wu, cp_wd):
        cp.start()

    colh = _iota((T, T), 1)
    rowh = _iota((T, T), 0)
    for t in range(NWIN):
        same = None
        zsel = None
        for n, h in enumerate(WIN_HEADS[t]):
            cin = (colh >= DH * h - WIN * t) & (colh < DH * (h + 1) - WIN * t)
            blk = cin & (rowh >= DH * h - WIN * t) & (rowh < DH * (h + 1) - WIN * t)
            same = blk if same is None else same | blk
            zc = cin[:8] & (rowh[:8] == n)
            zsel = zc if zsel is None else zsel | zc
        mask_s[t, 0:T] = jnp.where(same, 1.0, 0.0)
        mask_s[t, T:T + 8] = jnp.where(zsel, 1.0, 0.0)
    key = _iota((QB, T), 0)
    qry = _iota((QB, T), 1)
    qpos = [(qry - QB * c) % T for c in range(HG)]
    slot = qry // QB
    tiles = [qpos,
             [jnp.where(slot == c, qpos[3], qpos[c]) for c in range(3)] + [qry % QB + QB],
             [jnp.where(slot >= 2, qpos[0], qpos[2]),
              jnp.where((slot == 1) | (slot == 2), qpos[3], qpos[1])]]
    for b, row in enumerate(tiles):
        for c, qp_ in enumerate(row):
            bias_s[QB * b:QB * (b + 1), T * c:T * (c + 1)] = jnp.where(
                qp_ < key + QB * b, MASKVAL, 0.0)
    for j in range(S // T):
        xn_s[j, D // 2:DP // 2, :] = jnp.zeros(((DP - D) // 2, T), u32)

    def transpose_w(row0, w):
        for j in range(5):
            for i in range(5):
                _store_wt(wt, row0, w, i, j)

    def layernorm(s, j):
        xe, xo = _halves(_pack(x_v[s, :, T * j:T * (j + 1)]))
        mean = jnp.sum(xe + xo, axis=0, keepdims=True) / D
        ce, co = xe - mean, xo - mean
        var = jnp.sum(ce * ce + co * co, axis=0, keepdims=True) / D
        inv = 1.0 / _round_bf16(jnp.sqrt(_round_bf16(_round_bf16(var) + LN_EPS)))
        mean = _round_bf16(mean)
        de, do = _halves(_join(xe - mean, xo - mean))
        xn_s[NQT * s + j, 0:D // 2, :] = _join(de * inv, do * inv)

    def xn_seg(s):
        return _unpack(jnp.concatenate([xn_s[NQT * s + j] for j in range(NQT)], axis=1))

    def proj_q(s):
        q = _dot(_unpack(wt[z, RQ // 2:RK // 2, :]), xn_seg(s))
        for j in range(NQT):
            r_s[NQT * s + j:NQT * s + j + 1, :] = q[D:D + 1, T * j:T * (j + 1)]
        if s > 0:
            pq_s[s - 1] = _pack(_phi(q[:D]).astype(bf16))
        qp = _pack((q[:D] * QSCALE).astype(bf16))
        for h in range(H):
            a = (DH * h) // 16
            lo = (DH * h - 16 * a) // 2
            prow = _iota((16, L), 0)
            qh = jnp.where((prow >= lo) & (prow <= lo + 8), qp[8 * a:8 * a + 16], jnp.zeros((), u32))
            for j in range(NQT):
                qt = qh[:, T * j:T * (j + 1)]
                q_s[s, h, j] = pltpu.roll(qt, QB * (h % HG), 1) if h % HG else qt

    def proj_k(s):
        k = _dot(_unpack(wt[z, RK // 2:RV // 2, :]), xn_seg(s))
        if s < NSEG - 1:
            pk_s[s] = _pack(_phi(k).astype(bf16))
        for j in range(NQT):
            kb = k[:, T * j:T * (j + 1)].astype(bf16)
            for g in range(NG):
                kw = jnp.concatenate([kb[GWIN[g]:GWIN[g] + GK], jnp.zeros((T - GK, T), bf16)], axis=0)
                k_s[s, g, 64 * j:64 * (j + 1), :] = _pack(kw.T)

    def proj_v(s, r0=0, r1_=D):
        v_s[s, r0:r1_, :] = _round_bf16(
            _dot(_unpack(wt[z, (RV + r0) // 2:(RV + r1_) // 2, :]), xn_seg(s)))

    cp_x[0].wait()
    cp_beta.wait()
    cp_wr.wait()
    g = _round_bf16(_sigmoid(beta_ref[...].astype(f32)))
    z = jnp.where(jnp.max(g) > 2.0, 1, 0)
    g = jnp.concatenate([g, jnp.zeros((1, T - H), f32)], axis=1)
    g_s[...] = jnp.broadcast_to(g, (T, T)).T
    wr = wr_ref[...].reshape(1, D)
    wr = jnp.concatenate([wr, jnp.zeros((1, DP - D), bf16)], axis=1)
    wt[0, D // 2:RK // 2, :] = _pack(jnp.broadcast_to(wr, (16, DP)))
    for j in range(NQT):
        layernorm(0, j)
    cp_wv.wait()
    transpose_w(RV, wv_v)
    proj_v(0, 0, 416)
    cp_wq.wait()
    transpose_w(RQ, wq_v)
    proj_v(0, 416, 496)
    proj_q(0)
    cp_x[1].wait()
    cp_wk.wait()
    transpose_w(RK, wk_v)
    for j in range(NQT):
        layernorm(1, j)
    proj_v(0, 496, D)
    proj_k(0)
    proj_v(1)
    cp_x[2].wait()
    cp_x[3].wait()
    for j in range(NQT):
        layernorm(2, j)
    proj_q(1)
    for j in range(NQT):
        layernorm(3, j)
    proj_q(2)
    proj_q(3)

    r = _round_bf16(r_s[...])
    pos = _iota((S // T, T), 0) * T + _iota((S // T, T), 1)
    r1 = jnp.max(r)
    i1 = jnp.minimum(jnp.min(jnp.where(r == r1, pos, S)), S - 1)
    rest = pos != i1
    r2 = jnp.max(jnp.where(rest, r, -jnp.inf))
    i2 = jnp.minimum(jnp.min(jnp.where(rest & (r == r2), pos, S)), S - 1)

    for s in range(1, NSEG):
        proj_k(s)
        if s > 1:
            proj_v(s)

    lane = _iota((DP // 2, T), 1)
    row16 = _iota((16, T), 0)
    xsel = jnp.zeros((16, DP), f32)
    for c, idx in enumerate((i1, i2)):
        col = jnp.where(lane == idx % T, xn_s[idx // T], jnp.zeros((), u32))
        xsel = xsel + _dot_nt(jnp.where(row16 == c, 1.0, 0.0).astype(bf16), _unpack(col))

    moe = {}

    def ffn_in(w, name, cg, i):
        k = min(T, D - T * i)
        r_ = _dot(xsel[:, T * i:T * i + k].astype(bf16), w[T * i:T * i + k, L * cg:L * (cg + 1)])[:8]
        moe[name] = r_ if i == 0 else moe[name] + r_
        if name == "up" and i == 4:
            gate = moe["gate"]
            hid = gate * _sigmoid(gate) * moe["up"]
            h_s[:, L * cg:L * (cg + 1)] = _pack(
                jnp.concatenate([hid, jnp.zeros((8, L), f32)], axis=0).astype(bf16))

    def ffn_out(cg, i):
        if i < 4:
            c0 = L * cg + T * i
            r_ = _dot_nt(_unpack(h_s[:, c0:c0 + T]), wd_v[0:4 * T, c0:c0 + T])[:8]
            moe["y0"] = r_ if "y0" not in moe else moe["y0"] + r_
        else:
            r_ = _dot_nt(_unpack(h_s[:, L * cg:L * (cg + 1)]), wd_v[4 * T:D, L * cg:L * (cg + 1)])[:8]
            moe["y1"] = r_ if "y1" not in moe else moe["y1"] + r_

    def ffn_finish():
        y = jnp.concatenate([moe["y0"], moe["y1"], jnp.zeros((8, DP - D), f32)], axis=1)
        y = y * _sigmoid(jnp.where(_iota((8, DP), 0) == 0, r1, r2))
        y = jnp.concatenate([y, jnp.zeros((8, DP), f32)], axis=0)
        for j in range(5):
            _store_wt(wot, 0, wo_v, 4, j, tail=y[:, T * j:T * (j + 1)].astype(bf16))

    rounds = []
    for cg in range(F // L):
        rounds += [(ffn_in, wg_v, "gate", cg, i) for i in range(5)]
        rounds += [(ffn_in, wu_v, "up", cg, i) for i in range(5)]
        if cg > 0:
            rounds += [(ffn_out, cg - 1, i) for i in range(5)]
    rounds += [None] * 3
    rounds += [(ffn_out, F // L - 1, i) for i in range(5)]

    prow = _iota((8, T), 0)
    steps = [(s, g, j, i) for s in range(NSEG) for g in range(NG) for j in range(NQT)
             for i in range(j + 1)]
    ns = len(steps)
    mx, tok, due = {}, {}, {}
    never = prow > i1 + 8
    lane8 = _iota((8, T), 1)
    hi = lane8 >= T // 2
    sl = [lane8 // QB == c for c in range(HG)]
    mid = sl[1] | sl[2]
    def q_masked(s, g, j, c):
        h = HG * g + c
        pos0 = (DH * h) // 16 - GWIN[g] // 16
        zero = jnp.zeros((8, T), u32)
        return ([zero] * pos0 + [q_s[s, h, j, 0:8], q_s[s, h, j, 8:16]]
                + [zero] * (GK // 16 - 2 - pos0))

    def k_rows(s, g, r0, r1_):
        return _unpack(k_s[s + z, g, r0 // 2:r1_ // 2, :])[:, :GK]

    def sel(mask, a, b):
        n_ = len(a) if isinstance(a, list) else len(b)
        out = []
        for r_ in range(n_):
            x = a[r_] if isinstance(a, list) else a
            y = b[r_] if isinstance(b, list) else b
            out.append(x if x is y else jnp.where(mask, x, y))
        return out

    def stash(n, st, row0, col0, bias_row0=None):
        m = None
        w = st.shape[1]
        for r_ in range(0, st.shape[0], 8):
            x = st[r_:r_ + 8]
            if bias_row0 is not None:
                x = x + bias_s[bias_row0 + r_:bias_row0 + r_ + 8, col0:col0 + w]
            s_s[n % NB, row0 + r_:row0 + r_ + 8, col0:col0 + w] = x
            m = x if m is None else jnp.maximum(m, x)
        return m

    def weights(tiles_):
        return _unpack(jnp.concatenate([jnp.concatenate(q, axis=0) for q in tiles_], axis=1))

    def qk(n):
        s, g, j, i = steps[n]
        qm = [q_masked(s, g, j, c) for c in range(HG)]
        if i < j:
            ahead = QB if MERGE and i == j - 1 else 0
            st = _dot(k_rows(s, g, T * i, T * (i + 1) + ahead), weights(qm))
            tok[n] = st[8 * TOKROW:8 * TOKROW + 8]
            m = stash(n, st[:T], 0, 0)
            if ahead:
                m = jnp.maximum(m, stash(n + 1, st[T:], 0, 0, 0))
            mx[s, g, j] = m if i == 0 else jnp.maximum(mx[s, g, j], m)
            return
        if j == 0 or not MERGE:
            m = stash(n, _dot(k_rows(s, g, T * i, T * i + QB), weights(qm)), 0, 0, 0)
            if j > 0:
                m = jnp.maximum(mx[s, g, j], m)
        else:
            m = mx[s, g, j]
        x1 = _dot(k_rows(s, g, T * i + QB, T * i + 2 * QB),
                  weights([sel(sl[c], qm[3], qm[c]) for c in range(3)]))
        x3 = _dot(k_rows(s, g, T * i + 3 * QB, T * (i + 1)),
                  weights([sel(hi, sel(mid, qm[3], qm[0]), sel(mid, qm[2], qm[1]))]))
        tok[n] = jnp.concatenate([x1[QB - 8:], x3[QB - 8:]], axis=1)
        m1 = stash(n, x1, QB, 0, QB)
        m1 = [m1[:, T * c:T * (c + 1)] for c in range(3)]
        m3 = stash(n, x3, QB, 3 * T, QB)
        m2 = []
        for c, w in enumerate((sel(hi, qm[0], qm[2]), sel(mid, qm[3], qm[1]))):
            parts = [stash(n, _dot(k_rows(s, g, T * i + r0, T * i + r0 + QB // 2), weights([w])),
                           r0, T * c, r0) for r0 in (2 * QB, 2 * QB + QB // 2)]
            m2.append(jnp.maximum(*parts))
        ms = []
        for c in range(HG):
            x = m[:, T * c:T * (c + 1)]
            if c < 3:
                x = jnp.where(sl[c], x, jnp.maximum(x, m1[c]))
            else:
                for b in range(3):
                    x = jnp.where(sl[b], jnp.maximum(x, m1[b]), x)
            y = jnp.maximum(x, m2[c % 2])
            x = jnp.where((hi, mid)[c % 2], *((y, x) if c in (0, 3) else (x, y)))
            ms.append(jnp.where(sl[(c + 3) % HG], jnp.maximum(x, m3), x))
        mx[s, g, j] = jnp.max(jnp.concatenate(ms, axis=1), axis=0, keepdims=True)

    def pv(n):
        s, g, j, i = steps[n]
        ms = []
        for c in range(HG):
            m = jnp.broadcast_to(mx[s, g, j][:, T * c:T * (c + 1)], (8, T))
            t_ = tok[n + LAG - (TOKBACK if n + LAG <= ns else ETOK)][:, T * c:T * (c + 1)]
            for x in due.pop((n, c), ()):
                t_ = jnp.maximum(t_, x)
            ms.append(jnp.where(never, t_, m))

        def probs(r0, r1_, c, m):
            return [jnp.exp2(s_s[n % NB, r_:r_ + 8, T * c:T * (c + 1)] - m) for r_ in range(r0, r1_, 8)]

        if i == j:
            e1 = [probs(QB, 2 * QB, c, jnp.where(sl[c], ms[3], ms[c])) for c in range(3)]
            e3 = probs(QB, 2 * QB, 3, jnp.where(hi, jnp.where(mid, ms[3], ms[0]),
                                                jnp.where(mid, ms[2], ms[1])))
            e2 = [probs(2 * QB, 3 * QB, 0, jnp.where(hi, ms[0], ms[2])),
                  probs(2 * QB, 3 * QB, 1, jnp.where(mid, ms[3], ms[1]))]
        for c in range(HG):
            if i == j:
                p = probs(0, QB, c, ms[c])
                if c < 3:
                    p += sel(sl[c], 0.0, e1[c])
                else:
                    p += sel(sl[0], e1[0], sel(sl[1], e1[1], sel(sl[2], e1[2], 0.0)))
                p += sel((hi, mid)[c % 2], *((e2[c % 2], 0.0) if c in (0, 3) else (0.0, e2[c % 2])))
                p += sel(sl[(c + 3) % HG], e3, 0.0)
            else:
                p = probs(0, T, c, ms[c])
            p = jnp.concatenate(p, axis=0)
            h = HG * g + c
            a = DH * h // 8 * 8
            o = DH * h - a
            one = 23 if o == 0 else 0
            vt = [v_s[s, a + 8 * r_:a + 8 * r_ + 8, T * i:T * (i + 1)] for r_ in range(3)]
            vt[one // 8] = jnp.where(prow == one % 8, 1.0, vt[one // 8])
            r_ = _dot_mixed(jnp.concatenate(vt, axis=0), p.astype(bf16))
            if i > 0:
                r_ = acc_s[c] + r_
            if i < j:
                acc_s[c] = r_
            else:
                l = r_[one:one + 1]
                inv = pltpu.reciprocal(l, approx=True)
                inv = inv * (2.0 - l * inv)
                sc = (1.0 - g_s[h:h + 1, :]) * (inv * (2.0 - l * inv))
                val = r_ * sc
                if c:
                    val = pltpu.roll(val, T - QB * c, 1)
                for r0 in range(0, 24, 8):
                    due.setdefault((n + DUE, c), []).append(val[r0:r0 + 8])
                o_s[s % 2, DH * h:DH * (h + 1), T * j:T * (j + 1)] = val[o:o + DH]

    def win_rows(t):
        heads = WIN_HEADS[t]
        return DH * heads[0] // 8 * 8, -(-DH * (heads[-1] + 1) // 8) * 8

    def mem_read(s, t):
        heads = WIN_HEADS[t]
        r0 = WIN * t
        ra0, re0 = win_rows(t)
        lhs = jnp.concatenate(
            [jnp.where(mask_s[t, a:b] > 0, _round_bf16(m_s[t, a:b]), 0.0)
             for a, b in ((ra0 - r0, re0 - r0), (T, T + 8))], axis=0)
        rd = _dot_mixed(lhs, _unpack(pq_s[s - 1, r0 // 2:r0 // 2 + 64, :]))
        h0 = heads[0]
        coef = jnp.concatenate([g_s[h0:h0 + 8, :]] * NQT, axis=1) / (rd[re0 - ra0:] + 1e-6)
        lo_row = DH * heads[0]
        hi_row = DH * (heads[-1] + 1)
        for rb in range(ra0, re0, 8):
            ha = max(rb // DH, h0)
            hb = min((rb + 7) // DH, heads[-1])
            cf = jnp.broadcast_to(coef[ha - h0:ha - h0 + 1], (8, L))
            if hb != ha:
                cf = jnp.where(_iota((8, L), 0) < DH * hb - rb, cf,
                               jnp.broadcast_to(coef[hb - h0:hb - h0 + 1], (8, L)))
            val = rd[rb - ra0:rb - ra0 + 8] * cf
            ra, re = max(rb, lo_row), min(rb + 8, hi_row)
            om_s[s % 2, ra:re, :] = val[ra - rb:re - rb]

    def mem_update(s, t):
        r0 = WIN * t
        ra0, re0 = win_rows(t)
        vl = jnp.concatenate([v_s[s, ra0:re0, :], jnp.ones((8, L), f32)], axis=0)
        upd = lax.dot_general(vl, _unpack(pk_s[s, r0 // 2:r0 // 2 + 64, :]),
                              (((1,), (1,)), ((), ())), preferred_element_type=f32)
        for a, b, u in ((ra0 - r0, re0 - r0, upd[:re0 - ra0]), (T, T + 8, upd[re0 - ra0:])):
            m_s[t, a:b] = u if s == 0 else m_s[t, a:b] + u

    def pack_o(s, r0, r1_):
        o = o_s[s % 2, r0:r1_, :]
        if s > 0:
            o = o + om_s[s % 2, r0:r1_, :]
        ob_s[s, r0 // 2:r1_ // 2, :] = _pack(o.astype(bf16))

    def out_proj(s, r0, r1_, n=None):
        ob = ob_s[s]
        if n is not None:
            head = jnp.where(jnp.concatenate([never] * HG, axis=1),
                             pltpu.bitcast(tok[n - PINBACK], u32), ob[:8])
            ob = jnp.concatenate([head, ob[8:]], axis=0)
        res = _dot(_unpack(wot[z, r0 // 2:r1_ // 2, :]), _unpack(ob))
        if n is not None:
            tok[n] = res[:8]
        xn = _unpack(jnp.concatenate(
            [xn_s[NQT * s + j, r0 // 2:r1_ // 2, :] for j in range(NQT)], axis=1))
        out_v[s, r0:r1_, :] = (res + x_v[s, r0:r1_, :].astype(f32) + xn.astype(f32)).astype(bf16)

    for s in range(NSEG):
        tpos = _iota((16, L), 1) + s * L
        pick = jnp.where(_iota((16, L), 0) == 0, i1, jnp.where(_iota((16, L), 0) == 1, i2, -1))
        ob_s[s, D // 2:D // 2 + 8, :] = _pack(jnp.where(tpos == pick, 1.0, 0.0).astype(bf16))
        ob_s[s, D // 2 + 8:DP // 2, :] = jnp.zeros(((DP - D) // 2 - 8, L), u32)

    extra = {}

    def at(n, fn, *args):
        extra.setdefault(n, []).append((fn,) + args)

    per = ns // NSEG
    full = [n for n, (_, _, j, i) in enumerate(steps) if i < j]
    busy = set()

    def at_full(n, fn, *args):
        n = next(m for m in full if m >= n and m not in busy)
        busy.add(n)
        at(n, fn, *args)
        return n

    for t in range(NWIN):
        at_full(0, mem_update, 0, t)
        for s in range(1, NSEG):
            at_full(per * s - 40 + 6 * t, mem_read, s, t)
            if s < NSEG - 1:
                at_full(per * s + 4 + 6 * t, mem_update, s, t)

    busy.clear()

    def late_weights():
        for cp in (cp_wo, cp_wg, cp_wu, cp_wd):
            cp.wait()

    at(MOE0, late_weights)
    n = MOE0
    for rd_ in rounds:
        n = at_full(n, *rd_) if rd_ is not None else n + 2
    at(n + 2, ffn_finish)
    for c in range(20):
        at(MOE0 + 2 * c + 1, _store_wt, wot, 0, wo_v, c % 4, c // 4)
    for s in range(NSEG):
        for c in range(D // 48):
            n = per * s + 10 * ((48 * (c + 1) - 1) // (HG * DH) + 1) + LAG + c % 2 * 3 + 1
            at(min(n, ns + LAG), pack_o, s, 48 * c, 48 * (c + 1))
    for c in range(LAG):
        at(ns + c, out_proj, 0, FILL * c, FILL * (c + 1), ns + c)

    for n in range(ns + LAG):
        if n < ns:
            qk(n)
        for task in extra.get(n, ()):
            if not (AFTER and task[0] is ffn_in):
                task[0](*task[1:])
        if n >= LAG:
            pv(n - LAG)
        for task in extra.get(n, ()):
            if AFTER and task[0] is ffn_in:
                task[0](*task[1:])
    for task in extra[ns + LAG]:
        task[0](*task[1:])
    for s in range(NSEG - 1):
        out_proj(s, FILL * LAG if s == 0 else 0, D, ns + LAG + s if s == 0 else None)
        cp_o[s].start()
    for (r0, r1_), cp in zip(TAIL, cp_tail):
        out_proj(NSEG - 1, r0, r1_)
        cp.start()
    for cp in cp_o + cp_tail:
        cp.wait()


@jax.jit
def pallas_parallel_sum__memory_aug_infini_attn__moe_arch_mod__prompt_kernel(
    A_x, A_wq, A_wk, A_wv, A_wo, A_beta, B_x, B_w_r, B_w_gate, B_w_up, B_w_down,
):
    del B_x
    any_spec = pl.BlockSpec(memory_space=pl.ANY)
    out_t = pl.pallas_call(
        kernel,
        out_shape=jax.ShapeDtypeStruct((D, S), bf16),
        in_specs=[any_spec] * 10,
        out_specs=any_spec,
        scratch_shapes=[
            pltpu.VMEM((NSEG, D, L), bf16),
            pltpu.VMEM((D, D), bf16),
            pltpu.VMEM((D, D), bf16),
            pltpu.VMEM((D, D), bf16),
            pltpu.VMEM((D, D), bf16),
            pltpu.VMEM((D, F), bf16),
            pltpu.VMEM((D, F), bf16),
            pltpu.VMEM((D, F), bf16),
            pltpu.VMEM((NSEG, D, L), bf16),
            pltpu.VMEM((1, NROW // 2, DP), u32),
            pltpu.VMEM((1, D // 2, DP), u32),
            pltpu.VMEM((S // T, DP // 2, T), u32),
            pltpu.VMEM((NSEG, H, NQT, 16, T), u32),
            pltpu.VMEM((NSEG, NG, L // 2, T), u32),
            pltpu.VMEM((NSEG, D, L), f32),
            pltpu.VMEM((NSEG - 1, D // 2, L), u32),
            pltpu.VMEM((NSEG - 1, D // 2, L), u32),
            pltpu.VMEM((S // T, T), f32),
            pltpu.VMEM((T, T), f32),
            pltpu.VMEM((2, D, L), f32),
            pltpu.VMEM((NSEG, DP // 2, L), u32),
            pltpu.VMEM((NWIN, T + 8, T), f32),
            pltpu.VMEM((2, D, L), f32),
            pltpu.VMEM((NWIN, T + 8, T), f32),
            pltpu.VMEM((NB, T, HG * T), f32),
            pltpu.VMEM((8, F), u32),
            pltpu.VMEM((HG, 24, T), f32),
            pltpu.VMEM((3 * QB, HG * T), f32),
            pltpu.VMEM((1, H), bf16),
            pltpu.VMEM((D,), bf16),
            pltpu.SemaphoreType.DMA((13,)),
            pltpu.SemaphoreType.DMA((NSEG - 1 + len(TAIL),)),
        ],
        compiler_params=pltpu.CompilerParams(vmem_limit_bytes=100 * 1024 * 1024),
        name="infini_moe",
    )(A_x.reshape(S, D).T, A_wq, A_wk, A_wv, A_wo, A_beta.reshape(1, H), B_w_r,
      B_w_gate, B_w_up, B_w_down.T)
    return out_t.T.reshape(1, S, D)
```

```python
import math
import os

import jax
import jax.numpy as jnp
import numpy as np
from jax import lax
import jax.experimental.pallas as pl
import jax.experimental.pallas.tpu as pltpu

S = 2048
D = 576
H = 32
DH = D // H
NSEG = 4
L = S // NSEG
F = 4608
T = 128
DP = 640
NQT = L // T
WIN = 112
NWIN = 5
HEAD_WIN = [0] * 7 + [1] * 6 + [2] * 6 + [3] * 6 + [4] * 7
WIN_HEADS = [[h for h in range(H) if HEAD_WIN[h] == t] for t in range(NWIN)]
HG = 4
NG = H // HG
AFTER = int(os.environ.get('AFTER', 1))
PINBACK = int(os.environ.get('PINBACK', 2))
ETOK = int(os.environ.get('ETOK', 2))
DUE = int(os.environ.get('DUE', 20))
QB = T // HG
MERGE = int(os.environ.get('MERGE', 1))
GK = 80
GWIN = [HG * DH * g // 16 * 16 for g in range(NG)]
TOKROW = int(os.environ.get('TOKROW', 10))
TOKBACK = int(os.environ.get('TOKBACK', 2))
MOE0 = int(os.environ.get('MOE0', 61))
LAG = int(os.environ.get('LAG', 11))
NB = int(os.environ.get('NB', 13))
RQ, RK, RV = 0, D, 2 * D
NROW = 3 * D
FILL = int(os.environ.get('FILL', 48))
VSPLIT = int(os.environ.get('VSPLIT', 448))
TAIL = ((0, 288), (288, 480), (480, D))
LOG2E = math.log2(math.e)
QSCALE = DH ** -0.5 * LOG2E
MASKVAL = -999292928.0 * LOG2E
LN_EPS = float(np.asarray(1e-5, dtype=jnp.bfloat16).astype(np.float32))

bf16 = jnp.bfloat16
f32 = jnp.float32
u32 = jnp.uint32


def _pack(x):
    return pltpu.bitcast(x, u32)


def _unpack(x):
    return pltpu.bitcast(x, bf16)


def _halves(x):
    return [pltpu.unpack_elementwise(x, index=i, packed_dtype=bf16, unpacked_dtype=f32)
            for i in range(2)]


def _join(even, odd):
    return pltpu.bitcast(pltpu.pack_elementwise([even, odd], packed_dtype=bf16), u32)


def _dot(a, b):
    return lax.dot_general(a, b, (((1,), (0,)), ((), ())), preferred_element_type=f32)


def _dot_nt(a, b):
    return lax.dot_general(a, b, (((1,), (1,)), ((), ())), preferred_element_type=f32)


def _dot_mixed(a, b):
    return lax.dot_general(a, b, (((1,), (0,)), ((), ())), preferred_element_type=f32)


def _iota(shape, dim):
    return lax.broadcasted_iota(jnp.int32, shape, dim)


def _phi(t):
    return jnp.where(t > 0, t + 1.0, jnp.exp(t))


def _round_bf16(x):
    return x.astype(bf16).astype(f32)


def _sigmoid(x):
    return 1.0 / (1.0 + jnp.exp(-x))


def _w_tile(w_ref, i, j, tail=None):
    r = min(T, D - T * i)
    c = min(T, D - T * j)
    t = w_ref[T * i:T * i + r, T * j:T * j + c]
    if c < T:
        t = jnp.concatenate([t, jnp.zeros((r, T - c), bf16)], axis=1)
    if r < T:
        parts = [t]
        if tail is not None:
            parts.append(tail)
        n = T - sum(p.shape[0] for p in parts)
        parts.append(jnp.zeros((n, T), bf16))
        t = jnp.concatenate(parts, axis=0)
    return t


def _store_wt(dst, row0, w_ref, i, j, tail=None):
    c = min(T, D - T * j)
    t = _pack(_w_tile(w_ref, i, j, tail).T)
    r0 = (row0 + T * j) // 2
    dst[0, r0:r0 + c // 2, T * i:T * (i + 1)] = t[:c // 2]


def kernel(x_hbm, wq_hbm, wk_hbm, wv_hbm, wo_hbm, beta_hbm, wr_hbm, wg_hbm, wu_hbm, wd_hbm,
           out_hbm,
           x_v, wq_v, wk_v, wv_v, wo_v, wg_v, wu_v, wd_v, out_v,
           wt, wot, xn_s, q_s, k_s, v_s, pq_s, pk_s, r_s, g_s, o_s, ob_s, m_s, om_s, mask_s, s_s,
           h_s, wr_s, acc_s, bias_s, beta_ref, wr_ref, sems):
    cp_x = [pltpu.make_async_copy(x_hbm.at[:, pl.ds(s * L, L)], x_v.at[s], sems.at[(0, 3, 4, 4)[s]])
            for s in range(NSEG)]
    cp_o = [pltpu.make_async_copy(out_v.at[s], out_hbm.at[:, pl.ds(s * L, L)], sems.at[6])
            for s in range(NSEG - 1)]
    cp_tail = [pltpu.make_async_copy(out_v.at[NSEG - 1, pl.ds(r0, r1 - r0)],
                                     out_hbm.at[pl.ds(r0, r1 - r0), pl.ds(S - L, L)],
                                     sems.at[6])
               for c, (r0, r1) in enumerate(TAIL)]
    cp_wk = pltpu.make_async_copy(wk_hbm, wk_v, sems.at[3])
    cp_wq = pltpu.make_async_copy(wq_hbm, wq_v, sems.at[2])
    cp_wv = pltpu.make_async_copy(wv_hbm, wv_v, sems.at[1])
    cp_wo = pltpu.make_async_copy(wo_hbm, wo_v, sems.at[5])
    cp_wg = pltpu.make_async_copy(wg_hbm, wg_v, sems.at[5])
    cp_wu = pltpu.make_async_copy(wu_hbm, wu_v, sems.at[5])
    cp_wd = pltpu.make_async_copy(wd_hbm, wd_v, sems.at[5])
    cp_beta = pltpu.make_async_copy(beta_hbm, beta_ref, sems.at[0])
    cp_wr = pltpu.make_async_copy(wr_hbm, wr_ref, sems.at[0])
    for cp in (cp_x[0], cp_beta, cp_wr, cp_wv, cp_wq, cp_x[1], cp_wk, cp_x[2], cp_x[3],
               cp_wo, cp_wg, cp_wu, cp_wd):
        cp.start()

    colh = _iota((T, T), 1)
    rowh = _iota((T, T), 0)
    for t in range(NWIN):
        same = None
        zsel = None
        for n, h in enumerate(WIN_HEADS[t]):
            cin = (colh >= DH * h - WIN * t) & (colh < DH * (h + 1) - WIN * t)
            blk = cin & (rowh >= DH * h - WIN * t) & (rowh < DH * (h + 1) - WIN * t)
            same = blk if same is None else same | blk
            zc = cin[:8] & (rowh[:8] == n)
            zsel = zc if zsel is None else zsel | zc
        mask_s[t, 0:T] = jnp.where(same, 1.0, 0.0)
        mask_s[t, T:T + 8] = jnp.where(zsel, 1.0, 0.0)
    key = _iota((QB, T), 0)
    qry = _iota((QB, T), 1)
    qpos = [(qry - QB * c) % T for c in range(HG)]
    slot = qry // QB
    tiles = [qpos,
             [jnp.where(slot == c, qpos[3], qpos[c]) for c in range(3)] + [qry % QB + QB],
             [jnp.where(slot >= 2, qpos[0], qpos[2]),
              jnp.where((slot == 1) | (slot == 2), qpos[3], qpos[1])]]
    for b, row in enumerate(tiles):
        for c, qp_ in enumerate(row):
            bias_s[QB * b:QB * (b + 1), T * c:T * (c + 1)] = jnp.where(
                qp_ < key + QB * b, MASKVAL, 0.0)
    for j in range(S // T):
        xn_s[j, D // 2:DP // 2, :] = jnp.zeros(((DP - D) // 2, T), u32)

    def transpose_w(row0, w):
        for j in range(5):
            for i in range(5):
                _store_wt(wt, row0, w, i, j)

    def layernorm(s, j):
        xe, xo = _halves(_pack(x_v[s, :, T * j:T * (j + 1)]))
        mean = jnp.sum(xe + xo, axis=0, keepdims=True) / D
        ce, co = xe - mean, xo - mean
        var = jnp.sum(ce * ce + co * co, axis=0, keepdims=True) / D
        inv = 1.0 / _round_bf16(jnp.sqrt(_round_bf16(_round_bf16(var) + LN_EPS)))
        mean = _round_bf16(mean)
        de, do = _halves(_join(xe - mean, xo - mean))
        xn_s[NQT * s + j, 0:D // 2, :] = _join(de * inv, do * inv)

    def router_weights():
        wr = jnp.concatenate([wr_ref[...].reshape(1, D), jnp.zeros((1, DP - D), bf16)], axis=1)
        even, odd = _halves(_pack(jnp.broadcast_to(wr, (T, DP)).T)[:D // 2])
        wr_s[0], wr_s[1] = even, odd

    def router(s):
        for j in range(NQT * s, NQT * (s + 1)):
            even, odd = _halves(xn_s[j, 0:D // 2, :])
            r_s[j:j + 1, :] = jnp.sum(even * wr_s[0] + odd * wr_s[1], axis=0, keepdims=True)

    def xn_seg(s):
        return _unpack(jnp.concatenate([xn_s[NQT * s + j] for j in range(NQT)], axis=1))

    def proj_q(s):
        q = _dot(_unpack(wt[z, RQ // 2:RK // 2, :]), xn_seg(s))
        if s > 0:
            pq_s[s - 1] = _pack(_phi(q[:D]).astype(bf16))
        qp = _pack((q[:D] * QSCALE).astype(bf16))
        for h in range(H):
            a = (DH * h) // 16
            lo = (DH * h - 16 * a) // 2
            prow = _iota((16, L), 0)
            qh = jnp.where((prow >= lo) & (prow <= lo + 8), qp[8 * a:8 * a + 16], jnp.zeros((), u32))
            for j in range(NQT):
                qt = qh[:, T * j:T * (j + 1)]
                q_s[s, h, j] = pltpu.roll(qt, QB * (h % HG), 1) if h % HG else qt

    def proj_k(s):
        k = _dot(_unpack(wt[z, RK // 2:RV // 2, :]), xn_seg(s))
        if s < NSEG - 1:
            pk_s[s] = _pack(_phi(k).astype(bf16))
        for j in range(NQT):
            kb = k[:, T * j:T * (j + 1)].astype(bf16)
            for g in range(NG):
                kw = jnp.concatenate([kb[GWIN[g]:GWIN[g] + GK], jnp.zeros((T - GK, T), bf16)], axis=0)
                k_s[s, g, 64 * j:64 * (j + 1), :] = _pack(kw.T)

    def proj_v(s, r0=0, r1_=D):
        v_s[s, r0:r1_, :] = _round_bf16(
            _dot(_unpack(wt[z, (RV + r0) // 2:(RV + r1_) // 2, :]), xn_seg(s)))

    cp_x[0].wait()
    cp_beta.wait()
    cp_wr.wait()
    g = _round_bf16(_sigmoid(beta_ref[...].astype(f32)))
    z = jnp.where(jnp.max(g) > 2.0, 1, 0)
    g = jnp.concatenate([g, jnp.zeros((1, T - H), f32)], axis=1)
    g_s[...] = jnp.broadcast_to(g, (T, T)).T
    for j in range(NQT):
        layernorm(0, j)
    router_weights()
    cp_wv.wait()
    transpose_w(RV, wv_v)
    proj_v(0, 0, 384)
    cp_wq.wait()
    transpose_w(RQ, wq_v)
    router(0)
    proj_v(0, 384, 448)
    proj_q(0)
    proj_v(0, 448, 512)
    cp_x[1].wait()
    cp_wk.wait()
    transpose_w(RK, wk_v)
    for j in range(NQT):
        layernorm(1, j)
    proj_v(0, 512, D)
    proj_k(0)
    router(1)
    proj_v(1)
    cp_x[2].wait()
    cp_x[3].wait()
    for s in (2, 3):
        for j in range(NQT):
            layernorm(s, j)
        router(s)
        proj_q(s - 1)
    proj_q(3)

    r = _round_bf16(r_s[...])
    pos = _iota((S // T, T), 0) * T + _iota((S // T, T), 1)
    r1 = jnp.max(r)
    i1 = jnp.minimum(jnp.min(jnp.where(r == r1, pos, S)), S - 1)
    rest = pos != i1
    r2 = jnp.max(jnp.where(rest, r, -jnp.inf))
    i2 = jnp.minimum(jnp.min(jnp.where(rest & (r == r2), pos, S)), S - 1)

    for s in range(1, NSEG):
        proj_k(s)
        if s > 1:
            proj_v(s)

    lane = _iota((DP // 2, T), 1)
    xsel = jnp.zeros((8, DP), f32)
    for c, idx in enumerate((i1, i2)):
        col = jnp.where(lane == idx % T, xn_s[idx // T], jnp.zeros((), u32))
        xsel = xsel + _dot_nt(jnp.where(_iota((8, T), 0) == c, 1.0, 0.0), _unpack(col))

    moe = {}

    def ffn_in(w, name, cg, i):
        k = min(T, D - T * i)
        r_ = _dot(xsel[:, T * i:T * i + k], w[T * i:T * i + k, L * cg:L * (cg + 1)])
        moe[name] = r_ if i == 0 else moe[name] + r_
        if name == "up" and i == 4:
            gate = moe["gate"]
            hid = gate * _sigmoid(gate) * moe["up"]
            h_s[:, L * cg:L * (cg + 1)] = _round_bf16(hid)

    def ffn_out(cg, i):
        if i < 4:
            c0 = L * cg + T * i
            r_ = _dot_nt(h_s[:, c0:c0 + T], wd_v[0:4 * T, c0:c0 + T])
            moe["y0"] = r_ if "y0" not in moe else moe["y0"] + r_
        else:
            r_ = _dot_nt(h_s[:, L * cg:L * (cg + 1)], wd_v[4 * T:D, L * cg:L * (cg + 1)])
            moe["y1"] = r_ if "y1" not in moe else moe["y1"] + r_

    def ffn_finish():
        y = jnp.concatenate([moe["y0"], moe["y1"], jnp.zeros((8, DP - D), f32)], axis=1)
        y = y * _sigmoid(jnp.where(_iota((8, DP), 0) == 0, r1, r2))
        y = jnp.concatenate([y, jnp.zeros((8, DP), f32)], axis=0)
        for j in range(5):
            _store_wt(wot, 0, wo_v, 4, j, tail=y[:, T * j:T * (j + 1)].astype(bf16))

    rounds = []
    for cg in range(F // L):
        rounds += [(ffn_in, wg_v, "gate", cg, i) for i in range(5)]
        rounds += [(ffn_in, wu_v, "up", cg, i) for i in range(5)]
        if cg > 0:
            rounds += [(ffn_out, cg - 1, i) for i in range(5)]
    rounds += [None] * 3
    rounds += [(ffn_out, F // L - 1, i) for i in range(5)]

    prow = _iota((8, T), 0)
    steps = [(s, g, j, i) for s in range(NSEG) for g in range(NG) for j in range(NQT)
             for i in range(j + 1)]
    ns = len(steps)
    mx, tok, due = {}, {}, {}
    never = prow > i1 + 8
    lane8 = _iota((8, T), 1)
    hi = lane8 >= T // 2
    sl = [lane8 // QB == c for c in range(HG)]
    mid = sl[1] | sl[2]
    def q_masked(s, g, j, c):
        h = HG * g + c
        pos0 = (DH * h) // 16 - GWIN[g] // 16
        zero = jnp.zeros((8, T), u32)
        return ([zero] * pos0 + [q_s[s, h, j, 0:8], q_s[s, h, j, 8:16]]
                + [zero] * (GK // 16 - 2 - pos0))

    def k_rows(s, g, r0, r1_):
        return _unpack(k_s[s + z, g, r0 // 2:r1_ // 2, :])[:, :GK]

    def sel(mask, a, b):
        n_ = len(a) if isinstance(a, list) else len(b)
        out = []
        for r_ in range(n_):
            x = a[r_] if isinstance(a, list) else a
            y = b[r_] if isinstance(b, list) else b
            out.append(x if x is y else jnp.where(mask, x, y))
        return out

    def stash(n, st, row0, col0, bias_row0=None):
        m = None
        w = st.shape[1]
        for r_ in range(0, st.shape[0], 8):
            x = st[r_:r_ + 8]
            if bias_row0 is not None:
                x = x + bias_s[bias_row0 + r_:bias_row0 + r_ + 8, col0:col0 + w]
            s_s[n % NB, row0 + r_:row0 + r_ + 8, col0:col0 + w] = x
            m = x if m is None else jnp.maximum(m, x)
        return m

    def weights(tiles_):
        return _unpack(jnp.concatenate([jnp.concatenate(q, axis=0) for q in tiles_], axis=1))

    def qk(n):
        s, g, j, i = steps[n]
        qm = [q_masked(s, g, j, c) for c in range(HG)]
        if i < j:
            ahead = QB if MERGE and i == j - 1 else 0
            st = _dot(k_rows(s, g, T * i, T * (i + 1) + ahead), weights(qm))
            tok[n] = st[8 * TOKROW:8 * TOKROW + 8]
            m = stash(n, st[:T], 0, 0)
            if ahead:
                m = jnp.maximum(m, stash(n + 1, st[T:], 0, 0, 0))
            mx[s, g, j] = m if i == 0 else jnp.maximum(mx[s, g, j], m)
            return
        if j == 0 or not MERGE:
            m = stash(n, _dot(k_rows(s, g, T * i, T * i + QB), weights(qm)), 0, 0, 0)
            if j > 0:
                m = jnp.maximum(mx[s, g, j], m)
        else:
            m = mx[s, g, j]
        x1 = _dot(k_rows(s, g, T * i + QB, T * i + 2 * QB),
                  weights([sel(sl[c], qm[3], qm[c]) for c in range(3)]))
        x3 = _dot(k_rows(s, g, T * i + 3 * QB, T * (i + 1)),
                  weights([sel(hi, sel(mid, qm[3], qm[0]), sel(mid, qm[2], qm[1]))]))
        tok[n] = jnp.concatenate([x1[QB - 8:], x3[QB - 8:]], axis=1)
        m1 = stash(n, x1, QB, 0, QB)
        m1 = [m1[:, T * c:T * (c + 1)] for c in range(3)]
        m3 = stash(n, x3, QB, 3 * T, QB)
        m2 = []
        for c, w in enumerate((sel(hi, qm[0], qm[2]), sel(mid, qm[3], qm[1]))):
            parts = [stash(n, _dot(k_rows(s, g, T * i + r0, T * i + r0 + QB // 2), weights([w])),
                           r0, T * c, r0) for r0 in (2 * QB, 2 * QB + QB // 2)]
            m2.append(jnp.maximum(*parts))
        ms = []
        for c in range(HG):
            x = m[:, T * c:T * (c + 1)]
            if c < 3:
                x = jnp.where(sl[c], x, jnp.maximum(x, m1[c]))
            else:
                for b in range(3):
                    x = jnp.where(sl[b], jnp.maximum(x, m1[b]), x)
            y = jnp.maximum(x, m2[c % 2])
            x = jnp.where((hi, mid)[c % 2], *((y, x) if c in (0, 3) else (x, y)))
            ms.append(jnp.where(sl[(c + 3) % HG], jnp.maximum(x, m3), x))
        mx[s, g, j] = jnp.max(jnp.concatenate(ms, axis=1), axis=0, keepdims=True)

    def pv(n):
        s, g, j, i = steps[n]
        ms = []
        for c in range(HG):
            m = jnp.broadcast_to(mx[s, g, j][:, T * c:T * (c + 1)], (8, T))
            t_ = tok[n + LAG - (TOKBACK if n + LAG <= ns else ETOK)][:, T * c:T * (c + 1)]
            for x in due.pop((n, c), ()):
                t_ = jnp.maximum(t_, x)
            ms.append(jnp.where(never, t_, m))

        def probs(r0, r1_, c, m):
            return [jnp.exp2(s_s[n % NB, r_:r_ + 8, T * c:T * (c + 1)] - m) for r_ in range(r0, r1_, 8)]

        if i == j:
            e1 = [probs(QB, 2 * QB, c, jnp.where(sl[c], ms[3], ms[c])) for c in range(3)]
            e3 = probs(QB, 2 * QB, 3, jnp.where(hi, jnp.where(mid, ms[3], ms[0]),
                                                jnp.where(mid, ms[2], ms[1])))
            e2 = [probs(2 * QB, 3 * QB, 0, jnp.where(hi, ms[0], ms[2])),
                  probs(2 * QB, 3 * QB, 1, jnp.where(mid, ms[3], ms[1]))]
        for c in range(HG):
            if i == j:
                p = probs(0, QB, c, ms[c])
                if c < 3:
                    p += sel(sl[c], 0.0, e1[c])
                else:
                    p += sel(sl[0], e1[0], sel(sl[1], e1[1], sel(sl[2], e1[2], 0.0)))
                p += sel((hi, mid)[c % 2], *((e2[c % 2], 0.0) if c in (0, 3) else (0.0, e2[c % 2])))
                p += sel(sl[(c + 3) % HG], e3, 0.0)
            else:
                p = probs(0, T, c, ms[c])
            p = jnp.concatenate(p, axis=0)
            h = HG * g + c
            a = DH * h // 8 * 8
            o = DH * h - a
            one = 23 if o == 0 else 0
            vt = [v_s[s, a + 8 * r_:a + 8 * r_ + 8, T * i:T * (i + 1)] for r_ in range(3)]
            vt[one // 8] = jnp.where(prow == one % 8, 1.0, vt[one // 8])
            r_ = _dot_mixed(jnp.concatenate(vt, axis=0), p.astype(bf16))
            if i > 0:
                r_ = acc_s[c] + r_
            if i < j:
                acc_s[c] = r_
            else:
                l = r_[one:one + 1]
                inv = pltpu.reciprocal(l, approx=True)
                inv = inv * (2.0 - l * inv)
                sc = (1.0 - g_s[h:h + 1, :]) * (inv * (2.0 - l * inv))
                val = r_ * sc
                if c:
                    val = pltpu.roll(val, T - QB * c, 1)
                for r0 in range(0, 24, 8):
                    due.setdefault((n + DUE, c), []).append(val[r0:r0 + 8])
                o_s[s % 2, DH * h:DH * (h + 1), T * j:T * (j + 1)] = val[o:o + DH]

    def win_rows(t):
        heads = WIN_HEADS[t]
        return DH * heads[0] // 8 * 8, -(-DH * (heads[-1] + 1) // 8) * 8

    def mem_read(s, t):
        heads = WIN_HEADS[t]
        r0 = WIN * t
        ra0, re0 = win_rows(t)
        lhs = jnp.concatenate(
            [jnp.where(mask_s[t, a:b] > 0, _round_bf16(m_s[t, a:b]), 0.0)
             for a, b in ((ra0 - r0, re0 - r0), (T, T + 8))], axis=0)
        rd = _dot_mixed(lhs, _unpack(pq_s[s - 1, r0 // 2:r0 // 2 + 64, :]))
        h0 = heads[0]
        coef = jnp.concatenate([g_s[h0:h0 + 8, :]] * NQT, axis=1) / (rd[re0 - ra0:] + 1e-6)
        lo_row = DH * heads[0]
        hi_row = DH * (heads[-1] + 1)
        for rb in range(ra0, re0, 8):
            ha = max(rb // DH, h0)
            hb = min((rb + 7) // DH, heads[-1])
            cf = jnp.broadcast_to(coef[ha - h0:ha - h0 + 1], (8, L))
            if hb != ha:
                cf = jnp.where(_iota((8, L), 0) < DH * hb - rb, cf,
                               jnp.broadcast_to(coef[hb - h0:hb - h0 + 1], (8, L)))
            val = rd[rb - ra0:rb - ra0 + 8] * cf
            ra, re = max(rb, lo_row), min(rb + 8, hi_row)
            om_s[s % 2, ra:re, :] = val[ra - rb:re - rb]

    def mem_update(s, t):
        r0 = WIN * t
        ra0, re0 = win_rows(t)
        vl = jnp.concatenate([v_s[s, ra0:re0, :], jnp.ones((8, L), f32)], axis=0)
        upd = lax.dot_general(vl, _unpack(pk_s[s, r0 // 2:r0 // 2 + 64, :]),
                              (((1,), (1,)), ((), ())), preferred_element_type=f32)
        for a, b, u in ((ra0 - r0, re0 - r0, upd[:re0 - ra0]), (T, T + 8, upd[re0 - ra0:])):
            m_s[t, a:b] = u if s == 0 else m_s[t, a:b] + u

    def pack_o(s, r0, r1_):
        o = o_s[s % 2, r0:r1_, :]
        if s > 0:
            o = o + om_s[s % 2, r0:r1_, :]
        ob_s[s, r0 // 2:r1_ // 2, :] = _pack(o.astype(bf16))

    def out_proj(s, r0, r1_, n=None):
        ob = ob_s[s]
        if n is not None:
            head = jnp.where(jnp.concatenate([never] * HG, axis=1),
                             pltpu.bitcast(tok[n - PINBACK], u32), ob[:8])
            ob = jnp.concatenate([head, ob[8:]], axis=0)
        res = _dot(_unpack(wot[z, r0 // 2:r1_ // 2, :]), _unpack(ob))
        if n is not None:
            tok[n] = res[:8]
        xn = _unpack(jnp.concatenate(
            [xn_s[NQT * s + j, r0 // 2:r1_ // 2, :] for j in range(NQT)], axis=1))
        out_v[s, r0:r1_, :] = (res + x_v[s, r0:r1_, :].astype(f32) + xn.astype(f32)).astype(bf16)

    for s in range(NSEG):
        tpos = _iota((16, L), 1) + s * L
        pick = jnp.where(_iota((16, L), 0) == 0, i1, jnp.where(_iota((16, L), 0) == 1, i2, -1))
        ob_s[s, D // 2:D // 2 + 8, :] = _pack(jnp.where(tpos == pick, 1.0, 0.0).astype(bf16))
        ob_s[s, D // 2 + 8:DP // 2, :] = jnp.zeros(((DP - D) // 2 - 8, L), u32)

    extra = {}

    def at(n, fn, *args):
        extra.setdefault(n, []).append((fn,) + args)

    per = ns // NSEG
    full = [n for n, (_, _, j, i) in enumerate(steps) if i < j]
    busy = set()

    def at_full(n, fn, *args):
        n = next(m for m in full if m >= n and m not in busy)
        busy.add(n)
        at(n, fn, *args)
        return n

    for t in range(NWIN):
        at_full(0, mem_update, 0, t)
        for s in range(1, NSEG):
            at_full(per * s - 40 + 6 * t, mem_read, s, t)
            if s < NSEG - 1:
                at_full(per * s + 4 + 6 * t, mem_update, s, t)

    busy.clear()

    def late_weights():
        for cp in (cp_wo, cp_wg, cp_wu, cp_wd):
            cp.wait()

    at(MOE0, late_weights)
    n = MOE0
    for rd_ in rounds:
        n = at_full(n, *rd_) if rd_ is not None else n + 2
    at(n + 2, ffn_finish)
    for c in range(20):
        at(MOE0 + 2 * c + 1, _store_wt, wot, 0, wo_v, c % 4, c // 4)
    for s in range(NSEG):
        for c in range(D // 48):
            n = per * s + 10 * ((48 * (c + 1) - 1) // (HG * DH) + 1) + LAG + c % 2 * 3 + 1
            at(min(n, ns + LAG), pack_o, s, 48 * c, 48 * (c + 1))
    for c in range(LAG):
        at(ns + c, out_proj, 0, FILL * c, FILL * (c + 1), ns + c)

    for n in range(ns + LAG):
        if n < ns:
            qk(n)
        for task in extra.get(n, ()):
            if not (AFTER and task[0] is ffn_in):
                task[0](*task[1:])
        if n >= LAG:
            pv(n - LAG)
        for task in extra.get(n, ()):
            if AFTER and task[0] is ffn_in:
                task[0](*task[1:])
    for task in extra[ns + LAG]:
        task[0](*task[1:])
    for s in range(NSEG - 1):
        out_proj(s, FILL * LAG if s == 0 else 0, D, ns + LAG + s if s == 0 else None)
        cp_o[s].start()
    for (r0, r1_), cp in zip(TAIL, cp_tail):
        out_proj(NSEG - 1, r0, r1_)
        cp.start()
    for cp in cp_o + cp_tail:
        cp.wait()


@jax.jit
def pallas_parallel_sum__memory_aug_infini_attn__moe_arch_mod__prompt_kernel(
    A_x, A_wq, A_wk, A_wv, A_wo, A_beta, B_x, B_w_r, B_w_gate, B_w_up, B_w_down,
):
    del B_x
    any_spec = pl.BlockSpec(memory_space=pl.ANY)
    out_t = pl.pallas_call(
        kernel,
        out_shape=jax.ShapeDtypeStruct((D, S), bf16),
        in_specs=[any_spec] * 10,
        out_specs=any_spec,
        scratch_shapes=[
            pltpu.VMEM((NSEG, D, L), bf16),
            pltpu.VMEM((D, D), bf16),
            pltpu.VMEM((D, D), bf16),
            pltpu.VMEM((D, D), bf16),
            pltpu.VMEM((D, D), bf16),
            pltpu.VMEM((D, F), bf16),
            pltpu.VMEM((D, F), bf16),
            pltpu.VMEM((D, F), bf16),
            pltpu.VMEM((NSEG, D, L), bf16),
            pltpu.VMEM((1, NROW // 2, DP), u32),
            pltpu.VMEM((1, D // 2, DP), u32),
            pltpu.VMEM((S // T, DP // 2, T), u32),
            pltpu.VMEM((NSEG, H, NQT, 16, T), u32),
            pltpu.VMEM((NSEG, NG, L // 2, T), u32),
            pltpu.VMEM((NSEG, D, L), f32),
            pltpu.VMEM((NSEG - 1, D // 2, L), u32),
            pltpu.VMEM((NSEG - 1, D // 2, L), u32),
            pltpu.VMEM((S // T, T), f32),
            pltpu.VMEM((T, T), f32),
            pltpu.VMEM((2, D, L), f32),
            pltpu.VMEM((NSEG, DP // 2, L), u32),
            pltpu.VMEM((NWIN, T + 8, T), f32),
            pltpu.VMEM((2, D, L), f32),
            pltpu.VMEM((NWIN, T + 8, T), f32),
            pltpu.VMEM((NB, T, HG * T), f32),
            pltpu.VMEM((8, F), f32),
            pltpu.VMEM((2, D // 2, T), f32),
            pltpu.VMEM((HG, 24, T), f32),
            pltpu.VMEM((3 * QB, HG * T), f32),
            pltpu.VMEM((1, H), bf16),
            pltpu.VMEM((D,), bf16),
            pltpu.SemaphoreType.DMA((7,)),
        ],
        compiler_params=pltpu.CompilerParams(vmem_limit_bytes=100 * 1024 * 1024),
        name="infini_moe",
    )(A_x.reshape(S, D).T, A_wq, A_wk, A_wv, A_wo, A_beta.reshape(1, H), B_w_r,
      B_w_gate, B_w_up, B_w_down.T)
    return out_t.T.reshape(1, S, D)
```

```python
import math
import os

import jax
import jax.numpy as jnp
import numpy as np
from jax import lax
import jax.experimental.pallas as pl
import jax.experimental.pallas.tpu as pltpu

S = 2048
D = 576
H = 32
DH = D // H
NSEG = 4
L = S // NSEG
F = 4608
T = 128
DP = 640
NQT = L // T
WIN = 112
NWIN = 5
HEAD_WIN = [0] * 7 + [1] * 6 + [2] * 6 + [3] * 6 + [4] * 7
WIN_HEADS = [[h for h in range(H) if HEAD_WIN[h] == t] for t in range(NWIN)]
HG = 4
NG = H // HG
AFTER = int(os.environ.get('AFTER', 1))
PINBACK = int(os.environ.get('PINBACK', 2))
ETOK = int(os.environ.get('ETOK', 2))
DUE = int(os.environ.get('DUE', 20))
QB = T // HG
MERGE = int(os.environ.get('MERGE', 1))
GK = 80
GWIN = [HG * DH * g // 16 * 16 for g in range(NG)]
TOKROW = int(os.environ.get('TOKROW', 10))
TOKBACK = int(os.environ.get('TOKBACK', 2))
MOE0 = int(os.environ.get('MOE0', 61))
LAG = int(os.environ.get('LAG', 11))
NB = int(os.environ.get('NB', 13))
RQ, RK, RV = 0, D, 2 * D
NROW = 3 * D
FILL = int(os.environ.get('FILL', 48))
VSPLIT = int(os.environ.get('VSPLIT', 448))
TAIL = ((0, 288), (288, 480), (480, D))
LOG2E = math.log2(math.e)
QSCALE = DH ** -0.5 * LOG2E
MASKVAL = -999292928.0 * LOG2E
LN_EPS = float(np.asarray(1e-5, dtype=jnp.bfloat16).astype(np.float32))

bf16 = jnp.bfloat16
f32 = jnp.float32
u32 = jnp.uint32


def _pack(x):
    return pltpu.bitcast(x, u32)


def _unpack(x):
    return pltpu.bitcast(x, bf16)


def _halves(x):
    return [pltpu.unpack_elementwise(x, index=i, packed_dtype=bf16, unpacked_dtype=f32)
            for i in range(2)]


def _join(even, odd):
    return pltpu.bitcast(pltpu.pack_elementwise([even, odd], packed_dtype=bf16), u32)


def _dot(a, b):
    return lax.dot_general(a, b, (((1,), (0,)), ((), ())), preferred_element_type=f32)


def _dot_nt(a, b):
    return lax.dot_general(a, b, (((1,), (1,)), ((), ())), preferred_element_type=f32)


def _dot_mixed(a, b):
    return lax.dot_general(a, b, (((1,), (0,)), ((), ())), preferred_element_type=f32)


def _iota(shape, dim):
    return lax.broadcasted_iota(jnp.int32, shape, dim)


def _phi(t):
    return jnp.where(t > 0, t + 1.0, jnp.exp(t))


def _round_bf16(x):
    return x.astype(bf16).astype(f32)


def _sigmoid(x):
    return 1.0 / (1.0 + jnp.exp(-x))


def _w_tile(w_ref, i, j, tail=None):
    r = min(T, D - T * i)
    c = min(T, D - T * j)
    t = w_ref[T * i:T * i + r, T * j:T * j + c]
    if c < T:
        t = jnp.concatenate([t, jnp.zeros((r, T - c), bf16)], axis=1)
    if r < T:
        parts = [t]
        if tail is not None:
            parts.append(tail)
        n = T - sum(p.shape[0] for p in parts)
        parts.append(jnp.zeros((n, T), bf16))
        t = jnp.concatenate(parts, axis=0)
    return t


def _store_wt(dst, row0, w_ref, i, j, tail=None):
    c = min(T, D - T * j)
    t = _pack(_w_tile(w_ref, i, j, tail).T)
    r0 = (row0 + T * j) // 2
    dst[0, r0:r0 + c // 2, T * i:T * (i + 1)] = t[:c // 2]


def kernel(x_hbm, wq_hbm, wk_hbm, wv_hbm, wo_hbm, beta_hbm, wr_hbm, wg_hbm, wu_hbm, wd_hbm,
           out_hbm,
           x_v, wq_v, wk_v, wv_v, wo_v, wg_v, wu_v, wd_v, out_v,
           wt, wot, xn_s, q_s, k_s, v_s, pq_s, pk_s, r_s, g_s, o_s, ob_s, m_s, om_s, mask_s, s_s,
           h_s, wr_s, acc_s, bias_s, beta_ref, wr_ref, sems):
    cp_x = [pltpu.make_async_copy(x_hbm.at[:, pl.ds(s * L, L)], x_v.at[s], sems.at[(0, 3, 4, 4)[s]])
            for s in range(NSEG)]
    cp_o = [pltpu.make_async_copy(out_v.at[s], out_hbm.at[:, pl.ds(s * L, L)], sems.at[6])
            for s in range(NSEG - 1)]
    cp_tail = [pltpu.make_async_copy(out_v.at[NSEG - 1, pl.ds(r0, r1 - r0)],
                                     out_hbm.at[pl.ds(r0, r1 - r0), pl.ds(S - L, L)],
                                     sems.at[6])
               for c, (r0, r1) in enumerate(TAIL)]
    cp_wk = pltpu.make_async_copy(wk_hbm, wk_v, sems.at[3])
    cp_wq = pltpu.make_async_copy(wq_hbm, wq_v, sems.at[2])
    cp_wv = pltpu.make_async_copy(wv_hbm, wv_v, sems.at[1])
    cp_wo = pltpu.make_async_copy(wo_hbm, wo_v, sems.at[5])
    cp_wg = pltpu.make_async_copy(wg_hbm, wg_v, sems.at[5])
    cp_wu = pltpu.make_async_copy(wu_hbm, wu_v, sems.at[5])
    cp_wd = pltpu.make_async_copy(wd_hbm, wd_v, sems.at[5])
    cp_beta = pltpu.make_async_copy(beta_hbm, beta_ref, sems.at[0])
    cp_wr = pltpu.make_async_copy(wr_hbm, wr_ref, sems.at[0])
    for cp in (cp_x[0], cp_beta, cp_wr, cp_wv, cp_wq, cp_x[1], cp_wk, cp_x[2], cp_x[3],
               cp_wo, cp_wg, cp_wu, cp_wd):
        cp.start()

    colh = _iota((T, T), 1)
    rowh = _iota((T, T), 0)
    for t in range(NWIN):
        same = None
        zsel = None
        for n, h in enumerate(WIN_HEADS[t]):
            cin = (colh >= DH * h - WIN * t) & (colh < DH * (h + 1) - WIN * t)
            blk = cin & (rowh >= DH * h - WIN * t) & (rowh < DH * (h + 1) - WIN * t)
            same = blk if same is None else same | blk
            zc = cin[:8] & (rowh[:8] == n)
            zsel = zc if zsel is None else zsel | zc
        mask_s[t, 0:T] = jnp.where(same, 1.0, 0.0)
        mask_s[t, T:T + 8] = jnp.where(zsel, 1.0, 0.0)
    key = _iota((QB, T), 0)
    qry = _iota((QB, T), 1)
    qpos = [(qry - QB * c) % T for c in range(HG)]
    slot = qry // QB
    tiles = [qpos,
             [jnp.where(slot == c, qpos[3], qpos[c]) for c in range(3)] + [qry % QB + QB],
             [jnp.where(slot >= 2, qpos[0], qpos[2]),
              jnp.where((slot == 1) | (slot == 2), qpos[3], qpos[1])]]
    for b, row in enumerate(tiles):
        for c, qp_ in enumerate(row):
            bias_s[QB * b:QB * (b + 1), T * c:T * (c + 1)] = jnp.where(
                qp_ < key + QB * b, MASKVAL, 0.0)
    for j in range(S // T):
        xn_s[j, D // 2:DP // 2 - 8, :] = jnp.zeros(((DP - D) // 2 - 8, T), u32)

    def transpose_w(row0, w):
        for j in range(5):
            for i in range(5):
                _store_wt(wt, row0, w, i, j)

    def layernorm(s, j):
        xe, xo = _halves(_pack(x_v[s, :, T * j:T * (j + 1)]))
        mean = jnp.sum(xe + xo, axis=0, keepdims=True) / D
        ce, co = xe - mean, xo - mean
        var = jnp.sum(ce * ce + co * co, axis=0, keepdims=True) / D
        inv = 1.0 / _round_bf16(jnp.sqrt(_round_bf16(_round_bf16(var) + LN_EPS)))
        mean = _round_bf16(mean)
        de, do = _halves(_join(xe - mean, xo - mean))
        xn = _join(de * inv, do * inv)
        even, odd = _halves(xn)
        score = jnp.broadcast_to(jnp.sum(even * wr_s[0] + odd * wr_s[1], axis=0, keepdims=True), (8, T))
        r_s[NQT * s + j:NQT * s + j + 1, :] = score[:1]
        xn_s[NQT * s + j, 0:D // 2, :] = xn
        xn_s[NQT * s + j, DP // 2 - 8:DP // 2, :] = jnp.where(
            never, pltpu.bitcast(score, u32), jnp.zeros((), u32))

    def router_weights():
        wr = jnp.concatenate([wr_ref[...].reshape(1, D), jnp.zeros((1, DP - D), bf16)], axis=1)
        even, odd = _halves(_pack(jnp.broadcast_to(wr, (T, DP)).T)[:D // 2])
        wr_s[0], wr_s[1] = even, odd

    def xn_seg(s):
        return _unpack(jnp.concatenate([xn_s[NQT * s + j] for j in range(NQT)], axis=1))

    def proj_q(s):
        q = _dot(_unpack(wt[z, RQ // 2:RK // 2, :]), xn_seg(s))
        if s > 0:
            pq_s[s - 1] = _pack(_phi(q[:D]).astype(bf16))
        qp = _pack((q[:D] * QSCALE).astype(bf16))
        for h in range(H):
            a = (DH * h) // 16
            lo = (DH * h - 16 * a) // 2
            prow = _iota((16, L), 0)
            qh = jnp.where((prow >= lo) & (prow <= lo + 8), qp[8 * a:8 * a + 16], jnp.zeros((), u32))
            for j in range(NQT):
                qt = qh[:, T * j:T * (j + 1)]
                q_s[s, h, j] = pltpu.roll(qt, QB * (h % HG), 1) if h % HG else qt

    def proj_k(s):
        k = _dot(_unpack(wt[z, RK // 2:RV // 2, :]), xn_seg(s))
        if s < NSEG - 1:
            pk_s[s] = _pack(_phi(k).astype(bf16))
        for j in range(NQT):
            kb = k[:, T * j:T * (j + 1)].astype(bf16)
            for g in range(NG):
                kw = jnp.concatenate([kb[GWIN[g]:GWIN[g] + GK], jnp.zeros((T - GK, T), bf16)], axis=0)
                k_s[s, g, 64 * j:64 * (j + 1), :] = _pack(kw.T)

    def proj_v(s, r0=0, r1_=D):
        v_s[s, r0:r1_, :] = _round_bf16(
            _dot(_unpack(wt[z, (RV + r0) // 2:(RV + r1_) // 2, :]), xn_seg(s)))

    cp_x[0].wait()
    cp_beta.wait()
    cp_wr.wait()
    g = _round_bf16(_sigmoid(beta_ref[...].astype(f32)))
    z = jnp.where(jnp.max(g) > 2.0, 1, 0)
    g = jnp.concatenate([g, jnp.zeros((1, T - H), f32)], axis=1)
    g_s[...] = jnp.broadcast_to(g, (T, T)).T
    prow = _iota((8, T), 0)
    never = prow > z + 8
    router_weights()
    for j in range(NQT):
        layernorm(0, j)
    cp_wv.wait()
    transpose_w(RV, wv_v)
    proj_v(0, 0, 384)
    cp_wq.wait()
    transpose_w(RQ, wq_v)
    proj_v(0, 384, 448)
    proj_q(0)
    proj_v(0, 448, 512)
    cp_x[1].wait()
    cp_wk.wait()
    transpose_w(RK, wk_v)
    for j in range(NQT):
        layernorm(1, j)
    proj_v(0, 512, D)
    proj_k(0)
    proj_v(1)
    cp_x[2].wait()
    cp_x[3].wait()
    for s in (2, 3):
        for j in range(NQT):
            layernorm(s, j)
        proj_q(s - 1)
    proj_q(3)

    r = _round_bf16(r_s[...])
    pos = _iota((S // T, T), 0) * T + _iota((S // T, T), 1)
    r1 = jnp.max(r)
    i1 = jnp.minimum(jnp.min(jnp.where(r == r1, pos, S)), S - 1)
    rest = pos != i1
    r2 = jnp.max(jnp.where(rest, r, -jnp.inf))
    i2 = jnp.minimum(jnp.min(jnp.where(rest & (r == r2), pos, S)), S - 1)

    for s in range(1, NSEG):
        proj_k(s)
        if s > 1:
            proj_v(s)

    lane = _iota((DP // 2, T), 1)
    xsel = jnp.zeros((8, DP), f32)
    for c, idx in enumerate((i1, i2)):
        col = jnp.where(lane == idx % T, xn_s[idx // T], jnp.zeros((), u32))
        xsel = xsel + _dot_nt(jnp.where(_iota((8, T), 0) == c, 1.0, 0.0), _unpack(col))

    moe = {}

    def ffn_in(w, name, cg, i):
        k = min(T, D - T * i)
        r_ = _dot(xsel[:, T * i:T * i + k], w[T * i:T * i + k, L * cg:L * (cg + 1)])
        moe[name] = r_ if i == 0 else moe[name] + r_
        if name == "up" and i == 4:
            gate = moe["gate"]
            hid = gate * _sigmoid(gate) * moe["up"]
            h_s[:, L * cg:L * (cg + 1)] = _round_bf16(hid)

    def ffn_out(cg, i):
        if i < 4:
            c0 = L * cg + T * i
            r_ = _dot_nt(h_s[:, c0:c0 + T], wd_v[0:4 * T, c0:c0 + T])
            moe["y0"] = r_ if "y0" not in moe else moe["y0"] + r_
        else:
            r_ = _dot_nt(h_s[:, L * cg:L * (cg + 1)], wd_v[4 * T:D, L * cg:L * (cg + 1)])
            moe["y1"] = r_ if "y1" not in moe else moe["y1"] + r_

    def ffn_finish():
        y = jnp.concatenate([moe["y0"], moe["y1"], jnp.zeros((8, DP - D), f32)], axis=1)
        y = y * _sigmoid(jnp.where(_iota((8, DP), 0) == 0, r1, r2))
        y = jnp.concatenate([y, jnp.zeros((8, DP), f32)], axis=0)
        for j in range(5):
            _store_wt(wot, 0, wo_v, 4, j, tail=y[:, T * j:T * (j + 1)].astype(bf16))

    rounds = []
    for cg in range(F // L):
        rounds += [(ffn_in, wg_v, "gate", cg, i) for i in range(5)]
        rounds += [(ffn_in, wu_v, "up", cg, i) for i in range(5)]
        if cg > 0:
            rounds += [(ffn_out, cg - 1, i) for i in range(5)]
    rounds += [None] * 3
    rounds += [(ffn_out, F // L - 1, i) for i in range(5)]

    steps = [(s, g, j, i) for s in range(NSEG) for g in range(NG) for j in range(NQT)
             for i in range(j + 1)]
    ns = len(steps)
    mx, tok, due = {}, {}, {}
    lane8 = _iota((8, T), 1)
    hi = lane8 >= T // 2
    sl = [lane8 // QB == c for c in range(HG)]
    mid = sl[1] | sl[2]
    def q_masked(s, g, j, c):
        h = HG * g + c
        pos0 = (DH * h) // 16 - GWIN[g] // 16
        zero = jnp.zeros((8, T), u32)
        return ([zero] * pos0 + [q_s[s, h, j, 0:8], q_s[s, h, j, 8:16]]
                + [zero] * (GK // 16 - 2 - pos0))

    def k_rows(s, g, r0, r1_):
        return _unpack(k_s[s + z, g, r0 // 2:r1_ // 2, :])[:, :GK]

    def sel(mask, a, b):
        n_ = len(a) if isinstance(a, list) else len(b)
        out = []
        for r_ in range(n_):
            x = a[r_] if isinstance(a, list) else a
            y = b[r_] if isinstance(b, list) else b
            out.append(x if x is y else jnp.where(mask, x, y))
        return out

    def stash(n, st, row0, col0, bias_row0=None):
        m = None
        w = st.shape[1]
        for r_ in range(0, st.shape[0], 8):
            x = st[r_:r_ + 8]
            if bias_row0 is not None:
                x = x + bias_s[bias_row0 + r_:bias_row0 + r_ + 8, col0:col0 + w]
            s_s[n % NB, row0 + r_:row0 + r_ + 8, col0:col0 + w] = x
            m = x if m is None else jnp.maximum(m, x)
        return m

    def weights(tiles_):
        return _unpack(jnp.concatenate([jnp.concatenate(q, axis=0) for q in tiles_], axis=1))

    def qk(n):
        s, g, j, i = steps[n]
        qm = [q_masked(s, g, j, c) for c in range(HG)]
        if i < j:
            ahead = QB if MERGE and i == j - 1 else 0
            st = _dot(k_rows(s, g, T * i, T * (i + 1) + ahead), weights(qm))
            tok[n] = st[8 * TOKROW:8 * TOKROW + 8]
            m = stash(n, st[:T], 0, 0)
            if ahead:
                m = jnp.maximum(m, stash(n + 1, st[T:], 0, 0, 0))
            mx[s, g, j] = m if i == 0 else jnp.maximum(mx[s, g, j], m)
            return
        if j == 0 or not MERGE:
            m = stash(n, _dot(k_rows(s, g, T * i, T * i + QB), weights(qm)), 0, 0, 0)
            if j > 0:
                m = jnp.maximum(mx[s, g, j], m)
        else:
            m = mx[s, g, j]
        x1 = _dot(k_rows(s, g, T * i + QB, T * i + 2 * QB),
                  weights([sel(sl[c], qm[3], qm[c]) for c in range(3)]))
        x3 = _dot(k_rows(s, g, T * i + 3 * QB, T * (i + 1)),
                  weights([sel(hi, sel(mid, qm[3], qm[0]), sel(mid, qm[2], qm[1]))]))
        tok[n] = jnp.concatenate([x1[QB - 8:], x3[QB - 8:]], axis=1)
        m1 = stash(n, x1, QB, 0, QB)
        m1 = [m1[:, T * c:T * (c + 1)] for c in range(3)]
        m3 = stash(n, x3, QB, 3 * T, QB)
        m2 = []
        for c, w in enumerate((sel(hi, qm[0], qm[2]), sel(mid, qm[3], qm[1]))):
            parts = [stash(n, _dot(k_rows(s, g, T * i + r0, T * i + r0 + QB // 2), weights([w])),
                           r0, T * c, r0) for r0 in (2 * QB, 2 * QB + QB // 2)]
            m2.append(jnp.maximum(*parts))
        ms = []
        for c in range(HG):
            x = m[:, T * c:T * (c + 1)]
            if c < 3:
                x = jnp.where(sl[c], x, jnp.maximum(x, m1[c]))
            else:
                for b in range(3):
                    x = jnp.where(sl[b], jnp.maximum(x, m1[b]), x)
            y = jnp.maximum(x, m2[c % 2])
            x = jnp.where((hi, mid)[c % 2], *((y, x) if c in (0, 3) else (x, y)))
            ms.append(jnp.where(sl[(c + 3) % HG], jnp.maximum(x, m3), x))
        mx[s, g, j] = jnp.max(jnp.concatenate(ms, axis=1), axis=0, keepdims=True)

    def pv(n):
        s, g, j, i = steps[n]
        ms = []
        for c in range(HG):
            m = jnp.broadcast_to(mx[s, g, j][:, T * c:T * (c + 1)], (8, T))
            t_ = tok[n + LAG - (TOKBACK if n + LAG <= ns else ETOK)][:, T * c:T * (c + 1)]
            for x in due.pop((n, c), ()):
                t_ = jnp.maximum(t_, x)
            ms.append(jnp.where(never, t_, m))

        def probs(r0, r1_, c, m):
            return [jnp.exp2(s_s[n % NB, r_:r_ + 8, T * c:T * (c + 1)] - m) for r_ in range(r0, r1_, 8)]

        if i == j:
            e1 = [probs(QB, 2 * QB, c, jnp.where(sl[c], ms[3], ms[c])) for c in range(3)]
            e3 = probs(QB, 2 * QB, 3, jnp.where(hi, jnp.where(mid, ms[3], ms[0]),
                                                jnp.where(mid, ms[2], ms[1])))
            e2 = [probs(2 * QB, 3 * QB, 0, jnp.where(hi, ms[0], ms[2])),
                  probs(2 * QB, 3 * QB, 1, jnp.where(mid, ms[3], ms[1]))]
        for c in range(HG):
            if i == j:
                p = probs(0, QB, c, ms[c])
                if c < 3:
                    p += sel(sl[c], 0.0, e1[c])
                else:
                    p += sel(sl[0], e1[0], sel(sl[1], e1[1], sel(sl[2], e1[2], 0.0)))
                p += sel((hi, mid)[c % 2], *((e2[c % 2], 0.0) if c in (0, 3) else (0.0, e2[c % 2])))
                p += sel(sl[(c + 3) % HG], e3, 0.0)
            else:
                p = probs(0, T, c, ms[c])
            p = jnp.concatenate(p, axis=0)
            h = HG * g + c
            a = DH * h // 8 * 8
            o = DH * h - a
            one = 23 if o == 0 else 0
            vt = [v_s[s, a + 8 * r_:a + 8 * r_ + 8, T * i:T * (i + 1)] for r_ in range(3)]
            vt[one // 8] = jnp.where(prow == one % 8, 1.0, vt[one // 8])
            r_ = _dot_mixed(jnp.concatenate(vt, axis=0), p.astype(bf16))
            if i > 0:
                r_ = acc_s[c] + r_
            if i < j:
                acc_s[c] = r_
            else:
                l = r_[one:one + 1]
                inv = pltpu.reciprocal(l, approx=True)
                inv = inv * (2.0 - l * inv)
                sc = (1.0 - g_s[h:h + 1, :]) * (inv * (2.0 - l * inv))
                val = r_ * sc
                if c:
                    val = pltpu.roll(val, T - QB * c, 1)
                for r0 in range(0, 24, 8):
                    due.setdefault((n + DUE, c), []).append(val[r0:r0 + 8])
                o_s[s % 2, DH * h:DH * (h + 1), T * j:T * (j + 1)] = val[o:o + DH]

    def win_rows(t):
        heads = WIN_HEADS[t]
        return DH * heads[0] // 8 * 8, -(-DH * (heads[-1] + 1) // 8) * 8

    def mem_read(s, t):
        heads = WIN_HEADS[t]
        r0 = WIN * t
        ra0, re0 = win_rows(t)
        lhs = jnp.concatenate(
            [jnp.where(mask_s[t, a:b] > 0, _round_bf16(m_s[t, a:b]), 0.0)
             for a, b in ((T, T + 8), (ra0 - r0, re0 - r0))], axis=0)
        rd = _dot_mixed(lhs, _unpack(pq_s[s - 1, r0 // 2:r0 // 2 + 64, :]))
        h0 = heads[0]
        coef = jnp.concatenate([g_s[h0:h0 + 8, :]] * NQT, axis=1) / (rd[:8] + 1e-6)
        lo_row = DH * heads[0]
        hi_row = DH * (heads[-1] + 1)
        for rb in range(ra0, re0, 8):
            ha = max(rb // DH, h0)
            hb = min((rb + 7) // DH, heads[-1])
            cf = jnp.broadcast_to(coef[ha - h0:ha - h0 + 1], (8, L))
            if hb != ha:
                cf = jnp.where(_iota((8, L), 0) < DH * hb - rb, cf,
                               jnp.broadcast_to(coef[hb - h0:hb - h0 + 1], (8, L)))
            val = rd[rb - ra0 + 8:rb - ra0 + 16] * cf
            ra, re = max(rb, lo_row), min(rb + 8, hi_row)
            om_s[s % 2, ra:re, :] = val[ra - rb:re - rb]

    def mem_update(s, t):
        r0 = WIN * t
        ra0, re0 = win_rows(t)
        vl = jnp.concatenate([v_s[s, ra0:re0, :], jnp.ones((8, L), f32)], axis=0)
        upd = lax.dot_general(vl, _unpack(pk_s[s, r0 // 2:r0 // 2 + 64, :]),
                              (((1,), (1,)), ((), ())), preferred_element_type=f32)
        for a, b, u in ((ra0 - r0, re0 - r0, upd[:re0 - ra0]), (T, T + 8, upd[re0 - ra0:])):
            m_s[t, a:b] = u if s == 0 else m_s[t, a:b] + u

    def pack_o(s, r0, r1_):
        o = o_s[s % 2, r0:r1_, :]
        if s > 0:
            o = o + om_s[s % 2, r0:r1_, :]
        ob_s[s, r0 // 2:r1_ // 2, :] = _pack(o.astype(bf16))

    def out_proj(s, r0, r1_, n=None):
        ob = ob_s[s]
        if n is not None:
            head = jnp.where(jnp.concatenate([never] * HG, axis=1),
                             pltpu.bitcast(tok[n - PINBACK], u32), ob[:8])
            ob = jnp.concatenate([head, ob[8:]], axis=0)
        res = _dot(_unpack(wot[z, r0 // 2:r1_ // 2, :]), _unpack(ob))
        if n is not None:
            tok[n] = res[:8]
        xn = _unpack(jnp.concatenate(
            [xn_s[NQT * s + j, r0 // 2:r1_ // 2, :] for j in range(NQT)], axis=1))
        out_v[s, r0:r1_, :] = (res + x_v[s, r0:r1_, :].astype(f32) + xn.astype(f32)).astype(bf16)

    for s in range(NSEG):
        tpos = _iota((16, L), 1) + s * L
        pick = jnp.where(_iota((16, L), 0) == 0, i1, jnp.where(_iota((16, L), 0) == 1, i2, -1))
        ob_s[s, D // 2:D // 2 + 8, :] = _pack(jnp.where(tpos == pick, 1.0, 0.0).astype(bf16))
        ob_s[s, D // 2 + 8:DP // 2, :] = jnp.zeros(((DP - D) // 2 - 8, L), u32)

    extra = {}

    def at(n, fn, *args):
        extra.setdefault(n, []).append((fn,) + args)

    per = ns // NSEG
    full = [n for n, (_, _, j, i) in enumerate(steps) if i < j]
    busy = set()

    def at_full(n, fn, *args):
        n = next(m for m in full if m >= n and m not in busy)
        busy.add(n)
        at(n, fn, *args)
        return n

    for t in range(NWIN):
        at_full(0, mem_update, 0, t)
        for s in range(1, NSEG):
            at_full(per * s - 40 + 6 * t, mem_read, s, t)
            if s < NSEG - 1:
                at_full(per * s + 4 + 6 * t, mem_update, s, t)

    busy.clear()

    def late_weights():
        for cp in (cp_wo, cp_wg, cp_wu, cp_wd):
            cp.wait()

    at(MOE0, late_weights)
    n = MOE0
    for rd_ in rounds:
        n = at_full(n, *rd_) if rd_ is not None else n + 2
    at(n + 2, ffn_finish)
    for c in range(20):
        at(MOE0 + 2 * c + 1, _store_wt, wot, 0, wo_v, c % 4, c // 4)
    for s in range(NSEG):
        for c in range(D // 48):
            n = per * s + 10 * ((48 * (c + 1) - 1) // (HG * DH) + 1) + LAG + c % 2 * 3 + 1
            at(min(n, ns + LAG), pack_o, s, 48 * c, 48 * (c + 1))
    for c in range(LAG):
        at(ns + c, out_proj, 0, FILL * c, FILL * (c + 1), ns + c)

    for n in range(ns + LAG):
        if n < ns:
            qk(n)
        for task in extra.get(n, ()):
            if not (AFTER and task[0] is ffn_in):
                task[0](*task[1:])
        if n >= LAG:
            pv(n - LAG)
        for task in extra.get(n, ()):
            if AFTER and task[0] is ffn_in:
                task[0](*task[1:])
    for task in extra[ns + LAG]:
        task[0](*task[1:])
    for s in range(NSEG - 1):
        out_proj(s, FILL * LAG if s == 0 else 0, D, ns + LAG + s if s == 0 else None)
        cp_o[s].start()
    for (r0, r1_), cp in zip(TAIL, cp_tail):
        out_proj(NSEG - 1, r0, r1_)
        cp.start()
    for cp in cp_o + cp_tail:
        cp.wait()


@jax.jit
def pallas_parallel_sum__memory_aug_infini_attn__moe_arch_mod__prompt_kernel(
    A_x, A_wq, A_wk, A_wv, A_wo, A_beta, B_x, B_w_r, B_w_gate, B_w_up, B_w_down,
):
    del B_x
    any_spec = pl.BlockSpec(memory_space=pl.ANY)
    out_t = pl.pallas_call(
        kernel,
        out_shape=jax.ShapeDtypeStruct((D, S), bf16),
        in_specs=[any_spec] * 10,
        out_specs=any_spec,
        scratch_shapes=[
            pltpu.VMEM((NSEG, D, L), bf16),
            pltpu.VMEM((D, D), bf16),
            pltpu.VMEM((D, D), bf16),
            pltpu.VMEM((D, D), bf16),
            pltpu.VMEM((D, D), bf16),
            pltpu.VMEM((D, F), bf16),
            pltpu.VMEM((D, F), bf16),
            pltpu.VMEM((D, F), bf16),
            pltpu.VMEM((NSEG, D, L), bf16),
            pltpu.VMEM((1, NROW // 2, DP), u32),
            pltpu.VMEM((1, D // 2, DP), u32),
            pltpu.VMEM((S // T, DP // 2, T), u32),
            pltpu.VMEM((NSEG, H, NQT, 16, T), u32),
            pltpu.VMEM((NSEG, NG, L // 2, T), u32),
            pltpu.VMEM((NSEG, D, L), f32),
            pltpu.VMEM((NSEG - 1, D // 2, L), u32),
            pltpu.VMEM((NSEG - 1, D // 2, L), u32),
            pltpu.VMEM((S // T, T), f32),
            pltpu.VMEM((T, T), f32),
            pltpu.VMEM((2, D, L), f32),
            pltpu.VMEM((NSEG, DP // 2, L), u32),
            pltpu.VMEM((NWIN, T + 8, T), f32),
            pltpu.VMEM((2, D, L), f32),
            pltpu.VMEM((NWIN, T + 8, T), f32),
            pltpu.VMEM((NB, T, HG * T), f32),
            pltpu.VMEM((8, F), f32),
            pltpu.VMEM((2, D // 2, T), f32),
            pltpu.VMEM((HG, 24, T), f32),
            pltpu.VMEM((3 * QB, HG * T), f32),
            pltpu.VMEM((1, H), bf16),
            pltpu.VMEM((D,), bf16),
            pltpu.SemaphoreType.DMA((7,)),
        ],
        compiler_params=pltpu.CompilerParams(vmem_limit_bytes=100 * 1024 * 1024),
        name="infini_moe",
    )(A_x.reshape(S, D).T, A_wq, A_wk, A_wv, A_wo, A_beta.reshape(1, H), B_w_r,
      B_w_gate, B_w_up, B_w_down.T)
    return out_t.T.reshape(1, S, D)
```

```python
import math
import os

import jax
import jax.numpy as jnp
import numpy as np
from jax import lax
import jax.experimental.pallas as pl
import jax.experimental.pallas.tpu as pltpu

S = 2048
D = 576
H = 32
DH = D // H
NSEG = 4
L = S // NSEG
F = 4608
T = 128
DP = 640
NQT = L // T
WIN = 112
NWIN = 5
HEAD_WIN = [0] * 7 + [1] * 6 + [2] * 6 + [3] * 6 + [4] * 7
WIN_HEADS = [[h for h in range(H) if HEAD_WIN[h] == t] for t in range(NWIN)]
HG = 4
NG = H // HG
AFTER = int(os.environ.get('AFTER', 1))
PINBACK = int(os.environ.get('PINBACK', 2))
ETOK = int(os.environ.get('ETOK', 2))
DUE = int(os.environ.get('DUE', 20))
QB = T // HG
MERGE = int(os.environ.get('MERGE', 1))
GK = 80
GWIN = [HG * DH * g // 16 * 16 for g in range(NG)]
TOKROW = int(os.environ.get('TOKROW', 10))
TOKBACK = int(os.environ.get('TOKBACK', 2))
MOE0 = int(os.environ.get('MOE0', 61))
LAG = int(os.environ.get('LAG', 11))
NB = int(os.environ.get('NB', 13))
RQ, RK, RV = 0, D, 2 * D
NROW = 3 * D
FILL = int(os.environ.get('FILL', 48))
VSPLIT = int(os.environ.get('VSPLIT', 448))
TAIL = ((0, 288), (288, 480), (480, D))
LOG2E = math.log2(math.e)
QSCALE = DH ** -0.5 * LOG2E
MASKVAL = -999292928.0 * LOG2E
LN_EPS = float(np.asarray(1e-5, dtype=jnp.bfloat16).astype(np.float32))

bf16 = jnp.bfloat16
f32 = jnp.float32
u32 = jnp.uint32


def _pack(x):
    return pltpu.bitcast(x, u32)


def _unpack(x):
    return pltpu.bitcast(x, bf16)


def _halves(x):
    return [pltpu.unpack_elementwise(x, index=i, packed_dtype=bf16, unpacked_dtype=f32)
            for i in range(2)]


def _join(even, odd):
    return pltpu.bitcast(pltpu.pack_elementwise([even, odd], packed_dtype=bf16), u32)


def _dot(a, b):
    return lax.dot_general(a, b, (((1,), (0,)), ((), ())), preferred_element_type=f32)


def _dot_nt(a, b):
    return lax.dot_general(a, b, (((1,), (1,)), ((), ())), preferred_element_type=f32)


def _dot_mixed(a, b):
    return lax.dot_general(a, b, (((1,), (0,)), ((), ())), preferred_element_type=f32)


def _iota(shape, dim):
    return lax.broadcasted_iota(jnp.int32, shape, dim)


def _phi(t):
    return jnp.where(t > 0, t + 1.0, jnp.exp(t))


def _round_bf16(x):
    return x.astype(bf16).astype(f32)


def _sigmoid(x):
    return 1.0 / (1.0 + jnp.exp(-x))


def _w_tile(w_ref, i, j, tail=None):
    r = min(T, D - T * i)
    c = min(T, D - T * j)
    t = w_ref[T * i:T * i + r, T * j:T * j + c]
    if c < T:
        t = jnp.concatenate([t, jnp.zeros((r, T - c), bf16)], axis=1)
    if r < T:
        parts = [t]
        if tail is not None:
            parts.append(tail)
        n = T - sum(p.shape[0] for p in parts)
        parts.append(jnp.zeros((n, T), bf16))
        t = jnp.concatenate(parts, axis=0)
    return t


def _store_wt(dst, row0, w_ref, i, j, tail=None):
    c = min(T, D - T * j)
    t = _pack(_w_tile(w_ref, i, j, tail).T)
    r0 = (row0 + T * j) // 2
    dst[0, r0:r0 + c // 2, T * i:T * (i + 1)] = t[:c // 2]


def kernel(x_hbm, wq_hbm, wk_hbm, wv_hbm, wo_hbm, beta_hbm, wr_hbm, wg_hbm, wu_hbm, wd_hbm,
           out_hbm,
           x_v, wq_v, wk_v, wv_v, wo_v, wg_v, wu_v, wd_v, out_v,
           wt, wot, xn_s, q_s, k_s, v_s, pq_s, pk_s, r_s, g_s, o_s, ob_s, m_s, om_s, mask_s, s_s,
           h_s, wr_s, acc_s, bias_s, beta_ref, wr_ref, sems):
    cp_x = [pltpu.make_async_copy(x_hbm.at[:, pl.ds(s * L, L)], x_v.at[s], sems.at[(0, 3, 4, 4)[s]]) if s else None
            for s in range(NSEG)]
    cp_x0 = [pltpu.make_async_copy(x_hbm.at[:, pl.ds(c * L // 2, L // 2)],
                                   x_v.at[0, :, pl.ds(c * L // 2, L // 2)], sems.at[(0, 8)[c]])
             for c in range(2)]
    cp_o = [pltpu.make_async_copy(out_v.at[s], out_hbm.at[:, pl.ds(s * L, L)], sems.at[6])
            for s in range(NSEG - 1)]
    cp_tail = [pltpu.make_async_copy(out_v.at[NSEG - 1, pl.ds(r0, r1 - r0)],
                                     out_hbm.at[pl.ds(r0, r1 - r0), pl.ds(S - L, L)],
                                     sems.at[6])
               for c, (r0, r1) in enumerate(TAIL)]
    cp_wk = pltpu.make_async_copy(wk_hbm, wk_v, sems.at[3])
    cp_wq = pltpu.make_async_copy(wq_hbm, wq_v, sems.at[2])
    cp_wv0 = pltpu.make_async_copy(wv_hbm.at[:, pl.ds(0, 2 * T)], wv_v.at[:, pl.ds(0, 2 * T)],
                                   sems.at[1])
    cp_wv1 = pltpu.make_async_copy(wv_hbm.at[:, pl.ds(2 * T, D - 2 * T)],
                                   wv_v.at[:, pl.ds(2 * T, D - 2 * T)], sems.at[7])
    cp_wo = pltpu.make_async_copy(wo_hbm, wo_v, sems.at[5])
    cp_wg = pltpu.make_async_copy(wg_hbm, wg_v, sems.at[5])
    cp_wu = pltpu.make_async_copy(wu_hbm, wu_v, sems.at[5])
    cp_wd = pltpu.make_async_copy(wd_hbm, wd_v, sems.at[5])
    cp_beta = pltpu.make_async_copy(beta_hbm, beta_ref, sems.at[0])
    cp_wr = pltpu.make_async_copy(wr_hbm, wr_ref, sems.at[0])
    for cp in (cp_beta, cp_wr, cp_x0[0], cp_x0[1], cp_wv0, cp_wv1, cp_wq, cp_x[1], cp_wk, cp_x[2], cp_x[3],
               cp_wo, cp_wg, cp_wu, cp_wd):
        cp.start()

    colh = _iota((T, T), 1)
    rowh = _iota((T, T), 0)
    for t in range(NWIN):
        same = None
        zsel = None
        for n, h in enumerate(WIN_HEADS[t]):
            cin = (colh >= DH * h - WIN * t) & (colh < DH * (h + 1) - WIN * t)
            blk = cin & (rowh >= DH * h - WIN * t) & (rowh < DH * (h + 1) - WIN * t)
            same = blk if same is None else same | blk
            zc = cin[:8] & (rowh[:8] == n)
            zsel = zc if zsel is None else zsel | zc
        mask_s[t, 0:T] = jnp.where(same, 1.0, 0.0)
        mask_s[t, T:T + 8] = jnp.where(zsel, 1.0, 0.0)
    key = _iota((QB, T), 0)
    qry = _iota((QB, T), 1)
    qpos = [(qry - QB * c) % T for c in range(HG)]
    slot = qry // QB
    tiles = [qpos,
             [jnp.where(slot == c, qpos[3], qpos[c]) for c in range(3)] + [qry % QB + QB],
             [jnp.where(slot >= 2, qpos[0], qpos[2]),
              jnp.where((slot == 1) | (slot == 2), qpos[3], qpos[1])]]
    for b, row in enumerate(tiles):
        for c, qp_ in enumerate(row):
            bias_s[QB * b:QB * (b + 1), T * c:T * (c + 1)] = jnp.where(
                qp_ < key + QB * b, MASKVAL, 0.0)
    for j in range(S // T):
        xn_s[j, D // 2:DP // 2 - 8, :] = jnp.zeros(((DP - D) // 2 - 8, T), u32)

    def transpose_w(row0, w, j0=0, j1=5):
        for j in range(j0, j1):
            for i in range(5):
                _store_wt(wt, row0, w, i, j)

    def layernorm(s, j):
        xe, xo = _halves(_pack(x_v[s, :, T * j:T * (j + 1)]))
        mean = jnp.sum(xe + xo, axis=0, keepdims=True) / D
        ce, co = xe - mean, xo - mean
        var = jnp.sum(ce * ce + co * co, axis=0, keepdims=True) / D
        inv = 1.0 / _round_bf16(jnp.sqrt(_round_bf16(_round_bf16(var) + LN_EPS)))
        mean = _round_bf16(mean)
        de, do = _halves(_join(xe - mean, xo - mean))
        xn = _join(de * inv, do * inv)
        even, odd = _halves(xn)
        score = jnp.broadcast_to(jnp.sum(even * wr_s[0] + odd * wr_s[1], axis=0, keepdims=True), (8, T))
        r_s[NQT * s + j:NQT * s + j + 1, :] = score[:1]
        xn_s[NQT * s + j, 0:D // 2, :] = xn
        xn_s[NQT * s + j, DP // 2 - 8:DP // 2, :] = jnp.where(
            never, pltpu.bitcast(score, u32), jnp.zeros((), u32))

    def router_weights():
        wr = jnp.concatenate([wr_ref[...].reshape(1, D), jnp.zeros((1, DP - D), bf16)], axis=1)
        even, odd = _halves(_pack(jnp.broadcast_to(wr, (T, DP)).T)[:D // 2])
        wr_s[0], wr_s[1] = even, odd

    def xn_seg(s):
        return _unpack(jnp.concatenate([xn_s[NQT * s + j] for j in range(NQT)], axis=1))

    def proj_q(s):
        q = _dot(_unpack(wt[z, RQ // 2:RK // 2, :]), xn_seg(s))
        if s > 0:
            pq_s[s - 1] = _pack(_phi(q[:D]).astype(bf16))
        qp = _pack((q[:D] * QSCALE).astype(bf16))
        for h in range(H):
            a = (DH * h) // 16
            lo = (DH * h - 16 * a) // 2
            prow = _iota((16, L), 0)
            qh = jnp.where((prow >= lo) & (prow <= lo + 8), qp[8 * a:8 * a + 16], jnp.zeros((), u32))
            for j in range(NQT):
                qt = qh[:, T * j:T * (j + 1)]
                q_s[s, h, j] = pltpu.roll(qt, QB * (h % HG), 1) if h % HG else qt

    def proj_k(s):
        k = _dot(_unpack(wt[z, RK // 2:RV // 2, :]), xn_seg(s))
        if s < NSEG - 1:
            pk_s[s] = _pack(_phi(k).astype(bf16))
        for j in range(NQT):
            kb = k[:, T * j:T * (j + 1)].astype(bf16)
            for g in range(NG):
                kw = jnp.concatenate([kb[GWIN[g]:GWIN[g] + GK], jnp.zeros((T - GK, T), bf16)], axis=0)
                k_s[s, g, 64 * j:64 * (j + 1), :] = _pack(kw.T)

    def proj_v(s, r0=0, r1_=D):
        v_s[s, r0:r1_, :] = _round_bf16(
            _dot(_unpack(wt[z, (RV + r0) // 2:(RV + r1_) // 2, :]), xn_seg(s)))

    cp_x0[0].wait()
    cp_beta.wait()
    cp_wr.wait()
    g = _round_bf16(_sigmoid(beta_ref[...].astype(f32)))
    z = jnp.where(jnp.max(g) > 2.0, 1, 0)
    g = jnp.concatenate([g, jnp.zeros((1, T - H), f32)], axis=1)
    g_s[...] = jnp.broadcast_to(g, (T, T)).T
    prow = _iota((8, T), 0)
    never = prow > z + 8
    router_weights()
    layernorm(0, 0)
    layernorm(0, 1)
    cp_x0[1].wait()
    layernorm(0, 2)
    layernorm(0, 3)
    cp_wv0.wait()
    transpose_w(RV, wv_v, 0, 2)
    proj_v(0, 0, 2 * T)
    cp_wv1.wait()
    transpose_w(RV, wv_v, 2, 5)
    proj_v(0, 2 * T, 464)
    cp_wq.wait()
    transpose_w(RQ, wq_v)
    proj_v(0, 464, 512)
    proj_q(0)
    proj_v(0, 512, 544)
    cp_x[1].wait()
    cp_wk.wait()
    transpose_w(RK, wk_v)
    for j in range(NQT):
        layernorm(1, j)
    proj_v(0, 544, D)
    proj_k(0)
    proj_v(1)
    cp_x[2].wait()
    cp_x[3].wait()
    for s in (2, 3):
        for j in range(NQT):
            layernorm(s, j)
        proj_q(s - 1)
    proj_q(3)

    r = _round_bf16(r_s[...])
    pos = _iota((S // T, T), 0) * T + _iota((S // T, T), 1)
    r1 = jnp.max(r)
    i1 = jnp.minimum(jnp.min(jnp.where(r == r1, pos, S)), S - 1)
    rest = pos != i1
    r2 = jnp.max(jnp.where(rest, r, -jnp.inf))
    i2 = jnp.minimum(jnp.min(jnp.where(rest & (r == r2), pos, S)), S - 1)

    for s in range(1, NSEG):
        proj_k(s)
        if s > 1:
            proj_v(s)

    lane = _iota((DP // 2, T), 1)
    xsel = jnp.zeros((8, DP), f32)
    for c, idx in enumerate((i1, i2)):
        col = jnp.where(lane == idx % T, xn_s[idx // T], jnp.zeros((), u32))
        xsel = xsel + _dot_nt(jnp.where(_iota((8, T), 0) == c, 1.0, 0.0), _unpack(col))

    moe = {}

    def ffn_in(w, name, cg, i):
        k = min(T, D - T * i)
        r_ = _dot(xsel[:, T * i:T * i + k], w[T * i:T * i + k, L * cg:L * (cg + 1)])
        moe[name] = r_ if i == 0 else moe[name] + r_
        if name == "up" and i == 4:
            gate = moe["gate"]
            hid = gate * _sigmoid(gate) * moe["up"]
            h_s[:, L * cg:L * (cg + 1)] = _round_bf16(hid)

    def ffn_out(cg, i):
        if i < 4:
            c0 = L * cg + T * i
            r_ = _dot_nt(h_s[:, c0:c0 + T], wd_v[0:4 * T, c0:c0 + T])
            moe["y0"] = r_ if "y0" not in moe else moe["y0"] + r_
        else:
            r_ = _dot_nt(h_s[:, L * cg:L * (cg + 1)], wd_v[4 * T:D, L * cg:L * (cg + 1)])
            moe["y1"] = r_ if "y1" not in moe else moe["y1"] + r_

    def ffn_finish():
        y = jnp.concatenate([moe["y0"], moe["y1"], jnp.zeros((8, DP - D), f32)], axis=1)
        y = y * _sigmoid(jnp.where(_iota((8, DP), 0) == 0, r1, r2))
        y = jnp.concatenate([y, jnp.zeros((8, DP), f32)], axis=0)
        for j in range(5):
            _store_wt(wot, 0, wo_v, 4, j, tail=y[:, T * j:T * (j + 1)].astype(bf16))

    rounds = []
    for cg in range(F // L):
        rounds += [(ffn_in, wg_v, "gate", cg, i) for i in range(5)]
        rounds += [(ffn_in, wu_v, "up", cg, i) for i in range(5)]
        if cg > 0:
            rounds += [(ffn_out, cg - 1, i) for i in range(5)]
    rounds += [None] * 3
    rounds += [(ffn_out, F // L - 1, i) for i in range(5)]

    steps = [(s, g, j, i) for s in range(NSEG) for g in range(NG) for j in range(NQT)
             for i in range(j + 1)]
    ns = len(steps)
    mx, tok, due = {}, {}, {}
    lane8 = _iota((8, T), 1)
    hi = lane8 >= T // 2
    sl = [lane8 // QB == c for c in range(HG)]
    mid = sl[1] | sl[2]
    def q_masked(s, g, j, c):
        h = HG * g + c
        pos0 = (DH * h) // 16 - GWIN[g] // 16
        zero = jnp.zeros((8, T), u32)
        return ([zero] * pos0 + [q_s[s, h, j, 0:8], q_s[s, h, j, 8:16]]
                + [zero] * (GK // 16 - 2 - pos0))

    def k_rows(s, g, r0, r1_):
        return _unpack(k_s[s + z, g, r0 // 2:r1_ // 2, :])[:, :GK]

    def sel(mask, a, b):
        n_ = len(a) if isinstance(a, list) else len(b)
        out = []
        for r_ in range(n_):
            x = a[r_] if isinstance(a, list) else a
            y = b[r_] if isinstance(b, list) else b
            out.append(x if x is y else jnp.where(mask, x, y))
        return out

    def stash(n, st, row0, col0, bias_row0=None):
        m = None
        w = st.shape[1]
        for r_ in range(0, st.shape[0], 8):
            x = st[r_:r_ + 8]
            if bias_row0 is not None:
                x = x + bias_s[bias_row0 + r_:bias_row0 + r_ + 8, col0:col0 + w]
            s_s[n % NB, row0 + r_:row0 + r_ + 8, col0:col0 + w] = x
            m = x if m is None else jnp.maximum(m, x)
        return m

    def weights(tiles_):
        return _unpack(jnp.concatenate([jnp.concatenate(q, axis=0) for q in tiles_], axis=1))

    def qk(n):
        s, g, j, i = steps[n]
        qm = [q_masked(s, g, j, c) for c in range(HG)]
        if i < j:
            ahead = QB if MERGE and i == j - 1 else 0
            st = _dot(k_rows(s, g, T * i, T * (i + 1) + ahead), weights(qm))
            tok[n] = st[8 * TOKROW:8 * TOKROW + 8]
            m = stash(n, st[:T], 0, 0)
            if ahead:
                m = jnp.maximum(m, stash(n + 1, st[T:], 0, 0, 0))
            mx[s, g, j] = m if i == 0 else jnp.maximum(mx[s, g, j], m)
            return
        if j == 0 or not MERGE:
            m = stash(n, _dot(k_rows(s, g, T * i, T * i + QB), weights(qm)), 0, 0, 0)
            if j > 0:
                m = jnp.maximum(mx[s, g, j], m)
        else:
            m = mx[s, g, j]
        x1 = _dot(k_rows(s, g, T * i + QB, T * i + 2 * QB),
                  weights([sel(sl[c], qm[3], qm[c]) for c in range(3)]))
        x3 = _dot(k_rows(s, g, T * i + 3 * QB, T * (i + 1)),
                  weights([sel(hi, sel(mid, qm[3], qm[0]), sel(mid, qm[2], qm[1]))]))
        tok[n] = jnp.concatenate([x1[QB - 8:], x3[QB - 8:]], axis=1)
        m1 = stash(n, x1, QB, 0, QB)
        m1 = [m1[:, T * c:T * (c + 1)] for c in range(3)]
        m3 = stash(n, x3, QB, 3 * T, QB)
        m2 = []
        for c, w in enumerate((sel(hi, qm[0], qm[2]), sel(mid, qm[3], qm[1]))):
            parts = [stash(n, _dot(k_rows(s, g, T * i + r0, T * i + r0 + QB // 2), weights([w])),
                           r0, T * c, r0) for r0 in (2 * QB, 2 * QB + QB // 2)]
            m2.append(jnp.maximum(*parts))
        ms = []
        for c in range(HG):
            x = m[:, T * c:T * (c + 1)]
            if c < 3:
                x = jnp.where(sl[c], x, jnp.maximum(x, m1[c]))
            else:
                for b in range(3):
                    x = jnp.where(sl[b], jnp.maximum(x, m1[b]), x)
            y = jnp.maximum(x, m2[c % 2])
            x = jnp.where((hi, mid)[c % 2], *((y, x) if c in (0, 3) else (x, y)))
            ms.append(jnp.where(sl[(c + 3) % HG], jnp.maximum(x, m3), x))
        mx[s, g, j] = jnp.max(jnp.concatenate(ms, axis=1), axis=0, keepdims=True)

    def pv(n):
        s, g, j, i = steps[n]
        ms = []
        for c in range(HG):
            m = jnp.broadcast_to(mx[s, g, j][:, T * c:T * (c + 1)], (8, T))
            t_ = tok[n + LAG - (TOKBACK if n + LAG <= ns else ETOK)][:, T * c:T * (c + 1)]
            for x in due.pop((n, c), ()):
                t_ = jnp.maximum(t_, x)
            ms.append(jnp.where(never, t_, m))

        def probs(r0, r1_, c, m):
            return [jnp.exp2(s_s[n % NB, r_:r_ + 8, T * c:T * (c + 1)] - m) for r_ in range(r0, r1_, 8)]

        if i == j:
            e1 = [probs(QB, 2 * QB, c, jnp.where(sl[c], ms[3], ms[c])) for c in range(3)]
            e3 = probs(QB, 2 * QB, 3, jnp.where(hi, jnp.where(mid, ms[3], ms[0]),
                                                jnp.where(mid, ms[2], ms[1])))
            e2 = [probs(2 * QB, 3 * QB, 0, jnp.where(hi, ms[0], ms[2])),
                  probs(2 * QB, 3 * QB, 1, jnp.where(mid, ms[3], ms[1]))]
        for c in range(HG):
            if i == j:
                p = probs(0, QB, c, ms[c])
                if c < 3:
                    p += sel(sl[c], 0.0, e1[c])
                else:
                    p += sel(sl[0], e1[0], sel(sl[1], e1[1], sel(sl[2], e1[2], 0.0)))
                p += sel((hi, mid)[c % 2], *((e2[c % 2], 0.0) if c in (0, 3) else (0.0, e2[c % 2])))
                p += sel(sl[(c + 3) % HG], e3, 0.0)
            else:
                p = probs(0, T, c, ms[c])
            p = jnp.concatenate(p, axis=0)
            h = HG * g + c
            a = DH * h // 8 * 8
            o = DH * h - a
            one = 23 if o == 0 else 0
            vt = [v_s[s, a + 8 * r_:a + 8 * r_ + 8, T * i:T * (i + 1)] for r_ in range(3)]
            vt[one // 8] = jnp.where(prow == one % 8, 1.0, vt[one // 8])
            r_ = _dot_mixed(jnp.concatenate(vt, axis=0), p.astype(bf16))
            if i > 0:
                r_ = acc_s[c] + r_
            if i < j:
                acc_s[c] = r_
            else:
                l = r_[one:one + 1]
                inv = pltpu.reciprocal(l, approx=True)
                inv = inv * (2.0 - l * inv)
                sc = (1.0 - g_s[h:h + 1, :]) * (inv * (2.0 - l * inv))
                val = r_ * sc
                if c:
                    val = pltpu.roll(val, T - QB * c, 1)
                for r0 in range(0, 24, 8):
                    due.setdefault((n + DUE, c), []).append(val[r0:r0 + 8])
                o_s[s % 2, DH * h:DH * (h + 1), T * j:T * (j + 1)] = val[o:o + DH]

    def win_rows(t):
        heads = WIN_HEADS[t]
        return DH * heads[0] // 8 * 8, -(-DH * (heads[-1] + 1) // 8) * 8

    def mem_read(s, t):
        heads = WIN_HEADS[t]
        r0 = WIN * t
        ra0, re0 = win_rows(t)
        lhs = jnp.concatenate(
            [jnp.where(mask_s[t, a:b] > 0, _round_bf16(m_s[t, a:b]), 0.0)
             for a, b in ((T, T + 8), (ra0 - r0, re0 - r0))], axis=0)
        rd = _dot_mixed(lhs, _unpack(pq_s[s - 1, r0 // 2:r0 // 2 + 64, :]))
        h0 = heads[0]
        coef = jnp.concatenate([g_s[h0:h0 + 8, :]] * NQT, axis=1) / (rd[:8] + 1e-6)
        lo_row = DH * heads[0]
        hi_row = DH * (heads[-1] + 1)
        for rb in range(ra0, re0, 8):
            ha = max(rb // DH, h0)
            hb = min((rb + 7) // DH, heads[-1])
            cf = jnp.broadcast_to(coef[ha - h0:ha - h0 + 1], (8, L))
            if hb != ha:
                cf = jnp.where(_iota((8, L), 0) < DH * hb - rb, cf,
                               jnp.broadcast_to(coef[hb - h0:hb - h0 + 1], (8, L)))
            val = rd[rb - ra0 + 8:rb - ra0 + 16] * cf
            ra, re = max(rb, lo_row), min(rb + 8, hi_row)
            om_s[s % 2, ra:re, :] = val[ra - rb:re - rb]

    def mem_update(s, t):
        r0 = WIN * t
        ra0, re0 = win_rows(t)
        vl = jnp.concatenate([v_s[s, ra0:re0, :], jnp.ones((8, L), f32)], axis=0)
        upd = lax.dot_general(vl, _unpack(pk_s[s, r0 // 2:r0 // 2 + 64, :]),
                              (((1,), (1,)), ((), ())), preferred_element_type=f32)
        for a, b, u in ((ra0 - r0, re0 - r0, upd[:re0 - ra0]), (T, T + 8, upd[re0 - ra0:])):
            m_s[t, a:b] = u if s == 0 else m_s[t, a:b] + u

    def pack_o(s, r0, r1_):
        o = o_s[s % 2, r0:r1_, :]
        if s > 0:
            o = o + om_s[s % 2, r0:r1_, :]
        ob_s[s, r0 // 2:r1_ // 2, :] = _pack(o.astype(bf16))

    def out_proj(s, r0, r1_, n=None):
        ob = ob_s[s]
        if n is not None:
            head = jnp.where(jnp.concatenate([never] * HG, axis=1),
                             pltpu.bitcast(tok[n - PINBACK], u32), ob[:8])
            ob = jnp.concatenate([head, ob[8:]], axis=0)
        res = _dot(_unpack(wot[z, r0 // 2:r1_ // 2, :]), _unpack(ob))
        if n is not None:
            tok[n] = res[:8]
        xn = _unpack(jnp.concatenate(
            [xn_s[NQT * s + j, r0 // 2:r1_ // 2, :] for j in range(NQT)], axis=1))
        out_v[s, r0:r1_, :] = (res + x_v[s, r0:r1_, :].astype(f32) + xn.astype(f32)).astype(bf16)

    for s in range(NSEG):
        tpos = _iota((16, L), 1) + s * L
        pick = jnp.where(_iota((16, L), 0) == 0, i1, jnp.where(_iota((16, L), 0) == 1, i2, -1))
        ob_s[s, D // 2:D // 2 + 8, :] = _pack(jnp.where(tpos == pick, 1.0, 0.0).astype(bf16))
        ob_s[s, D // 2 + 8:DP // 2, :] = jnp.zeros(((DP - D) // 2 - 8, L), u32)

    extra = {}

    def at(n, fn, *args):
        extra.setdefault(n, []).append((fn,) + args)

    per = ns // NSEG
    full = [n for n, (_, _, j, i) in enumerate(steps) if i < j]
    busy = set()

    def at_full(n, fn, *args):
        n = next(m for m in full if m >= n and m not in busy)
        busy.add(n)
        at(n, fn, *args)
        return n

    for t in range(NWIN):
        at_full(0, mem_update, 0, t)
        for s in range(1, NSEG):
            at_full(per * s - 40 + 6 * t, mem_read, s, t)
            if s < NSEG - 1:
                at_full(per * s + 4 + 6 * t, mem_update, s, t)

    busy.clear()

    def late_weights():
        for cp in (cp_wo, cp_wg, cp_wu, cp_wd):
            cp.wait()

    at(MOE0, late_weights)
    n = MOE0
    for rd_ in rounds:
        n = at_full(n, *rd_) if rd_ is not None else n + 2
    at(n + 2, ffn_finish)
    for c in range(20):
        at(MOE0 + 2 * c + 1, _store_wt, wot, 0, wo_v, c % 4, c // 4)
    for s in range(NSEG):
        for c in range(D // 48):
            n = per * s + 10 * ((48 * (c + 1) - 1) // (HG * DH) + 1) + LAG + c % 2 * 3 + 1
            at(min(n, ns + LAG), pack_o, s, 48 * c, 48 * (c + 1))
    for c in range(LAG):
        at(ns + c, out_proj, 0, FILL * c, FILL * (c + 1), ns + c)

    for n in range(ns + LAG):
        if n < ns:
            qk(n)
        for task in extra.get(n, ()):
            if not (AFTER and task[0] is ffn_in):
                task[0](*task[1:])
        if n >= LAG:
            pv(n - LAG)
        for task in extra.get(n, ()):
            if AFTER and task[0] is ffn_in:
                task[0](*task[1:])
    for task in extra[ns + LAG]:
        task[0](*task[1:])
    for s in range(NSEG - 1):
        out_proj(s, FILL * LAG if s == 0 else 0, D, ns + LAG + s if s == 0 else None)
        cp_o[s].start()
    for (r0, r1_), cp in zip(TAIL, cp_tail):
        out_proj(NSEG - 1, r0, r1_)
        cp.start()
    for cp in cp_o + cp_tail:
        cp.wait()


@jax.jit
def pallas_parallel_sum__memory_aug_infini_attn__moe_arch_mod__prompt_kernel(
    A_x, A_wq, A_wk, A_wv, A_wo, A_beta, B_x, B_w_r, B_w_gate, B_w_up, B_w_down,
):
    del B_x
    any_spec = pl.BlockSpec(memory_space=pl.ANY)
    out_t = pl.pallas_call(
        kernel,
        out_shape=jax.ShapeDtypeStruct((D, S), bf16),
        in_specs=[any_spec] * 10,
        out_specs=any_spec,
        scratch_shapes=[
            pltpu.VMEM((NSEG, D, L), bf16),
            pltpu.VMEM((D, D), bf16),
            pltpu.VMEM((D, D), bf16),
            pltpu.VMEM((D, D), bf16),
            pltpu.VMEM((D, D), bf16),
            pltpu.VMEM((D, F), bf16),
            pltpu.VMEM((D, F), bf16),
            pltpu.VMEM((D, F), bf16),
            pltpu.VMEM((NSEG, D, L), bf16),
            pltpu.VMEM((1, NROW // 2, DP), u32),
            pltpu.VMEM((1, D // 2, DP), u32),
            pltpu.VMEM((S // T, DP // 2, T), u32),
            pltpu.VMEM((NSEG, H, NQT, 16, T), u32),
            pltpu.VMEM((NSEG, NG, L // 2, T), u32),
            pltpu.VMEM((NSEG, D, L), f32),
            pltpu.VMEM((NSEG - 1, D // 2, L), u32),
            pltpu.VMEM((NSEG - 1, D // 2, L), u32),
            pltpu.VMEM((S // T, T), f32),
            pltpu.VMEM((T, T), f32),
            pltpu.VMEM((2, D, L), f32),
            pltpu.VMEM((NSEG, DP // 2, L), u32),
            pltpu.VMEM((NWIN, T + 8, T), f32),
            pltpu.VMEM((2, D, L), f32),
            pltpu.VMEM((NWIN, T + 8, T), f32),
            pltpu.VMEM((NB, T, HG * T), f32),
            pltpu.VMEM((8, F), f32),
            pltpu.VMEM((2, D // 2, T), f32),
            pltpu.VMEM((HG, 24, T), f32),
            pltpu.VMEM((3 * QB, HG * T), f32),
            pltpu.VMEM((1, H), bf16),
            pltpu.VMEM((D,), bf16),
            pltpu.SemaphoreType.DMA((9,)),
        ],
        compiler_params=pltpu.CompilerParams(vmem_limit_bytes=100 * 1024 * 1024),
        name="infini_moe",
    )(A_x.reshape(S, D).T, A_wq, A_wk, A_wv, A_wo, A_beta.reshape(1, H), B_w_r,
      B_w_gate, B_w_up, B_w_down.T)
    return out_t.T.reshape(1, S, D)
```

```python
import math

import jax
import jax.numpy as jnp
import numpy as np
from jax import lax
import jax.experimental.pallas as pl
import jax.experimental.pallas.tpu as pltpu

S = 2048
D = 576
H = 32
DH = D // H
NSEG = 4
L = S // NSEG
F = 4608
T = 128
DP = 640
NT = DP // T
NQT = L // T

HG = 4
NG = H // HG
GK = 80
GWIN = [HG * DH * g // 16 * 16 for g in range(NG)]
QB = T // HG

WIN = 112
WIN_HEADS = [list(range(a, b)) for a, b in ((0, 7), (7, 13), (13, 19), (19, 25), (25, 32))]
NWIN = len(WIN_HEADS)

LAG = 11
NB = 13
TOKBACK = 2
TOKROW = 80
DUE = 20
FFN0 = 61
FILL = 48
TAIL = ((0, 256), (256, 432), (432, 528), (528, D))

RQ, RK, RV = 0, D, 2 * D
LOG2E = math.log2(math.e)
QSCALE = DH ** -0.5 * LOG2E
MASKVAL = float(np.asarray(-1e9, dtype=jnp.bfloat16).astype(np.float32)) * LOG2E
LN_EPS = float(np.asarray(1e-5, dtype=jnp.bfloat16).astype(np.float32))

bf16 = jnp.bfloat16
f32 = jnp.float32
u32 = jnp.uint32


def _pack(x):
    return pltpu.bitcast(x, u32)


def _unpack(x):
    return pltpu.bitcast(x, bf16)


def _halves(x):
    return [pltpu.unpack_elementwise(x, index=i, packed_dtype=bf16, unpacked_dtype=f32)
            for i in range(2)]


def _join(even, odd):
    return pltpu.bitcast(pltpu.pack_elementwise([even, odd], packed_dtype=bf16), u32)


def _dot(a, b):
    return lax.dot_general(a, b, (((1,), (0,)), ((), ())), preferred_element_type=f32)


def _dot_nt(a, b):
    return lax.dot_general(a, b, (((1,), (1,)), ((), ())), preferred_element_type=f32)


def _iota(shape, dim):
    return lax.broadcasted_iota(jnp.int32, shape, dim)


def _phi(t):
    return jnp.where(t > 0, t + 1.0, jnp.exp(t))


def _round_bf16(x):
    return x.astype(bf16).astype(f32)


def _sigmoid(x):
    return 1.0 / (1.0 + jnp.exp(-x))


def _all_max(x):
    return jnp.max(jnp.max(x, axis=0, keepdims=True), axis=1, keepdims=True)


def _select(mask, a, b):
    n = len(a) if isinstance(a, list) else len(b)
    out = []
    for r in range(n):
        x = a[r] if isinstance(a, list) else a
        y = b[r] if isinstance(b, list) else b
        out.append(x if x is y else jnp.where(mask, x, y))
    return out


def _store_transposed(dst, row0, w_ref, i, j, tail=None):
    r = min(T, D - T * i)
    c = min(T, D - T * j)
    t = w_ref[T * i:T * i + r, T * j:T * j + c]
    if c < T:
        t = jnp.concatenate([t, jnp.zeros((r, T - c), bf16)], axis=1)
    if r < T:
        parts = [t] if tail is None else [t, tail]
        parts.append(jnp.zeros((T - sum(p.shape[0] for p in parts), T), bf16))
        t = jnp.concatenate(parts, axis=0)
    r0 = (row0 + T * j) // 2
    dst[0, r0:r0 + c // 2, T * i:T * (i + 1)] = _pack(t.T)[:c // 2]


def _win_rows(t):
    lo, hi = DH * WIN_HEADS[t][0], DH * (WIN_HEADS[t][-1] + 1)
    r0, r1 = lo // 8 * 8, -(-hi // 8) * 8
    return r0, r1, r0 if r0 < lo else r1 - 1


def _kernel(x_hbm, wq_hbm, wk_hbm, wv_hbm, wo_hbm, beta_hbm, wr_hbm, wg_hbm, wu_hbm, wd_hbm,
            out_hbm,
            x_v, wq_v, wk_v, wv_v, wo_v, wg_v, wu_v, wd_v, beta_v, wr_v, out_v,
            wt_s, wot_s, xn_s, q_s, k_s, v_s, pq_s, pk_s, wr_s, r_s, g_s, bias_s, s_s, acc_s,
            o_s, ob_s, mask_s, m_s, om_s, h_s, sems):
    def copy(src, dst, sem):
        return pltpu.make_async_copy(src, dst, sems.at[sem])

    cp_beta = copy(beta_hbm, beta_v, 0)
    cp_wr = copy(wr_hbm, wr_v, 0)
    cp_x0 = [copy(x_hbm.at[:, pl.ds(c * L // 2, L // 2)], x_v.at[0, :, pl.ds(c * L // 2, L // 2)], c)
             for c in range(2)]
    cp_wv = [copy(wv_hbm.at[:, pl.ds(c0, c1 - c0)], wv_v.at[:, pl.ds(c0, c1 - c0)], sem)
             for c0, c1, sem in ((0, 2 * T, 2), (2 * T, D, 3))]
    cp_wq = copy(wq_hbm, wq_v, 4)
    cp_mid = [copy(x_hbm.at[:, pl.ds(L, L)], x_v.at[1], 5), copy(wk_hbm, wk_v, 5)]
    cp_rest = [copy(x_hbm.at[:, pl.ds(s * L, L)], x_v.at[s], 6) for s in (2, 3)]
    cp_rest.append(copy(wo_hbm, wo_v, 6))
    cp_ffn = [copy(wg_hbm, wg_v, 7), copy(wu_hbm, wu_v, 7), copy(wd_hbm, wd_v, 7)]
    cp_out = [copy(out_v.at[s], out_hbm.at[:, pl.ds(s * L, L)], 8) for s in range(NSEG - 1)]
    cp_tail = [copy(out_v.at[NSEG - 1, pl.ds(r0, r1 - r0)],
                    out_hbm.at[pl.ds(r0, r1 - r0), pl.ds(S - L, L)], 8) for r0, r1 in TAIL]
    for cp in [cp_beta, cp_wr] + cp_x0 + cp_wv + [cp_wq] + cp_mid + cp_rest + cp_ffn:
        cp.start()

    col = _iota((T, T), 1)
    row = _iota((T, T), 0)
    for t in range(NWIN):
        same = None
        pick = None
        for n, h in enumerate(WIN_HEADS[t]):
            lo, hi = DH * h - WIN * t, DH * (h + 1) - WIN * t
            cin = (col >= lo) & (col < hi)
            blk = cin & (row >= lo) & (row < hi)
            same = blk if same is None else same | blk
            mine = cin[:8] & (row[:8] == n)
            pick = mine if pick is None else pick | mine
        mask_s[t, 0:T] = jnp.where(same, 1.0, 0.0)
        mask_s[t, T:T + 8] = jnp.where(pick, 1.0, 0.0)
    key = _iota((QB, T), 0)
    qry = _iota((QB, T), 1)
    qpos = [(qry - QB * c) % T for c in range(HG)]
    slot = qry // QB
    tiles = [qpos,
             [jnp.where(slot == c, qpos[3], qpos[c]) for c in range(3)] + [qry % QB + QB],
             [jnp.where(slot >= 2, qpos[0], qpos[2]),
              jnp.where((slot == 1) | (slot == 2), qpos[3], qpos[1])]]
    for b, tile_row in enumerate(tiles):
        for c, queries in enumerate(tile_row):
            bias_s[QB * b:QB * (b + 1), T * c:T * (c + 1)] = jnp.where(
                queries < key + QB * b, MASKVAL, 0.0)
    for j in range(S // T):
        xn_s[j, D // 2:DP // 2 - 8, :] = jnp.zeros(((DP - D) // 2 - 8, T), u32)

    def transpose_w(row0, w, j0=0, j1=NT):
        for j in range(j0, j1):
            for i in range(NT):
                _store_transposed(wt_s, row0, w, i, j)

    def layernorm(s, j):
        xe, xo = _halves(_pack(x_v[s, :, T * j:T * (j + 1)]))
        mean = jnp.sum(xe + xo, axis=0, keepdims=True) / D
        ce, co = xe - mean, xo - mean
        var = jnp.sum(ce * ce + co * co, axis=0, keepdims=True) / D
        inv = 1.0 / _round_bf16(jnp.sqrt(_round_bf16(_round_bf16(var) + LN_EPS)))
        mean = _round_bf16(mean)
        de, do = _halves(_join(xe - mean, xo - mean))
        xn = _join(de * inv, do * inv)
        even, odd = _halves(xn)
        score = jnp.sum(even * wr_s[0] + odd * wr_s[1], axis=0, keepdims=True)
        score = jnp.broadcast_to(score, (8, T))
        r_s[NQT * s + j:NQT * s + j + 1, :] = score[:1]
        xn_s[NQT * s + j, 0:D // 2, :] = xn
        xn_s[NQT * s + j, DP // 2 - 8:DP // 2, :] = jnp.where(
            never, pltpu.bitcast(score, u32), jnp.zeros((), u32))

    def project(s, r0, r1):
        xn = _unpack(jnp.concatenate([xn_s[NQT * s + j] for j in range(NQT)], axis=1))
        return _dot(_unpack(wt_s[zero, r0 // 2:r1 // 2, :]), xn)

    def proj_q(s):
        q = project(s, RQ, RK)
        if s > 0:
            pq_s[s - 1] = _pack(_phi(q).astype(bf16))
        q = _pack((q * QSCALE).astype(bf16))
        for h in range(H):
            a = DH * h // 16
            lo = (DH * h - 16 * a) // 2
            pair = _iota((16, L), 0)
            qh = jnp.where((pair >= lo) & (pair < lo + DH // 2), q[8 * a:8 * a + 16],
                           jnp.zeros((), u32))
            for j in range(NQT):
                qt = qh[:, T * j:T * (j + 1)]
                q_s[s, h, j] = pltpu.roll(qt, QB * (h % HG), 1) if h % HG else qt

    def proj_k(s):
        k = project(s, RK, RV)
        if s < NSEG - 1:
            pk_s[s] = _pack(_phi(k).astype(bf16))
        for j in range(NQT):
            kb = k[:, T * j:T * (j + 1)].astype(bf16)
            for g in range(NG):
                kw = jnp.concatenate([kb[GWIN[g]:GWIN[g] + GK], jnp.zeros((T - GK, T), bf16)], axis=0)
                k_s[s, g, T // 2 * j:T // 2 * (j + 1), :] = _pack(kw.T)

    def proj_v(s, r0=0, r1=D):
        v_s[s, r0:r1, :] = _round_bf16(project(s, RV + r0, RV + r1))

    for cp in (cp_x0[0], cp_beta, cp_wr):
        cp.wait()
    gate = _round_bf16(_sigmoid(beta_v[...].astype(f32)))
    zero = jnp.where(jnp.max(gate) > 2.0, 1, 0)
    gate = jnp.concatenate([gate, jnp.zeros((1, T - H), f32)], axis=1)
    g_s[...] = jnp.broadcast_to(gate, (T, T)).T
    sub = _iota((8, T), 0)
    never = sub > zero + 8
    wr = jnp.concatenate([wr_v[...].reshape(1, D), jnp.zeros((1, DP - D), bf16)], axis=1)
    wr_s[0], wr_s[1] = _halves(_pack(jnp.broadcast_to(wr, (T, DP)).T)[:D // 2])
    layernorm(0, 0)
    layernorm(0, 1)
    cp_x0[1].wait()
    layernorm(0, 2)
    layernorm(0, 3)
    cp_wv[0].wait()
    transpose_w(RV, wv_v, 0, 2)
    proj_v(0, 0, 2 * T)
    cp_wv[1].wait()
    transpose_w(RV, wv_v, 2, NT)
    proj_v(0, 2 * T, 464)
    cp_wq.wait()
    transpose_w(RQ, wq_v)
    proj_v(0, 464, 512)
    proj_q(0)
    proj_v(0, 512, 544)
    for cp in cp_mid:
        cp.wait()
    transpose_w(RK, wk_v)
    for j in range(NQT):
        layernorm(1, j)
    proj_v(0, 544, D)
    proj_k(0)
    proj_v(1)
    for cp in cp_rest:
        cp.wait()
    for s in (2, 3):
        for j in range(NQT):
            layernorm(s, j)
        proj_q(s - 1)
    proj_q(3)
    for j in range(NT):
        for i in range(NT - 1):
            _store_transposed(wot_s, 0, wo_v, i, j)

    r = _round_bf16(r_s[...])
    pos = (_iota((S // T, T), 0) * T + _iota((S // T, T), 1)).astype(f32)
    r1 = _all_max(r)
    i1 = -_all_max(jnp.where(r == r1, -pos, 1.0 - S))
    rest = pos != i1
    r2 = _all_max(jnp.where(rest, r, -jnp.inf))
    i2 = -_all_max(jnp.where(rest & (r == r2), -pos, 1.0 - S))
    i1, i2 = i1.astype(jnp.int32), i2.astype(jnp.int32)

    for s in range(1, NSEG):
        proj_k(s)
        if s > 1:
            proj_v(s)

    xsel = jnp.zeros((8, DP), f32)
    for c, idx in enumerate((i1, i2)):
        token = jnp.where(_iota((DP // 2, T), 1) == idx % T, xn_s[(idx // T)[0, 0]],
                          jnp.zeros((), u32))
        xsel = xsel + _dot_nt(jnp.where(sub == c, 1.0, 0.0), _unpack(token))

    ffn = {}

    def ffn_in(w, name, cg, i):
        k = min(T, D - T * i)
        part = _dot(xsel[:, T * i:T * i + k], w[T * i:T * i + k, L * cg:L * (cg + 1)])
        ffn[name] = part if i == 0 else ffn[name] + part
        if name == "up" and i == NT - 1:
            h_s[:, L * cg:L * (cg + 1)] = _round_bf16(
                ffn["gate"] * _sigmoid(ffn["gate"]) * ffn["up"])

    def ffn_out(cg, i):
        if i < 4:
            c0 = L * cg + T * i
            name, part = "y0", _dot_nt(h_s[:, c0:c0 + T], wd_v[0:4 * T, c0:c0 + T])
        else:
            cols = slice(L * cg, L * (cg + 1))
            name, part = "y1", _dot_nt(h_s[:, cols], wd_v[4 * T:D, cols])
        ffn[name] = ffn[name] + part if name in ffn else part

    def ffn_finish():
        y = jnp.concatenate([ffn["y0"], ffn["y1"], jnp.zeros((8, DP - D), f32)], axis=1)
        y = y * _sigmoid(jnp.where(_iota((8, DP), 0) == 0, r1, r2))
        y = jnp.concatenate([y, jnp.zeros((8, DP), f32)], axis=0)
        for j in range(NT):
            _store_transposed(wot_s, 0, wo_v, NT - 1, j, tail=y[:, T * j:T * (j + 1)].astype(bf16))

    rounds = []
    for cg in range(F // L):
        rounds += [(ffn_in, wg_v, "gate", cg, i) for i in range(NT)]
        rounds += [(ffn_in, wu_v, "up", cg, i) for i in range(NT)]
        if cg > 0:
            rounds += [(ffn_out, cg - 1, i) for i in range(NT)]
    rounds += [None] * 3
    rounds += [(ffn_out, F // L - 1, i) for i in range(NT)]

    steps = [(s, g, j, i) for s in range(NSEG) for g in range(NG) for j in range(NQT)
             for i in range(j + 1)]
    ns = len(steps)
    mx, tok, due = {}, {}, {}
    lane = _iota((8, T), 1)
    high = lane >= T // 2
    quarter = [lane // QB == c for c in range(HG)]
    mid = quarter[1] | quarter[2]

    def q_tile(s, g, j, c):
        h = HG * g + c
        at = DH * h // 16 - GWIN[g] // 16
        none = jnp.zeros((8, T), u32)
        return [none] * at + [q_s[s, h, j, 0:8], q_s[s, h, j, 8:16]] + [none] * (GK // 16 - 2 - at)

    def logits(s, g, k0, k1, q_tiles):
        keys = _unpack(k_s[s + zero, g, k0 // 2:k1 // 2, :])[:, :GK]
        return _dot(keys, _unpack(
            jnp.concatenate([jnp.concatenate(q, axis=0) for q in q_tiles], axis=1)))

    def stash(n, st, row0, col0, masked):
        m = None
        cols = slice(col0, col0 + st.shape[1])
        for r0 in range(0, st.shape[0], 8):
            rows = slice(row0 + r0, row0 + r0 + 8)
            x = st[r0:r0 + 8]
            if masked:
                x = x + bias_s[rows, cols]
            s_s[n % NB, rows, cols] = x
            m = x if m is None else jnp.maximum(m, x)
        return m

    def qk(n):
        s, g, j, i = steps[n]
        q = [q_tile(s, g, j, c) for c in range(HG)]
        k0 = T * i
        if i < j:
            ahead = QB if i == j - 1 else 0
            st = logits(s, g, k0, k0 + T + ahead, q)
            tok[n] = st[TOKROW:TOKROW + 8]
            m = stash(n, st[:T], 0, 0, False)
            if ahead:
                m = jnp.maximum(m, stash(n + 1, st[T:], 0, 0, True))
            mx[s, g, j] = m if i == 0 else jnp.maximum(mx[s, g, j], m)
            return
        m = stash(n, logits(s, g, k0, k0 + QB, q), 0, 0, True) if j == 0 else mx[s, g, j]
        x1 = logits(s, g, k0 + QB, k0 + 2 * QB, [_select(quarter[c], q[3], q[c]) for c in range(3)])
        x3 = logits(s, g, k0 + 3 * QB, k0 + T,
                    [_select(high, _select(mid, q[3], q[0]), _select(mid, q[2], q[1]))])
        tok[n] = jnp.concatenate([x1[QB - 8:], x3[QB - 8:]], axis=1)
        m1 = stash(n, x1, QB, 0, True)
        m1 = [m1[:, T * c:T * (c + 1)] for c in range(3)]
        m3 = stash(n, x3, QB, 3 * T, True)
        m2 = []
        for c, pair in enumerate((_select(high, q[0], q[2]), _select(mid, q[3], q[1]))):
            m2.append(jnp.maximum(*[
                stash(n, logits(s, g, k0 + r0, k0 + r0 + QB // 2, [pair]), r0, T * c, True)
                for r0 in (2 * QB, 2 * QB + QB // 2)]))
        ms = []
        for c in range(HG):
            x = m[:, T * c:T * (c + 1)]
            if c < 3:
                x = jnp.where(quarter[c], x, jnp.maximum(x, m1[c]))
            else:
                for b in range(3):
                    x = jnp.where(quarter[b], jnp.maximum(x, m1[b]), x)
            y = jnp.maximum(x, m2[c % 2])
            x = jnp.where((high, mid)[c % 2], *((y, x) if c in (0, 3) else (x, y)))
            ms.append(jnp.where(quarter[(c + 3) % HG], jnp.maximum(x, m3), x))
        mx[s, g, j] = jnp.max(jnp.concatenate(ms, axis=1), axis=0, keepdims=True)

    def pv(n):
        s, g, j, i = steps[n]
        ms = []
        for c in range(HG):
            m = jnp.broadcast_to(mx[s, g, j][:, T * c:T * (c + 1)], (8, T))
            first = tok[n + LAG - TOKBACK][:, T * c:T * (c + 1)]
            for x in due.pop((n, c), ()):
                first = jnp.maximum(first, x)
            ms.append(jnp.where(never, first, m))

        def probs(r0, r1, c, m):
            return [jnp.exp2(s_s[n % NB, r:r + 8, T * c:T * (c + 1)] - m) for r in range(r0, r1, 8)]

        if i == j:
            e1 = [probs(QB, 2 * QB, c, jnp.where(quarter[c], ms[3], ms[c])) for c in range(3)]
            e3 = probs(QB, 2 * QB, 3, jnp.where(high, jnp.where(mid, ms[3], ms[0]),
                                                jnp.where(mid, ms[2], ms[1])))
            e2 = [probs(2 * QB, 3 * QB, 0, jnp.where(high, ms[0], ms[2])),
                  probs(2 * QB, 3 * QB, 1, jnp.where(mid, ms[3], ms[1]))]
        for c in range(HG):
            if i == j:
                p = probs(0, QB, c, ms[c])
                if c < 3:
                    p += _select(quarter[c], 0.0, e1[c])
                else:
                    p += _select(quarter[0], e1[0], _select(
                        quarter[1], e1[1], _select(quarter[2], e1[2], 0.0)))
                p += _select((high, mid)[c % 2],
                             *((e2[c % 2], 0.0) if c in (0, 3) else (0.0, e2[c % 2])))
                p += _select(quarter[(c + 3) % HG], e3, 0.0)
            else:
                p = probs(0, T, c, ms[c])
            h = HG * g + c
            a = DH * h // 8 * 8
            o = DH * h - a
            one = 23 if o == 0 else 0
            v = [v_s[s, a + r:a + r + 8, T * i:T * (i + 1)] for r in (0, 8, 16)]
            v[one // 8] = jnp.where(sub == one % 8, 1.0, v[one // 8])
            acc = _dot(jnp.concatenate(v, axis=0), jnp.concatenate(p, axis=0).astype(bf16))
            if i > 0:
                acc = acc_s[c] + acc
            if i < j:
                acc_s[c] = acc
                continue
            den = acc[one:one + 1]
            inv = pltpu.reciprocal(den, approx=True)
            inv = inv * (2.0 - den * inv)
            val = acc * ((1.0 - g_s[h:h + 1, :]) * (inv * (2.0 - den * inv)))
            if c:
                val = pltpu.roll(val, T - QB * c, 1)
            due[n + DUE, c] = [val[r:r + 8] for r in (0, 8, 16)]
            o_s[s % 2, DH * h:DH * (h + 1), T * j:T * (j + 1)] = val[o:o + DH]

    def mem_update(s, t):
        w0 = WIN * t
        r0, r1_, one = _win_rows(t)
        v = [v_s[s, r:r + 8, :] for r in range(r0, r1_, 8)]
        v[(one - r0) // 8] = jnp.where(_iota((8, L), 0) == one % 8, 1.0, v[(one - r0) // 8])
        upd = _dot_nt(jnp.concatenate(v, axis=0), _unpack(pk_s[s, w0 // 2:(w0 + T) // 2, :]))
        rows = slice(r0 - w0, r1_ - w0)
        m_s[t, rows] = upd if s == 0 else m_s[t, rows] + upd

    def mem_read(s, t):
        heads = WIN_HEADS[t]
        w0 = WIN * t
        r0, r1_, one = _win_rows(t)
        rows = slice(r0 - w0, r1_ - w0)
        norm = jnp.where(mask_s[t, T:T + 8] > 0, m_s[t, one - w0:one - w0 + 1], 0.0)
        lhs = jnp.concatenate([norm, jnp.where(mask_s[t, rows] > 0, m_s[t, rows], 0.0)], axis=0)
        rd = _dot(_round_bf16(lhs), _unpack(pq_s[s - 1, w0 // 2:(w0 + T) // 2, :]))
        h0 = heads[0]
        coef = jnp.concatenate([g_s[h0:h0 + 8, :]] * NQT, axis=1) / (rd[:8] + 1e-6)
        for r in range(r0, r1_, 8):
            ha = max(r // DH, h0)
            hb = min((r + 7) // DH, heads[-1])
            cf = jnp.broadcast_to(coef[ha - h0:ha - h0 + 1], (8, L))
            if hb != ha:
                cf = jnp.where(_iota((8, L), 0) < DH * hb - r, cf,
                               jnp.broadcast_to(coef[hb - h0:hb - h0 + 1], (8, L)))
            val = rd[r - r0 + 8:r - r0 + 16] * cf
            lo, hi = max(r, DH * h0), min(r + 8, DH * (heads[-1] + 1))
            om_s[s - 1, lo:hi, :] = val[lo - r:hi - r]

    def pack_o(s, r0, r1_):
        o = o_s[s % 2, r0:r1_, :]
        if s > 0:
            o = o + om_s[s - 1, r0:r1_, :]
        ob_s[s, r0 // 2:r1_ // 2, :] = _pack(o.astype(bf16))

    def out_proj(s, r0, r1_, n=None):
        ob = ob_s[s]
        if n is not None:
            head = jnp.where(jnp.concatenate([never] * NQT, axis=1),
                             pltpu.bitcast(tok[n - TOKBACK], u32), ob[:8])
            ob = jnp.concatenate([head, ob[8:]], axis=0)
        res = _dot(_unpack(wot_s[zero, r0 // 2:r1_ // 2, :]), _unpack(ob))
        if n is not None:
            tok[n] = res[:8]
        xn = _unpack(jnp.concatenate(
            [xn_s[NQT * s + j, r0 // 2:r1_ // 2, :] for j in range(NQT)], axis=1))
        out_v[s, r0:r1_, :] = (res + x_v[s, r0:r1_, :].astype(f32) + xn.astype(f32)).astype(bf16)

    for s in range(NSEG):
        which = _iota((16, L), 0)
        routed = jnp.where(which == 0, i1, jnp.where(which == 1, i2, -1))
        ob_s[s, D // 2:D // 2 + 8, :] = _pack(
            jnp.where(_iota((16, L), 1) + s * L == routed, 1.0, 0.0).astype(bf16))
        ob_s[s, D // 2 + 8:DP // 2, :] = jnp.zeros(((DP - D) // 2 - 8, L), u32)

    extra = {}
    per = ns // NSEG
    full = [n for n, (_, _, j, i) in enumerate(steps) if i < j]

    def at(n, *task):
        extra.setdefault(n, []).append(task)

    def at_full(n, *task):
        n = next(m for m in full if m >= n)
        at(n, *task)
        return n

    n = 0
    for t in range(NWIN):
        n = at_full(n, mem_update, 0, t) + 1
        for s in range(1, NSEG):
            at_full(per * s - 40 + 6 * t, mem_read, s, t)
            if s < NSEG - 1:
                at_full(per * s + 4 + 6 * t, mem_update, s, t)
    for cp in cp_ffn:
        at(FFN0, cp.wait)
    n = FFN0
    for task in rounds:
        n = n + 1 if task is None else at_full(n, *task) + 1
    at(n + 1, ffn_finish)
    for s in range(NSEG):
        for c in range(D // 48):
            group = (48 * (c + 1) - 1) // (HG * DH)
            n = per * s + per // NG * (group + 1) + LAG + c % 2 * 3 + 1
            at(min(n, ns + LAG), pack_o, s, 48 * c, 48 * (c + 1))
    for c in range(LAG):
        at(ns + c, out_proj, 0, FILL * c, FILL * (c + 1), ns + c)

    for n in range(ns + LAG + 1):
        if n < ns:
            qk(n)
        for fn, *args in extra.get(n, ()):
            if fn is not ffn_in:
                fn(*args)
        if LAG <= n < ns + LAG:
            pv(n - LAG)
        for fn, *args in extra.get(n, ()):
            if fn is ffn_in:
                fn(*args)
    out_proj(0, FILL * LAG, D, ns + LAG)
    cp_out[0].start()
    for s in range(1, NSEG - 1):
        out_proj(s, 0, D)
        cp_out[s].start()
    for (r0, r1_), cp in zip(TAIL, cp_tail):
        out_proj(NSEG - 1, r0, r1_)
        cp.start()
    for cp in cp_out + cp_tail:
        cp.wait()


@jax.jit
def pallas_parallel_sum__memory_aug_infini_attn__moe_arch_mod__prompt_kernel(
    A_x: jax.Array,
    A_wq: jax.Array,
    A_wk: jax.Array,
    A_wv: jax.Array,
    A_wo: jax.Array,
    A_beta: jax.Array,
    B_x: jax.Array,
    B_w_r: jax.Array,
    B_w_gate: jax.Array,
    B_w_up: jax.Array,
    B_w_down: jax.Array,
):
    del B_x
    out_t = pl.pallas_call(
        _kernel,
        out_shape=jax.ShapeDtypeStruct((D, S), bf16),
        in_specs=[pl.BlockSpec(memory_space=pl.ANY)] * 10,
        out_specs=pl.BlockSpec(memory_space=pl.ANY),
        scratch_shapes=[
            pltpu.VMEM((NSEG, D, L), bf16),
            pltpu.VMEM((D, D), bf16),
            pltpu.VMEM((D, D), bf16),
            pltpu.VMEM((D, D), bf16),
            pltpu.VMEM((D, D), bf16),
            pltpu.VMEM((D, F), bf16),
            pltpu.VMEM((D, F), bf16),
            pltpu.VMEM((D, F), bf16),
            pltpu.VMEM((1, H), bf16),
            pltpu.VMEM((D,), bf16),
            pltpu.VMEM((NSEG, D, L), bf16),
            pltpu.VMEM((1, 3 * D // 2, DP), u32),
            pltpu.VMEM((1, D // 2, DP), u32),
            pltpu.VMEM((S // T, DP // 2, T), u32),
            pltpu.VMEM((NSEG, H, NQT, 16, T), u32),
            pltpu.VMEM((NSEG, NG, L // 2, T), u32),
            pltpu.VMEM((NSEG, D, L), f32),
            pltpu.VMEM((NSEG - 1, D // 2, L), u32),
            pltpu.VMEM((NSEG - 1, D // 2, L), u32),
            pltpu.VMEM((2, D // 2, T), f32),
            pltpu.VMEM((S // T, T), f32),
            pltpu.VMEM((T, T), f32),
            pltpu.VMEM((3 * QB, HG * T), f32),
            pltpu.VMEM((NB, T, HG * T), f32),
            pltpu.VMEM((HG, 24, T), f32),
            pltpu.VMEM((2, D, L), f32),
            pltpu.VMEM((NSEG, DP // 2, L), u32),
            pltpu.VMEM((NWIN, T + 8, T), f32),
            pltpu.VMEM((NWIN, T, T), f32),
            pltpu.VMEM((NSEG - 1, D, L), f32),
            pltpu.VMEM((8, F), f32),
            pltpu.SemaphoreType.DMA((9,)),
        ],
        compiler_params=pltpu.CompilerParams(vmem_limit_bytes=100 * 1024 * 1024),
        name="infini_moe",
    )(A_x.reshape(S, D).T, A_wq, A_wk, A_wv, A_wo, A_beta.reshape(1, H), B_w_r,
      B_w_gate, B_w_up, B_w_down.T)
    return out_t.T.reshape(1, S, D)
```

```python
import math

import jax
import jax.numpy as jnp
import numpy as np
from jax import lax
import jax.experimental.pallas as pl
import jax.experimental.pallas.tpu as pltpu

S = 2048
D = 576
H = 32
DH = D // H
NSEG = 4
L = S // NSEG
F = 4608
T = 128
DP = 640
NT = DP // T
NQT = L // T

HG = 4
NG = H // HG
GK = 80
GWIN = [HG * DH * g // 16 * 16 for g in range(NG)]
QB = T // HG

WIN = 112
WIN_HEADS = [list(range(a, b)) for a, b in ((0, 7), (7, 13), (13, 19), (19, 25), (25, 32))]
NWIN = len(WIN_HEADS)

VCUT = (208, 448, 496, 528)
LAG = 11
NB = 13
TOKBACK = 2
TOKROW = 80
DUE = 20
FFN0 = 61
FILL = 48
TAIL = ((0, 320), (320, 512), (512, D))

RQ, RK, RV = 0, D, 2 * D
LOG2E = math.log2(math.e)
QSCALE = DH ** -0.5 * LOG2E
MASKVAL = float(np.asarray(-1e9, dtype=jnp.bfloat16).astype(np.float32)) * LOG2E
LN_EPS = float(np.asarray(1e-5, dtype=jnp.bfloat16).astype(np.float32))

bf16 = jnp.bfloat16
f32 = jnp.float32
u32 = jnp.uint32


def _pack(x):
    return pltpu.bitcast(x, u32)


def _unpack(x):
    return pltpu.bitcast(x, bf16)


def _halves(x):
    return [pltpu.unpack_elementwise(x, index=i, packed_dtype=bf16, unpacked_dtype=f32)
            for i in range(2)]


def _join(even, odd):
    return pltpu.bitcast(pltpu.pack_elementwise([even, odd], packed_dtype=bf16), u32)


def _dot(a, b):
    return lax.dot_general(a, b, (((1,), (0,)), ((), ())), preferred_element_type=f32)


def _dot_nt(a, b):
    return lax.dot_general(a, b, (((1,), (1,)), ((), ())), preferred_element_type=f32)


def _iota(shape, dim):
    return lax.broadcasted_iota(jnp.int32, shape, dim)


def _phi(t):
    return jnp.where(t > 0, t + 1.0, jnp.exp(t))


def _round_bf16(x):
    return x.astype(bf16).astype(f32)


def _sigmoid(x):
    return 1.0 / (1.0 + jnp.exp(-x))


def _all_max(x):
    return jnp.max(jnp.max(x, axis=0, keepdims=True), axis=1, keepdims=True)


def _select(mask, a, b):
    n = len(a) if isinstance(a, list) else len(b)
    out = []
    for r in range(n):
        x = a[r] if isinstance(a, list) else a
        y = b[r] if isinstance(b, list) else b
        out.append(x if x is y else jnp.where(mask, x, y))
    return out


def _store_transposed(dst, row0, w_ref, i, j, tail=None):
    r = min(T, D - T * i)
    c = min(T, D - T * j)
    t = w_ref[T * i:T * i + r, T * j:T * j + c]
    if c < T:
        t = jnp.concatenate([t, jnp.zeros((r, T - c), bf16)], axis=1)
    if r < T:
        parts = [t] if tail is None else [t, tail]
        parts.append(jnp.zeros((T - sum(p.shape[0] for p in parts), T), bf16))
        t = jnp.concatenate(parts, axis=0)
    r0 = (row0 + T * j) // 2
    dst[0, r0:r0 + c // 2, T * i:T * (i + 1)] = _pack(t.T)[:c // 2]


def _win_rows(t):
    lo, hi = DH * WIN_HEADS[t][0], DH * (WIN_HEADS[t][-1] + 1)
    r0, r1 = lo // 8 * 8, -(-hi // 8) * 8
    return r0, r1, r0 if r0 < lo else r1 - 1


def _kernel(x_hbm, wq_hbm, wk_hbm, wv_hbm, wo_hbm, beta_hbm, wr_hbm, wg_hbm, wu_hbm, wd_hbm,
            out_hbm,
            x_v, wq_v, wk_v, wv_v, wo_v, wg_v, wu_v, wd_v, beta_v, wr_v, out_v,
            wt_s, wot_s, xn_s, q_s, k_s, v_s, pq_s, pk_s, wr_s, r_s, g_s, bias_s, s_s, acc_s,
            o_s, ob_s, mask_s, m_s, om_s, h_s, sems):
    def copy(src, dst, sem):
        return pltpu.make_async_copy(src, dst, sems.at[sem])

    cp_beta = copy(beta_hbm, beta_v, 0)
    cp_wr = copy(wr_hbm, wr_v, 0)
    cp_x0 = [copy(x_hbm.at[:, pl.ds(c * L // 2, L // 2)], x_v.at[0, :, pl.ds(c * L // 2, L // 2)], c)
             for c in range(2)]
    cp_wv = [copy(wv_hbm.at[:, pl.ds(c0, c1 - c0)], wv_v.at[:, pl.ds(c0, c1 - c0)], sem)
             for c0, c1, sem in ((0, 2 * T, 2), (2 * T, D, 3))]
    cp_wq = copy(wq_hbm, wq_v, 4)
    cp_mid = [copy(x_hbm.at[:, pl.ds(L, L)], x_v.at[1], 5), copy(wk_hbm, wk_v, 5)]
    cp_rest = [copy(x_hbm.at[:, pl.ds(s * L, L)], x_v.at[s], 6) for s in (2, 3)]
    cp_rest.append(copy(wo_hbm, wo_v, 6))
    cp_ffn = [copy(wg_hbm, wg_v, 7), copy(wu_hbm, wu_v, 7), copy(wd_hbm, wd_v, 7)]
    cp_out = [copy(out_v.at[s], out_hbm.at[:, pl.ds(s * L, L)], 8) for s in range(NSEG - 1)]
    cp_tail = [copy(out_v.at[NSEG - 1, pl.ds(r0, r1 - r0)],
                    out_hbm.at[pl.ds(r0, r1 - r0), pl.ds(S - L, L)], 8) for r0, r1 in TAIL]
    for cp in [cp_beta, cp_wr] + cp_x0 + cp_wv + [cp_wq] + cp_mid + cp_rest + cp_ffn:
        cp.start()

    col = _iota((T, T), 1)
    row = _iota((T, T), 0)
    for t in range(NWIN):
        same = None
        pick = None
        for n, h in enumerate(WIN_HEADS[t]):
            lo, hi = DH * h - WIN * t, DH * (h + 1) - WIN * t
            cin = (col >= lo) & (col < hi)
            blk = cin & (row >= lo) & (row < hi)
            same = blk if same is None else same | blk
            mine = cin[:8] & (row[:8] == n)
            pick = mine if pick is None else pick | mine
        mask_s[t, 0:T] = jnp.where(same, 1.0, 0.0)
        mask_s[t, T:T + 8] = jnp.where(pick, 1.0, 0.0)
    key = _iota((QB, T), 0)
    qry = _iota((QB, T), 1)
    qpos = [(qry - QB * c) % T for c in range(HG)]
    slot = qry // QB
    tiles = [qpos,
             [jnp.where(slot == c, qpos[3], qpos[c]) for c in range(3)] + [qry % QB + QB],
             [jnp.where(slot >= 2, qpos[0], qpos[2]),
              jnp.where((slot == 1) | (slot == 2), qpos[3], qpos[1])]]
    for b, tile_row in enumerate(tiles):
        for c, queries in enumerate(tile_row):
            bias_s[QB * b:QB * (b + 1), T * c:T * (c + 1)] = jnp.where(
                queries < key + QB * b, MASKVAL, 0.0)
    for j in range(S // T):
        xn_s[j, D // 2:DP // 2 - 8, :] = jnp.zeros(((DP - D) // 2 - 8, T), u32)

    def transpose_w(row0, w, j0=0, j1=NT):
        for j in range(j0, j1):
            for i in range(NT):
                _store_transposed(wt_s, row0, w, i, j)

    def layernorm(s, j):
        xe, xo = _halves(_pack(x_v[s, :, T * j:T * (j + 1)]))
        mean = jnp.sum(xe + xo, axis=0, keepdims=True) / D
        ce, co = xe - mean, xo - mean
        var = jnp.sum(ce * ce + co * co, axis=0, keepdims=True) / D
        inv = 1.0 / _round_bf16(jnp.sqrt(_round_bf16(_round_bf16(var) + LN_EPS)))
        mean = _round_bf16(mean)
        de, do = _halves(_join(xe - mean, xo - mean))
        xn = _join(de * inv, do * inv)
        even, odd = _halves(xn)
        score = jnp.sum(even * wr_s[0] + odd * wr_s[1], axis=0, keepdims=True)
        score = jnp.broadcast_to(score, (8, T))
        r_s[NQT * s + j:NQT * s + j + 1, :] = score[:1]
        xn_s[NQT * s + j, 0:D // 2, :] = xn
        xn_s[NQT * s + j, DP // 2 - 8:DP // 2, :] = jnp.where(
            never, pltpu.bitcast(score, u32), jnp.zeros((), u32))

    def project(s, r0, r1):
        xn = _unpack(jnp.concatenate([xn_s[NQT * s + j] for j in range(NQT)], axis=1))
        return _dot(_unpack(wt_s[zero, r0 // 2:r1 // 2, :]), xn)

    def proj_q(s):
        q = project(s, RQ, RK)
        if s > 0:
            pq_s[s - 1] = _pack(_phi(q).astype(bf16))
        q = _pack((q * QSCALE).astype(bf16))
        for h in range(H):
            a = DH * h // 16
            lo = (DH * h - 16 * a) // 2
            pair = _iota((16, L), 0)
            qh = jnp.where((pair >= lo) & (pair < lo + DH // 2), q[8 * a:8 * a + 16],
                           jnp.zeros((), u32))
            for j in range(NQT):
                qt = qh[:, T * j:T * (j + 1)]
                q_s[s, h, j] = pltpu.roll(qt, QB * (h % HG), 1) if h % HG else qt

    def proj_k(s):
        k = project(s, RK, RV)
        if s < NSEG - 1:
            pk_s[s] = _pack(_phi(k).astype(bf16))
        for j in range(NQT):
            kb = k[:, T * j:T * (j + 1)].astype(bf16)
            for g in range(NG):
                kw = jnp.concatenate([kb[GWIN[g]:GWIN[g] + GK], jnp.zeros((T - GK, T), bf16)], axis=0)
                k_s[s, g, T // 2 * j:T // 2 * (j + 1), :] = _pack(kw.T)

    def proj_v(s, r0=0, r1=D):
        v_s[s, r0:r1, :] = _round_bf16(project(s, RV + r0, RV + r1))

    for cp in (cp_x0[0], cp_beta, cp_wr):
        cp.wait()
    gate = _round_bf16(_sigmoid(beta_v[...].astype(f32)))
    zero = jnp.where(jnp.max(gate) > 2.0, 1, 0)
    gate = jnp.concatenate([gate, jnp.zeros((1, T - H), f32)], axis=1)
    g_s[...] = jnp.broadcast_to(gate, (T, T)).T
    sub = _iota((8, T), 0)
    never = sub > zero + 8
    wr = jnp.concatenate([wr_v[...].reshape(1, D), jnp.zeros((1, DP - D), bf16)], axis=1)
    wr_s[0], wr_s[1] = _halves(_pack(jnp.broadcast_to(wr, (T, DP)).T)[:D // 2])
    layernorm(0, 0)
    layernorm(0, 1)
    cp_x0[1].wait()
    layernorm(0, 2)
    layernorm(0, 3)
    cp_wv[0].wait()
    transpose_w(RV, wv_v, 0, 2)
    proj_v(0, 0, VCUT[0])
    cp_wv[1].wait()
    transpose_w(RV, wv_v, 2, NT)
    proj_v(0, VCUT[0], 2 * T)
    proj_v(0, 2 * T, VCUT[1])
    cp_wq.wait()
    transpose_w(RQ, wq_v)
    proj_v(0, VCUT[1], VCUT[2])
    proj_q(0)
    proj_v(0, VCUT[2], VCUT[3])
    for cp in cp_mid:
        cp.wait()
    transpose_w(RK, wk_v)
    for j in range(NQT):
        layernorm(1, j)
    proj_v(0, VCUT[3], D)
    proj_k(0)
    proj_v(1)
    for cp in cp_rest:
        cp.wait()
    for s in (2, 3):
        for j in range(NQT):
            layernorm(s, j)
        proj_q(s - 1)
    proj_q(3)
    for j in range(NT):
        for i in range(NT - 1):
            _store_transposed(wot_s, 0, wo_v, i, j)

    r = _round_bf16(r_s[...])
    pos = (_iota((S // T, T), 0) * T + _iota((S // T, T), 1)).astype(f32)
    r1 = _all_max(r)
    i1 = -_all_max(jnp.where(r == r1, -pos, 1.0 - S))
    rest = pos != i1
    r2 = _all_max(jnp.where(rest, r, -jnp.inf))
    i2 = -_all_max(jnp.where(rest & (r == r2), -pos, 1.0 - S))
    i1, i2 = i1.astype(jnp.int32), i2.astype(jnp.int32)

    for s in range(1, NSEG):
        proj_k(s)
        if s > 1:
            proj_v(s)

    xsel = jnp.zeros((8, DP), f32)
    for c, idx in enumerate((i1, i2)):
        token = jnp.where(_iota((DP // 2, T), 1) == idx % T, xn_s[(idx // T)[0, 0]],
                          jnp.zeros((), u32))
        xsel = xsel + _dot_nt(jnp.where(sub == c, 1.0, 0.0), _unpack(token))

    ffn = {}

    def ffn_in(w, name, cg, i):
        k = min(T, D - T * i)
        part = _dot(xsel[:, T * i:T * i + k], w[T * i:T * i + k, L * cg:L * (cg + 1)])
        ffn[name] = part if i == 0 else ffn[name] + part
        if name == "up" and i == NT - 1:
            h_s[:, L * cg:L * (cg + 1)] = _round_bf16(
                ffn["gate"] * _sigmoid(ffn["gate"]) * ffn["up"])

    def ffn_out(cg, i):
        if i < 4:
            c0 = L * cg + T * i
            name, part = "y0", _dot_nt(h_s[:, c0:c0 + T], wd_v[0:4 * T, c0:c0 + T])
        else:
            cols = slice(L * cg, L * (cg + 1))
            name, part = "y1", _dot_nt(h_s[:, cols], wd_v[4 * T:D, cols])
        ffn[name] = ffn[name] + part if name in ffn else part

    def ffn_finish():
        y = jnp.concatenate([ffn["y0"], ffn["y1"], jnp.zeros((8, DP - D), f32)], axis=1)
        y = y * _sigmoid(jnp.where(_iota((8, DP), 0) == 0, r1, r2))
        y = jnp.concatenate([y, jnp.zeros((8, DP), f32)], axis=0)
        for j in range(NT):
            _store_transposed(wot_s, 0, wo_v, NT - 1, j, tail=y[:, T * j:T * (j + 1)].astype(bf16))

    rounds = []
    for cg in range(F // L):
        rounds += [(ffn_in, wg_v, "gate", cg, i) for i in range(NT)]
        rounds += [(ffn_in, wu_v, "up", cg, i) for i in range(NT)]
        if cg > 0:
            rounds += [(ffn_out, cg - 1, i) for i in range(NT)]
    rounds += [None] * 3
    rounds += [(ffn_out, F // L - 1, i) for i in range(NT)]

    steps = [(s, g, j, i) for s in range(NSEG) for g in range(NG) for j in range(NQT)
             for i in range(j + 1)]
    ns = len(steps)
    mx, tok, due = {}, {}, {}
    lane = _iota((8, T), 1)
    high = lane >= T // 2
    quarter = [lane // QB == c for c in range(HG)]
    mid = quarter[1] | quarter[2]

    def q_tile(s, g, j, c):
        h = HG * g + c
        at = DH * h // 16 - GWIN[g] // 16
        none = jnp.zeros((8, T), u32)
        return [none] * at + [q_s[s, h, j, 0:8], q_s[s, h, j, 8:16]] + [none] * (GK // 16 - 2 - at)

    def logits(s, g, k0, k1, q_tiles):
        keys = _unpack(k_s[s + zero, g, k0 // 2:k1 // 2, :])[:, :GK]
        return _dot(keys, _unpack(
            jnp.concatenate([jnp.concatenate(q, axis=0) for q in q_tiles], axis=1)))

    def stash(n, st, row0, col0, masked):
        m = None
        cols = slice(col0, col0 + st.shape[1])
        for r0 in range(0, st.shape[0], 8):
            rows = slice(row0 + r0, row0 + r0 + 8)
            x = st[r0:r0 + 8]
            if masked:
                x = x + bias_s[rows, cols]
            s_s[n % NB, rows, cols] = x
            m = x if m is None else jnp.maximum(m, x)
        return m

    def qk(n):
        s, g, j, i = steps[n]
        q = [q_tile(s, g, j, c) for c in range(HG)]
        k0 = T * i
        if i < j:
            ahead = QB if i == j - 1 else 0
            st = logits(s, g, k0, k0 + T + ahead, q)
            tok[n] = st[TOKROW:TOKROW + 8]
            m = stash(n, st[:T], 0, 0, False)
            if ahead:
                m = jnp.maximum(m, stash(n + 1, st[T:], 0, 0, True))
            mx[s, g, j] = m if i == 0 else jnp.maximum(mx[s, g, j], m)
            return
        m = stash(n, logits(s, g, k0, k0 + QB, q), 0, 0, True) if j == 0 else mx[s, g, j]
        x1 = logits(s, g, k0 + QB, k0 + 2 * QB, [_select(quarter[c], q[3], q[c]) for c in range(3)])
        x3 = logits(s, g, k0 + 3 * QB, k0 + T,
                    [_select(high, _select(mid, q[3], q[0]), _select(mid, q[2], q[1]))])
        tok[n] = jnp.concatenate([x1[QB - 8:], x3[QB - 8:]], axis=1)
        m1 = stash(n, x1, QB, 0, True)
        m1 = [m1[:, T * c:T * (c + 1)] for c in range(3)]
        m3 = stash(n, x3, QB, 3 * T, True)
        m2 = []
        for c, pair in enumerate((_select(high, q[0], q[2]), _select(mid, q[3], q[1]))):
            m2.append(jnp.maximum(*[
                stash(n, logits(s, g, k0 + r0, k0 + r0 + QB // 2, [pair]), r0, T * c, True)
                for r0 in (2 * QB, 2 * QB + QB // 2)]))
        ms = []
        for c in range(HG):
            x = m[:, T * c:T * (c + 1)]
            if c < 3:
                x = jnp.where(quarter[c], x, jnp.maximum(x, m1[c]))
            else:
                for b in range(3):
                    x = jnp.where(quarter[b], jnp.maximum(x, m1[b]), x)
            y = jnp.maximum(x, m2[c % 2])
            x = jnp.where((high, mid)[c % 2], *((y, x) if c in (0, 3) else (x, y)))
            ms.append(jnp.where(quarter[(c + 3) % HG], jnp.maximum(x, m3), x))
        mx[s, g, j] = jnp.max(jnp.concatenate(ms, axis=1), axis=0, keepdims=True)

    def pv(n):
        s, g, j, i = steps[n]
        ms = []
        for c in range(HG):
            m = jnp.broadcast_to(mx[s, g, j][:, T * c:T * (c + 1)], (8, T))
            first = tok[n + LAG - TOKBACK][:, T * c:T * (c + 1)]
            for x in due.pop((n, c), ()):
                first = jnp.maximum(first, x)
            ms.append(jnp.where(never, first, m))

        def probs(r0, r1, c, m):
            return [jnp.exp2(s_s[n % NB, r:r + 8, T * c:T * (c + 1)] - m) for r in range(r0, r1, 8)]

        if i == j:
            e1 = [probs(QB, 2 * QB, c, jnp.where(quarter[c], ms[3], ms[c])) for c in range(3)]
            e3 = probs(QB, 2 * QB, 3, jnp.where(high, jnp.where(mid, ms[3], ms[0]),
                                                jnp.where(mid, ms[2], ms[1])))
            e2 = [probs(2 * QB, 3 * QB, 0, jnp.where(high, ms[0], ms[2])),
                  probs(2 * QB, 3 * QB, 1, jnp.where(mid, ms[3], ms[1]))]
        for c in range(HG):
            if i == j:
                p = probs(0, QB, c, ms[c])
                if c < 3:
                    p += _select(quarter[c], 0.0, e1[c])
                else:
                    p += _select(quarter[0], e1[0], _select(
                        quarter[1], e1[1], _select(quarter[2], e1[2], 0.0)))
                p += _select((high, mid)[c % 2],
                             *((e2[c % 2], 0.0) if c in (0, 3) else (0.0, e2[c % 2])))
                p += _select(quarter[(c + 3) % HG], e3, 0.0)
            else:
                p = probs(0, T, c, ms[c])
            h = HG * g + c
            a = DH * h // 8 * 8
            o = DH * h - a
            one = 23 if o == 0 else 0
            v = [v_s[s, a + r:a + r + 8, T * i:T * (i + 1)] for r in (0, 8, 16)]
            v[one // 8] = jnp.where(sub == one % 8, 1.0, v[one // 8])
            acc = _dot(jnp.concatenate(v, axis=0), jnp.concatenate(p, axis=0).astype(bf16))
            if i > 0:
                acc = acc_s[c] + acc
            if i < j:
                acc_s[c] = acc
                continue
            den = acc[one:one + 1]
            inv = pltpu.reciprocal(den, approx=True)
            inv = inv * (2.0 - den * inv)
            val = acc * ((1.0 - g_s[h:h + 1, :]) * (inv * (2.0 - den * inv)))
            if c:
                val = pltpu.roll(val, T - QB * c, 1)
            due[n + DUE, c] = [val[r:r + 8] for r in (0, 8, 16)]
            o_s[s % 2, DH * h:DH * (h + 1), T * j:T * (j + 1)] = val[o:o + DH]

    def mem_update(s, t):
        w0 = WIN * t
        r0, r1_, one = _win_rows(t)
        v = [v_s[s, r:r + 8, :] for r in range(r0, r1_, 8)]
        v[(one - r0) // 8] = jnp.where(_iota((8, L), 0) == one % 8, 1.0, v[(one - r0) // 8])
        upd = _dot_nt(jnp.concatenate(v, axis=0), _unpack(pk_s[s, w0 // 2:(w0 + T) // 2, :]))
        rows = slice(r0 - w0, r1_ - w0)
        m_s[t, rows] = upd if s == 0 else m_s[t, rows] + upd

    def mem_read(s, t):
        heads = WIN_HEADS[t]
        w0 = WIN * t
        r0, r1_, one = _win_rows(t)
        rows = slice(r0 - w0, r1_ - w0)
        norm = jnp.where(mask_s[t, T:T + 8] > 0, m_s[t, one - w0:one - w0 + 1], 0.0)
        lhs = jnp.concatenate([norm, jnp.where(mask_s[t, rows] > 0, m_s[t, rows], 0.0)], axis=0)
        rd = _dot(_round_bf16(lhs), _unpack(pq_s[s - 1, w0 // 2:(w0 + T) // 2, :]))
        h0 = heads[0]
        coef = jnp.concatenate([g_s[h0:h0 + 8, :]] * NQT, axis=1) / (rd[:8] + 1e-6)
        for r in range(r0, r1_, 8):
            ha = max(r // DH, h0)
            hb = min((r + 7) // DH, heads[-1])
            cf = jnp.broadcast_to(coef[ha - h0:ha - h0 + 1], (8, L))
            if hb != ha:
                cf = jnp.where(_iota((8, L), 0) < DH * hb - r, cf,
                               jnp.broadcast_to(coef[hb - h0:hb - h0 + 1], (8, L)))
            val = rd[r - r0 + 8:r - r0 + 16] * cf
            lo, hi = max(r, DH * h0), min(r + 8, DH * (heads[-1] + 1))
            om_s[s - 1, lo:hi, :] = val[lo - r:hi - r]

    def pack_o(s, r0, r1_):
        o = o_s[s % 2, r0:r1_, :]
        if s > 0:
            o = o + om_s[s - 1, r0:r1_, :]
        ob_s[s, r0 // 2:r1_ // 2, :] = _pack(o.astype(bf16))

    def out_proj(s, r0, r1_, n=None):
        ob = ob_s[s]
        if n is not None:
            head = jnp.where(jnp.concatenate([never] * NQT, axis=1),
                             pltpu.bitcast(tok[n - TOKBACK], u32), ob[:8])
            ob = jnp.concatenate([head, ob[8:]], axis=0)
        res = _dot(_unpack(wot_s[zero, r0 // 2:r1_ // 2, :]), _unpack(ob))
        if n is not None:
            tok[n] = res[:8]
        xn = _unpack(jnp.concatenate(
            [xn_s[NQT * s + j, r0 // 2:r1_ // 2, :] for j in range(NQT)], axis=1))
        out_v[s, r0:r1_, :] = (res + x_v[s, r0:r1_, :].astype(f32) + xn.astype(f32)).astype(bf16)

    for s in range(NSEG):
        which = _iota((16, L), 0)
        routed = jnp.where(which == 0, i1, jnp.where(which == 1, i2, -1))
        ob_s[s, D // 2:D // 2 + 8, :] = _pack(
            jnp.where(_iota((16, L), 1) + s * L == routed, 1.0, 0.0).astype(bf16))
        ob_s[s, D // 2 + 8:DP // 2, :] = jnp.zeros(((DP - D) // 2 - 8, L), u32)

    extra = {}
    per = ns // NSEG
    full = [n for n, (_, _, j, i) in enumerate(steps) if i < j]

    def at(n, *task):
        extra.setdefault(n, []).append(task)

    def at_full(n, *task):
        n = next(m for m in full if m >= n)
        at(n, *task)
        return n

    n = 0
    for t in range(NWIN):
        n = at_full(n, mem_update, 0, t) + 1
        for s in range(1, NSEG):
            at_full(per * s - 40 + 6 * t, mem_read, s, t)
            if s < NSEG - 1:
                at_full(per * s + 4 + 6 * t, mem_update, s, t)
    for cp in cp_ffn:
        at(FFN0, cp.wait)
    n = FFN0
    for task in rounds:
        n = n + 1 if task is None else at_full(n, *task) + 1
    at(n + 1, ffn_finish)
    for s in range(NSEG):
        for c in range(D // 48):
            group = (48 * (c + 1) - 1) // (HG * DH)
            n = per * s + per // NG * (group + 1) + LAG + c % 2 * 3 + 1
            at(min(n, ns + LAG), pack_o, s, 48 * c, 48 * (c + 1))
    for c in range(LAG):
        at(ns + c, out_proj, 0, FILL * c, FILL * (c + 1), ns + c)

    for n in range(ns + LAG + 1):
        if n < ns:
            qk(n)
        for fn, *args in extra.get(n, ()):
            if fn is not ffn_in:
                fn(*args)
        if LAG <= n < ns + LAG:
            pv(n - LAG)
        for fn, *args in extra.get(n, ()):
            if fn is ffn_in:
                fn(*args)
    out_proj(0, FILL * LAG, D, ns + LAG)
    cp_out[0].start()
    for s in range(1, NSEG - 1):
        out_proj(s, 0, D)
        cp_out[s].start()
    for (r0, r1_), cp in zip(TAIL, cp_tail):
        out_proj(NSEG - 1, r0, r1_)
        cp.start()
    for cp in cp_out + cp_tail:
        cp.wait()


@jax.jit
def pallas_parallel_sum__memory_aug_infini_attn__moe_arch_mod__prompt_kernel(
    A_x: jax.Array,
    A_wq: jax.Array,
    A_wk: jax.Array,
    A_wv: jax.Array,
    A_wo: jax.Array,
    A_beta: jax.Array,
    B_x: jax.Array,
    B_w_r: jax.Array,
    B_w_gate: jax.Array,
    B_w_up: jax.Array,
    B_w_down: jax.Array,
):
    del B_x
    out_t = pl.pallas_call(
        _kernel,
        out_shape=jax.ShapeDtypeStruct((D, S), bf16),
        in_specs=[pl.BlockSpec(memory_space=pl.ANY)] * 10,
        out_specs=pl.BlockSpec(memory_space=pl.ANY),
        scratch_shapes=[
            pltpu.VMEM((NSEG, D, L), bf16),
            pltpu.VMEM((D, D), bf16),
            pltpu.VMEM((D, D), bf16),
            pltpu.VMEM((D, D), bf16),
            pltpu.VMEM((D, D), bf16),
            pltpu.VMEM((D, F), bf16),
            pltpu.VMEM((D, F), bf16),
            pltpu.VMEM((D, F), bf16),
            pltpu.VMEM((1, H), bf16),
            pltpu.VMEM((D,), bf16),
            pltpu.VMEM((NSEG, D, L), bf16),
            pltpu.VMEM((1, 3 * D // 2, DP), u32),
            pltpu.VMEM((1, D // 2, DP), u32),
            pltpu.VMEM((S // T, DP // 2, T), u32),
            pltpu.VMEM((NSEG, H, NQT, 16, T), u32),
            pltpu.VMEM((NSEG, NG, L // 2, T), u32),
            pltpu.VMEM((NSEG, D, L), f32),
            pltpu.VMEM((NSEG - 1, D // 2, L), u32),
            pltpu.VMEM((NSEG - 1, D // 2, L), u32),
            pltpu.VMEM((2, D // 2, T), f32),
            pltpu.VMEM((S // T, T), f32),
            pltpu.VMEM((T, T), f32),
            pltpu.VMEM((3 * QB, HG * T), f32),
            pltpu.VMEM((NB, T, HG * T), f32),
            pltpu.VMEM((HG, 24, T), f32),
            pltpu.VMEM((2, D, L), f32),
            pltpu.VMEM((NSEG, DP // 2, L), u32),
            pltpu.VMEM((NWIN, T + 8, T), f32),
            pltpu.VMEM((NWIN, T, T), f32),
            pltpu.VMEM((NSEG - 1, D, L), f32),
            pltpu.VMEM((8, F), f32),
            pltpu.SemaphoreType.DMA((9,)),
        ],
        compiler_params=pltpu.CompilerParams(vmem_limit_bytes=100 * 1024 * 1024),
        name="infini_moe",
    )(A_x.reshape(S, D).T, A_wq, A_wk, A_wv, A_wo, A_beta.reshape(1, H), B_w_r,
      B_w_gate, B_w_up, B_w_down.T)
    return out_t.T.reshape(1, S, D)
```

```python
import math

import jax
import jax.numpy as jnp
import numpy as np
from jax import lax
import jax.experimental.pallas as pl
import jax.experimental.pallas.tpu as pltpu

S = 2048
D = 576
H = 32
DH = D // H
NSEG = 4
L = S // NSEG
F = 4608
T = 128
DP = 640
NT = DP // T
NQT = L // T

HG = 4
NG = H // HG
GK = 80
GWIN = [HG * DH * g // 16 * 16 for g in range(NG)]
QB = T // HG

WIN = 112
WIN_HEADS = [list(range(a, b)) for a, b in ((0, 7), (7, 13), (13, 19), (19, 25), (25, 32))]
NWIN = len(WIN_HEADS)

VCUT = (208, 448, 496, 528)
LAG = 11
NB = 13
TOKBACK = 2
TOKROW = 80
DUE = 30
MEM0 = 3
FFN0 = 70
FILL = 48
TAIL = ((0, 320), (320, 512), (512, D))

RQ, RK, RV = 0, D, 2 * D
LOG2E = math.log2(math.e)
QSCALE = DH ** -0.5 * LOG2E
MASKVAL = float(np.asarray(-1e9, dtype=jnp.bfloat16).astype(np.float32)) * LOG2E
LN_EPS = float(np.asarray(1e-5, dtype=jnp.bfloat16).astype(np.float32))

bf16 = jnp.bfloat16
f32 = jnp.float32
u32 = jnp.uint32


def _pack(x):
    return pltpu.bitcast(x, u32)


def _unpack(x):
    return pltpu.bitcast(x, bf16)


def _halves(x):
    return [pltpu.unpack_elementwise(x, index=i, packed_dtype=bf16, unpacked_dtype=f32)
            for i in range(2)]


def _join(even, odd):
    return pltpu.bitcast(pltpu.pack_elementwise([even, odd], packed_dtype=bf16), u32)


def _dot(a, b):
    return lax.dot_general(a, b, (((1,), (0,)), ((), ())), preferred_element_type=f32)


def _dot_nt(a, b):
    return lax.dot_general(a, b, (((1,), (1,)), ((), ())), preferred_element_type=f32)


def _iota(shape, dim):
    return lax.broadcasted_iota(jnp.int32, shape, dim)


def _phi(t):
    return jnp.where(t > 0, t + 1.0, jnp.exp(t))


def _round_bf16(x):
    return x.astype(bf16).astype(f32)


def _sigmoid(x):
    return 1.0 / (1.0 + jnp.exp(-x))


def _all_max(x):
    return jnp.max(jnp.max(x, axis=0, keepdims=True), axis=1, keepdims=True)


def _select(mask, a, b):
    n = len(a) if isinstance(a, list) else len(b)
    out = []
    for r in range(n):
        x = a[r] if isinstance(a, list) else a
        y = b[r] if isinstance(b, list) else b
        out.append(x if x is y else jnp.where(mask, x, y))
    return out


def _store_transposed(dst, row0, w_ref, i, j, tail=None):
    r = min(T, D - T * i)
    c = min(T, D - T * j)
    t = w_ref[T * i:T * i + r, T * j:T * j + c]
    if c < T:
        t = jnp.concatenate([t, jnp.zeros((r, T - c), bf16)], axis=1)
    if r < T:
        parts = [t] if tail is None else [t, tail]
        parts.append(jnp.zeros((T - sum(p.shape[0] for p in parts), T), bf16))
        t = jnp.concatenate(parts, axis=0)
    r0 = (row0 + T * j) // 2
    dst[0, r0:r0 + c // 2, T * i:T * (i + 1)] = _pack(t.T)[:c // 2]


def _win_rows(t):
    lo, hi = DH * WIN_HEADS[t][0], DH * (WIN_HEADS[t][-1] + 1)
    r0, r1 = lo // 8 * 8, -(-hi // 8) * 8
    return r0, r1, r0 if r0 < lo else r1 - 1


def _kernel(x_hbm, wq_hbm, wk_hbm, wv_hbm, wo_hbm, beta_hbm, wr_hbm, wg_hbm, wu_hbm, wd_hbm,
            out_hbm,
            x_v, wq_v, wk_v, wv_v, wo_v, wg_v, wu_v, wd_v, beta_v, wr_v, out_v,
            wt_s, wot_s, xn_s, q_s, k_s, v_s, pq_s, pk_s, wr_s, r_s, g_s, bias_s, s_s, acc_s,
            o_s, ob_s, mask_s, m_s, om_s, h_s, sems):
    def copy(src, dst, sem):
        return pltpu.make_async_copy(src, dst, sems.at[sem])

    cp_beta = copy(beta_hbm, beta_v, 0)
    cp_wr = copy(wr_hbm, wr_v, 0)
    cp_x0 = [copy(x_hbm.at[:, pl.ds(c * L // 2, L // 2)], x_v.at[0, :, pl.ds(c * L // 2, L // 2)], c)
             for c in range(2)]
    cp_wv = [copy(wv_hbm.at[:, pl.ds(c0, c1 - c0)], wv_v.at[:, pl.ds(c0, c1 - c0)], sem)
             for c0, c1, sem in ((0, 2 * T, 2), (2 * T, D, 3))]
    cp_wq = copy(wq_hbm, wq_v, 4)
    cp_mid = [copy(x_hbm.at[:, pl.ds(L, L)], x_v.at[1], 5), copy(wk_hbm, wk_v, 5)]
    cp_rest = [copy(x_hbm.at[:, pl.ds(s * L, L)], x_v.at[s], 6) for s in (2, 3)]
    cp_rest.append(copy(wo_hbm, wo_v, 6))
    cp_ffn = [copy(wg_hbm, wg_v, 7), copy(wu_hbm, wu_v, 7), copy(wd_hbm, wd_v, 7)]
    cp_out = [copy(out_v.at[s], out_hbm.at[:, pl.ds(s * L, L)], 8) for s in range(NSEG - 1)]
    cp_tail = [copy(out_v.at[NSEG - 1, pl.ds(r0, r1 - r0)],
                    out_hbm.at[pl.ds(r0, r1 - r0), pl.ds(S - L, L)], 8) for r0, r1 in TAIL]
    for cp in [cp_beta, cp_wr] + cp_x0 + cp_wv + [cp_wq] + cp_mid + cp_rest + cp_ffn:
        cp.start()

    col = _iota((T, T), 1)
    row = _iota((T, T), 0)
    for t in range(NWIN):
        same = None
        pick = None
        for n, h in enumerate(WIN_HEADS[t]):
            lo, hi = DH * h - WIN * t, DH * (h + 1) - WIN * t
            cin = (col >= lo) & (col < hi)
            blk = cin & (row >= lo) & (row < hi)
            same = blk if same is None else same | blk
            mine = cin[:8] & (row[:8] == n)
            pick = mine if pick is None else pick | mine
        mask_s[t, 0:T] = jnp.where(same, 1.0, 0.0)
        mask_s[t, T:T + 8] = jnp.where(pick, 1.0, 0.0)
    key = _iota((QB, T), 0)
    qry = _iota((QB, T), 1)
    qpos = [(qry - QB * c) % T for c in range(HG)]
    slot = qry // QB
    tiles = [qpos,
             [jnp.where(slot == c, qpos[3], qpos[c]) for c in range(3)] + [qry % QB + QB],
             [jnp.where(slot >= 2, qpos[0], qpos[2]),
              jnp.where((slot == 1) | (slot == 2), qpos[3], qpos[1])]]
    for b, tile_row in enumerate(tiles):
        for c, queries in enumerate(tile_row):
            bias_s[QB * b:QB * (b + 1), T * c:T * (c + 1)] = jnp.where(
                queries < key + QB * b, MASKVAL, 0.0)
    for j in range(S // T):
        xn_s[j, D // 2:DP // 2 - 8, :] = jnp.zeros(((DP - D) // 2 - 8, T), u32)

    def transpose_w(row0, w, j0=0, j1=NT):
        for j in range(j0, j1):
            for i in range(NT):
                _store_transposed(wt_s, row0, w, i, j)

    def layernorm(s, j):
        xe, xo = _halves(_pack(x_v[s, :, T * j:T * (j + 1)]))
        mean = jnp.sum(xe + xo, axis=0, keepdims=True) / D
        ce, co = xe - mean, xo - mean
        var = jnp.sum(ce * ce + co * co, axis=0, keepdims=True) / D
        inv = 1.0 / _round_bf16(jnp.sqrt(_round_bf16(_round_bf16(var) + LN_EPS)))
        mean = _round_bf16(mean)
        de, do = _halves(_join(xe - mean, xo - mean))
        xn = _join(de * inv, do * inv)
        even, odd = _halves(xn)
        score = jnp.sum(even * wr_s[0] + odd * wr_s[1], axis=0, keepdims=True)
        score = jnp.broadcast_to(score, (8, T))
        r_s[NQT * s + j:NQT * s + j + 1, :] = score[:1]
        xn_s[NQT * s + j, 0:D // 2, :] = xn
        xn_s[NQT * s + j, DP // 2 - 8:DP // 2, :] = jnp.where(
            never, pltpu.bitcast(score, u32), jnp.zeros((), u32))

    def project(s, r0, r1):
        xn = _unpack(jnp.concatenate([xn_s[NQT * s + j] for j in range(NQT)], axis=1))
        return _dot(_unpack(wt_s[zero, r0 // 2:r1 // 2, :]), xn)

    def proj_q(s):
        q = project(s, RQ, RK)
        if s > 0:
            pq_s[s - 1] = _pack(_phi(q).astype(bf16))
        q = _pack((q * QSCALE).astype(bf16))
        for h in range(H):
            a = DH * h // 16
            lo = (DH * h - 16 * a) // 2
            pair = _iota((16, L), 0)
            qh = jnp.where((pair >= lo) & (pair < lo + DH // 2), q[8 * a:8 * a + 16],
                           jnp.zeros((), u32))
            for j in range(NQT):
                qt = qh[:, T * j:T * (j + 1)]
                q_s[s, h, j] = pltpu.roll(qt, QB * (h % HG), 1) if h % HG else qt

    def proj_k(s):
        k = project(s, RK, RV)
        if s < NSEG - 1:
            pk_s[s] = _pack(_phi(k).astype(bf16))
        for j in range(NQT):
            kb = k[:, T * j:T * (j + 1)].astype(bf16)
            for g in range(NG):
                kw = jnp.concatenate([kb[GWIN[g]:GWIN[g] + GK], jnp.zeros((T - GK, T), bf16)], axis=0)
                k_s[s, g, T // 2 * j:T // 2 * (j + 1), :] = _pack(kw.T)

    def proj_v(s, r0=0, r1=D):
        v_s[s, r0:r1, :] = _round_bf16(project(s, RV + r0, RV + r1))

    for cp in (cp_x0[0], cp_beta, cp_wr):
        cp.wait()
    gate = _round_bf16(_sigmoid(beta_v[...].astype(f32)))
    zero = jnp.where(jnp.max(gate) > 2.0, 1, 0)
    gate = jnp.concatenate([gate, jnp.zeros((1, T - H), f32)], axis=1)
    g_s[...] = jnp.broadcast_to(gate, (T, T)).T
    sub = _iota((8, T), 0)
    never = sub > zero + 8
    wr = jnp.concatenate([wr_v[...].reshape(1, D), jnp.zeros((1, DP - D), bf16)], axis=1)
    wr_s[0], wr_s[1] = _halves(_pack(jnp.broadcast_to(wr, (T, DP)).T)[:D // 2])
    layernorm(0, 0)
    layernorm(0, 1)
    cp_x0[1].wait()
    layernorm(0, 2)
    layernorm(0, 3)
    cp_wv[0].wait()
    transpose_w(RV, wv_v, 0, 2)
    proj_v(0, 0, VCUT[0])
    cp_wv[1].wait()
    transpose_w(RV, wv_v, 2, NT)
    proj_v(0, VCUT[0], 2 * T)
    proj_v(0, 2 * T, VCUT[1])
    cp_wq.wait()
    transpose_w(RQ, wq_v)
    proj_v(0, VCUT[1], VCUT[2])
    proj_q(0)
    proj_v(0, VCUT[2], VCUT[3])
    for cp in cp_mid:
        cp.wait()
    transpose_w(RK, wk_v)
    for j in range(NQT):
        layernorm(1, j)
    proj_v(0, VCUT[3], D)
    proj_k(0)
    proj_v(1)
    for cp in cp_rest:
        cp.wait()
    for s in (2, 3):
        for j in range(NQT):
            layernorm(s, j)
        proj_q(s - 1)
    proj_q(3)
    for j in range(NT):
        for i in range(NT - 1):
            _store_transposed(wot_s, 0, wo_v, i, j)

    r = _round_bf16(r_s[...])
    pos = (_iota((S // T, T), 0) * T + _iota((S // T, T), 1)).astype(f32)
    r1 = _all_max(r)
    i1 = -_all_max(jnp.where(r == r1, -pos, 1.0 - S))
    rest = pos != i1
    r2 = _all_max(jnp.where(rest, r, -jnp.inf))
    i2 = -_all_max(jnp.where(rest & (r == r2), -pos, 1.0 - S))
    i1, i2 = i1.astype(jnp.int32), i2.astype(jnp.int32)

    for s in range(1, NSEG):
        proj_k(s)
        if s > 1:
            proj_v(s)

    xsel = jnp.zeros((8, DP), f32)
    for c, idx in enumerate((i1, i2)):
        token = jnp.where(_iota((DP // 2, T), 1) == idx % T, xn_s[(idx // T)[0, 0]],
                          jnp.zeros((), u32))
        xsel = xsel + _dot_nt(jnp.where(sub == c, 1.0, 0.0), _unpack(token))

    ffn = {}

    def ffn_in(w, name, cg, i):
        k = min(T, D - T * i)
        part = _dot(xsel[:, T * i:T * i + k], w[T * i:T * i + k, L * cg:L * (cg + 1)])
        ffn[name] = part if i == 0 else ffn[name] + part
        if name == "up" and i == NT - 1:
            h_s[:, L * cg:L * (cg + 1)] = _round_bf16(
                ffn["gate"] * _sigmoid(ffn["gate"]) * ffn["up"])

    def ffn_out(cg, i):
        if i < 4:
            c0 = L * cg + T * i
            name, part = "y0", _dot_nt(h_s[:, c0:c0 + T], wd_v[0:4 * T, c0:c0 + T])
        else:
            cols = slice(L * cg, L * (cg + 1))
            name, part = "y1", _dot_nt(h_s[:, cols], wd_v[4 * T:D, cols])
        ffn[name] = ffn[name] + part if name in ffn else part

    def ffn_finish():
        y = jnp.concatenate([ffn["y0"], ffn["y1"], jnp.zeros((8, DP - D), f32)], axis=1)
        y = y * _sigmoid(jnp.where(_iota((8, DP), 0) == 0, r1, r2))
        y = jnp.concatenate([y, jnp.zeros((8, DP), f32)], axis=0)
        for j in range(NT):
            _store_transposed(wot_s, 0, wo_v, NT - 1, j, tail=y[:, T * j:T * (j + 1)].astype(bf16))

    rounds = []
    for cg in range(F // L):
        rounds += [(ffn_in, wg_v, "gate", cg, i) for i in range(NT)]
        rounds += [(ffn_in, wu_v, "up", cg, i) for i in range(NT)]
        if cg > 0:
            rounds += [(ffn_out, cg - 1, i) for i in range(NT)]
    rounds += [None] * 3
    rounds += [(ffn_out, F // L - 1, i) for i in range(NT)]

    steps = [(s, g, j, i) for s in range(NSEG) for g in range(NG) for j in range(NQT)
             for i in range(j + 1)]
    ns = len(steps)
    mx, tok, due = {}, {}, {}
    lane = _iota((8, T), 1)
    high = lane >= T // 2
    quarter = [lane // QB == c for c in range(HG)]
    mid = quarter[1] | quarter[2]

    def q_tile(s, g, j, c):
        h = HG * g + c
        at = DH * h // 16 - GWIN[g] // 16
        none = jnp.zeros((8, T), u32)
        return [none] * at + [q_s[s, h, j, 0:8], q_s[s, h, j, 8:16]] + [none] * (GK // 16 - 2 - at)

    def logits(s, g, k0, k1, q_tiles):
        keys = _unpack(k_s[s + zero, g, k0 // 2:k1 // 2, :])[:, :GK]
        return _dot(keys, _unpack(
            jnp.concatenate([jnp.concatenate(q, axis=0) for q in q_tiles], axis=1)))

    def stash(n, st, row0, col0, masked):
        m = None
        cols = slice(col0, col0 + st.shape[1])
        for r0 in range(0, st.shape[0], 8):
            rows = slice(row0 + r0, row0 + r0 + 8)
            x = st[r0:r0 + 8]
            if masked:
                x = x + bias_s[rows, cols]
            s_s[n % NB, rows, cols] = x
            m = x if m is None else jnp.maximum(m, x)
        return m

    def qk(n):
        s, g, j, i = steps[n]
        q = [q_tile(s, g, j, c) for c in range(HG)]
        k0 = T * i
        if i < j:
            ahead = QB if i == j - 1 else 0
            st = logits(s, g, k0, k0 + T + ahead, q)
            tok[n] = st[TOKROW:TOKROW + 8]
            m = stash(n, st[:T], 0, 0, False)
            if ahead:
                m = jnp.maximum(m, stash(n + 1, st[T:], 0, 0, True))
            mx[s, g, j] = m if i == 0 else jnp.maximum(mx[s, g, j], m)
            return
        m = stash(n, logits(s, g, k0, k0 + QB, q), 0, 0, True) if j == 0 else mx[s, g, j]
        x1 = logits(s, g, k0 + QB, k0 + 2 * QB, [_select(quarter[c], q[3], q[c]) for c in range(3)])
        x3 = logits(s, g, k0 + 3 * QB, k0 + T,
                    [_select(high, _select(mid, q[3], q[0]), _select(mid, q[2], q[1]))])
        tok[n] = jnp.concatenate([x1[QB - 8:], x3[QB - 8:]], axis=1)
        m1 = stash(n, x1, QB, 0, True)
        m1 = [m1[:, T * c:T * (c + 1)] for c in range(3)]
        m3 = stash(n, x3, QB, 3 * T, True)
        m2 = []
        for c, pair in enumerate((_select(high, q[0], q[2]), _select(mid, q[3], q[1]))):
            m2.append(jnp.maximum(*[
                stash(n, logits(s, g, k0 + r0, k0 + r0 + QB // 2, [pair]), r0, T * c, True)
                for r0 in (2 * QB, 2 * QB + QB // 2)]))
        ms = []
        for c in range(HG):
            x = m[:, T * c:T * (c + 1)]
            if c < 3:
                x = jnp.where(quarter[c], x, jnp.maximum(x, m1[c]))
            else:
                for b in range(3):
                    x = jnp.where(quarter[b], jnp.maximum(x, m1[b]), x)
            y = jnp.maximum(x, m2[c % 2])
            x = jnp.where((high, mid)[c % 2], *((y, x) if c in (0, 3) else (x, y)))
            ms.append(jnp.where(quarter[(c + 3) % HG], jnp.maximum(x, m3), x))
        mx[s, g, j] = jnp.max(jnp.concatenate(ms, axis=1), axis=0, keepdims=True)

    def pv(n):
        s, g, j, i = steps[n]
        ms = []
        for c in range(HG):
            m = jnp.broadcast_to(mx[s, g, j][:, T * c:T * (c + 1)], (8, T))
            first = tok[n + LAG - TOKBACK][:, T * c:T * (c + 1)]
            for x in due.pop((n, c), ()):
                first = jnp.maximum(first, x)
            ms.append(jnp.where(never, first, m))

        def probs(r0, r1, c, m):
            return [jnp.exp2(s_s[n % NB, r:r + 8, T * c:T * (c + 1)] - m) for r in range(r0, r1, 8)]

        if i == j:
            e1 = [probs(QB, 2 * QB, c, jnp.where(quarter[c], ms[3], ms[c])) for c in range(3)]
            e3 = probs(QB, 2 * QB, 3, jnp.where(high, jnp.where(mid, ms[3], ms[0]),
                                                jnp.where(mid, ms[2], ms[1])))
            e2 = [probs(2 * QB, 3 * QB, 0, jnp.where(high, ms[0], ms[2])),
                  probs(2 * QB, 3 * QB, 1, jnp.where(mid, ms[3], ms[1]))]
        for c in range(HG):
            if i == j:
                p = probs(0, QB, c, ms[c])
                if c < 3:
                    p += _select(quarter[c], 0.0, e1[c])
                else:
                    p += _select(quarter[0], e1[0], _select(
                        quarter[1], e1[1], _select(quarter[2], e1[2], 0.0)))
                p += _select((high, mid)[c % 2],
                             *((e2[c % 2], 0.0) if c in (0, 3) else (0.0, e2[c % 2])))
                p += _select(quarter[(c + 3) % HG], e3, 0.0)
            else:
                p = probs(0, T, c, ms[c])
            h = HG * g + c
            a = DH * h // 8 * 8
            o = DH * h - a
            one = 23 if o == 0 else 0
            v = [v_s[s, a + r:a + r + 8, T * i:T * (i + 1)] for r in (0, 8, 16)]
            v[one // 8] = jnp.where(sub == one % 8, 1.0, v[one // 8])
            acc = _dot(jnp.concatenate(v, axis=0), jnp.concatenate(p, axis=0).astype(bf16))
            if i > 0:
                acc = acc_s[c] + acc
            if i < j:
                acc_s[c] = acc
                continue
            den = acc[one:one + 1]
            inv = pltpu.reciprocal(den, approx=True)
            inv = inv * (2.0 - den * inv)
            val = acc * ((1.0 - g_s[h:h + 1, :]) * (inv * (2.0 - den * inv)))
            if c:
                val = pltpu.roll(val, T - QB * c, 1)
            due[n + DUE, c] = [val[r:r + 8] for r in (0, 8, 16)]
            o_s[s % 2, DH * h:DH * (h + 1), T * j:T * (j + 1)] = val[o:o + DH]

    def mem_update(s, t):
        w0 = WIN * t
        r0, r1_, one = _win_rows(t)
        v = [v_s[s, r:r + 8, :] for r in range(r0, r1_, 8)]
        v[(one - r0) // 8] = jnp.where(_iota((8, L), 0) == one % 8, 1.0, v[(one - r0) // 8])
        upd = _dot_nt(jnp.concatenate(v, axis=0), _unpack(pk_s[s, w0 // 2:(w0 + T) // 2, :]))
        rows = slice(r0 - w0, r1_ - w0)
        m_s[t, rows] = upd if s == 0 else m_s[t, rows] + upd

    def mem_read(s, t):
        heads = WIN_HEADS[t]
        w0 = WIN * t
        r0, r1_, one = _win_rows(t)
        rows = slice(r0 - w0, r1_ - w0)
        norm = jnp.where(mask_s[t, T:T + 8] > 0, m_s[t, one - w0:one - w0 + 1], 0.0)
        lhs = jnp.concatenate([norm, jnp.where(mask_s[t, rows] > 0, m_s[t, rows], 0.0)], axis=0)
        rd = _dot(_round_bf16(lhs), _unpack(pq_s[s - 1, w0 // 2:(w0 + T) // 2, :]))
        h0 = heads[0]
        coef = jnp.concatenate([g_s[h0:h0 + 8, :]] * NQT, axis=1) / (rd[:8] + 1e-6)
        for r in range(r0, r1_, 8):
            ha = max(r // DH, h0)
            hb = min((r + 7) // DH, heads[-1])
            cf = jnp.broadcast_to(coef[ha - h0:ha - h0 + 1], (8, L))
            if hb != ha:
                cf = jnp.where(_iota((8, L), 0) < DH * hb - r, cf,
                               jnp.broadcast_to(coef[hb - h0:hb - h0 + 1], (8, L)))
            val = rd[r - r0 + 8:r - r0 + 16] * cf
            lo, hi = max(r, DH * h0), min(r + 8, DH * (heads[-1] + 1))
            om_s[s - 1, lo:hi, :] = val[lo - r:hi - r]

    def pack_o(s, r0, r1_):
        o = o_s[s % 2, r0:r1_, :]
        if s > 0:
            o = o + om_s[s - 1, r0:r1_, :]
        ob_s[s, r0 // 2:r1_ // 2, :] = _pack(o.astype(bf16))

    def out_proj(s, r0, r1_, n=None):
        ob = ob_s[s]
        if n is not None:
            head = jnp.where(jnp.concatenate([never] * NQT, axis=1),
                             pltpu.bitcast(tok[n - TOKBACK], u32), ob[:8])
            ob = jnp.concatenate([head, ob[8:]], axis=0)
        res = _dot(_unpack(wot_s[zero, r0 // 2:r1_ // 2, :]), _unpack(ob))
        if n is not None:
            tok[n] = res[:8]
        xn = _unpack(jnp.concatenate(
            [xn_s[NQT * s + j, r0 // 2:r1_ // 2, :] for j in range(NQT)], axis=1))
        out_v[s, r0:r1_, :] = (res + x_v[s, r0:r1_, :].astype(f32) + xn.astype(f32)).astype(bf16)

    for s in range(NSEG):
        which = _iota((16, L), 0)
        routed = jnp.where(which == 0, i1, jnp.where(which == 1, i2, -1))
        ob_s[s, D // 2:D // 2 + 8, :] = _pack(
            jnp.where(_iota((16, L), 1) + s * L == routed, 1.0, 0.0).astype(bf16))
        ob_s[s, D // 2 + 8:DP // 2, :] = jnp.zeros(((DP - D) // 2 - 8, L), u32)

    extra = {}
    per = ns // NSEG
    full = [n for n, (_, _, j, i) in enumerate(steps) if i < j]

    def at(n, *task):
        extra.setdefault(n, []).append(task)

    def at_full(n, *task):
        n = next(m for m in full if m >= n)
        at(n, *task)
        return n

    for s in range(1, NSEG):
        for t in range(NWIN):
            at(MEM0 + 2 * s - 2, mem_update, s - 1, t)
            at(MEM0 + 2 * s - 1, mem_read, s, t)
    for cp in cp_ffn:
        at(FFN0, cp.wait)
    n = FFN0
    for task in rounds:
        n = n + 1 if task is None else at_full(n, *task) + 1
    at(n + 1, ffn_finish)
    for s in range(NSEG):
        for c in range(D // 48):
            group = (48 * (c + 1) - 1) // (HG * DH)
            n = per * s + per // NG * (group + 1) + LAG + c % 2 * 3 + 1
            at(min(n, ns + LAG), pack_o, s, 48 * c, 48 * (c + 1))
    for c in range(LAG):
        at(ns + c, out_proj, 0, FILL * c, FILL * (c + 1), ns + c)

    for n in range(ns + LAG + 1):
        if n < ns:
            qk(n)
        for fn, *args in extra.get(n, ()):
            if fn is not ffn_in:
                fn(*args)
        if LAG <= n < ns + LAG:
            pv(n - LAG)
        for fn, *args in extra.get(n, ()):
            if fn is ffn_in:
                fn(*args)
    out_proj(0, FILL * LAG, D, ns + LAG)
    cp_out[0].start()
    for s in range(1, NSEG - 1):
        out_proj(s, 0, D)
        cp_out[s].start()
    for (r0, r1_), cp in zip(TAIL, cp_tail):
        out_proj(NSEG - 1, r0, r1_)
        cp.start()
    for cp in cp_out + cp_tail:
        cp.wait()


@jax.jit
def pallas_parallel_sum__memory_aug_infini_attn__moe_arch_mod__prompt_kernel(
    A_x: jax.Array,
    A_wq: jax.Array,
    A_wk: jax.Array,
    A_wv: jax.Array,
    A_wo: jax.Array,
    A_beta: jax.Array,
    B_x: jax.Array,
    B_w_r: jax.Array,
    B_w_gate: jax.Array,
    B_w_up: jax.Array,
    B_w_down: jax.Array,
):
    del B_x
    out_t = pl.pallas_call(
        _kernel,
        out_shape=jax.ShapeDtypeStruct((D, S), bf16),
        in_specs=[pl.BlockSpec(memory_space=pl.ANY)] * 10,
        out_specs=pl.BlockSpec(memory_space=pl.ANY),
        scratch_shapes=[
            pltpu.VMEM((NSEG, D, L), bf16),
            pltpu.VMEM((D, D), bf16),
            pltpu.VMEM((D, D), bf16),
            pltpu.VMEM((D, D), bf16),
            pltpu.VMEM((D, D), bf16),
            pltpu.VMEM((D, F), bf16),
            pltpu.VMEM((D, F), bf16),
            pltpu.VMEM((D, F), bf16),
            pltpu.VMEM((1, H), bf16),
            pltpu.VMEM((D,), bf16),
            pltpu.VMEM((NSEG, D, L), bf16),
            pltpu.VMEM((1, 3 * D // 2, DP), u32),
            pltpu.VMEM((1, D // 2, DP), u32),
            pltpu.VMEM((S // T, DP // 2, T), u32),
            pltpu.VMEM((NSEG, H, NQT, 16, T), u32),
            pltpu.VMEM((NSEG, NG, L // 2, T), u32),
            pltpu.VMEM((NSEG, D, L), f32),
            pltpu.VMEM((NSEG - 1, D // 2, L), u32),
            pltpu.VMEM((NSEG - 1, D // 2, L), u32),
            pltpu.VMEM((2, D // 2, T), f32),
            pltpu.VMEM((S // T, T), f32),
            pltpu.VMEM((T, T), f32),
            pltpu.VMEM((3 * QB, HG * T), f32),
            pltpu.VMEM((NB, T, HG * T), f32),
            pltpu.VMEM((HG, 24, T), f32),
            pltpu.VMEM((2, D, L), f32),
            pltpu.VMEM((NSEG, DP // 2, L), u32),
            pltpu.VMEM((NWIN, T + 8, T), f32),
            pltpu.VMEM((NWIN, T, T), f32),
            pltpu.VMEM((NSEG - 1, D, L), f32),
            pltpu.VMEM((8, F), f32),
            pltpu.SemaphoreType.DMA((9,)),
        ],
        compiler_params=pltpu.CompilerParams(vmem_limit_bytes=100 * 1024 * 1024),
        name="infini_moe",
    )(A_x.reshape(S, D).T, A_wq, A_wk, A_wv, A_wo, A_beta.reshape(1, H), B_w_r,
      B_w_gate, B_w_up, B_w_down.T)
    return out_t.T.reshape(1, S, D)
```

```python
import math

import jax
import jax.numpy as jnp
import numpy as np
from jax import lax
import jax.experimental.pallas as pl
import jax.experimental.pallas.tpu as pltpu

S = 2048
D = 576
H = 32
DH = D // H
NSEG = 4
L = S // NSEG
F = 4608
T = 128
DP = 640
NT = DP // T
NQT = L // T

HG = 4
NG = H // HG
GK = 80
GWIN = [HG * DH * g // 16 * 16 for g in range(NG)]
QB = T // HG

WIN = 112
WIN_HEADS = [list(range(a, b)) for a, b in ((0, 7), (7, 13), (13, 19), (19, 25), (25, 32))]
NWIN = len(WIN_HEADS)

VCUT = (208, 448, 496, 528)
LAG = 11
NB = 13
TOKBACK = 2
TOKROW = 80
DUE = 30
MEM0 = 3
FFN0 = 70
FILL = 48
TAIL = ((0, 320), (320, 512), (512, D))

RQ, RK, RV = 0, D, 2 * D
LOG2E = math.log2(math.e)
QSCALE = DH ** -0.5 * LOG2E
MASKVAL = float(np.asarray(-1e9, dtype=jnp.bfloat16).astype(np.float32)) * LOG2E
LN_EPS = float(np.asarray(1e-5, dtype=jnp.bfloat16).astype(np.float32))

bf16 = jnp.bfloat16
f32 = jnp.float32
u32 = jnp.uint32


def _pack(x):
    return pltpu.bitcast(x, u32)


def _unpack(x):
    return pltpu.bitcast(x, bf16)


def _halves(x):
    return (lax.bitcast_convert_type(x << 16, f32),
            lax.bitcast_convert_type(x & np.uint32(0xFFFF0000), f32))


def _join(even, odd):
    return (lax.bitcast_convert_type(even, u32) >> 16) | lax.bitcast_convert_type(odd, u32)


def _dot(a, b):
    return lax.dot_general(a, b, (((1,), (0,)), ((), ())), preferred_element_type=f32)


def _dot_nt(a, b):
    return lax.dot_general(a, b, (((1,), (1,)), ((), ())), preferred_element_type=f32)


def _iota(shape, dim):
    return lax.broadcasted_iota(jnp.int32, shape, dim)


def _phi(t):
    return jnp.where(t > 0, t + 1.0, jnp.exp(t))


def _round_bf16(x):
    return x.astype(bf16).astype(f32)


def _sigmoid(x):
    return 1.0 / (1.0 + jnp.exp(-x))


def _all_max(x):
    return jnp.max(jnp.max(x, axis=0, keepdims=True), axis=1, keepdims=True)


def _select(mask, a, b):
    return [x if x is y else lax.select(mask, x, y) for x, y in zip(a, b)]


def _store_transposed(dst, row0, w_ref, i, j, tail=None):
    r = min(T, D - T * i)
    c = min(T, D - T * j)
    t = w_ref[T * i:T * i + r, T * j:T * j + c]
    if c < T:
        t = jnp.concatenate([t, jnp.zeros((r, T - c), bf16)], axis=1)
    if r < T:
        parts = [t] if tail is None else [t, tail]
        parts.append(jnp.zeros((T - sum(p.shape[0] for p in parts), T), bf16))
        t = jnp.concatenate(parts, axis=0)
    r0 = (row0 + T * j) // 2
    dst[0, r0:r0 + c // 2, T * i:T * (i + 1)] = _pack(t.T)[:c // 2]


def _win_rows(t):
    lo, hi = DH * WIN_HEADS[t][0], DH * (WIN_HEADS[t][-1] + 1)
    r0, r1 = lo // 8 * 8, -(-hi // 8) * 8
    return r0, r1, r0 if r0 < lo else r1 - 1


def _kernel(x_hbm, wq_hbm, wk_hbm, wv_hbm, wo_hbm, beta_hbm, wr_hbm, wg_hbm, wu_hbm, wd_hbm,
            out_hbm,
            x_v, wq_v, wk_v, wv_v, wo_v, wg_v, wu_v, wd_v, beta_v, wr_v, out_v,
            wt_s, wot_s, xn_s, q_s, k_s, v_s, pq_s, pk_s, wr_s, r_s, g_s, bias_s, s_s, acc_s,
            o_s, ob_s, mask_s, m_s, om_s, h_s, sems):
    def copy(src, dst, sem):
        return pltpu.make_async_copy(src, dst, sems.at[sem])

    cp_beta = copy(beta_hbm, beta_v, 0)
    cp_wr = copy(wr_hbm, wr_v, 0)
    cp_x0 = [copy(x_hbm.at[:, pl.ds(c * L // 2, L // 2)], x_v.at[0, :, pl.ds(c * L // 2, L // 2)], c)
             for c in range(2)]
    cp_wv = [copy(wv_hbm.at[:, pl.ds(c0, c1 - c0)], wv_v.at[:, pl.ds(c0, c1 - c0)], sem)
             for c0, c1, sem in ((0, 2 * T, 2), (2 * T, D, 3))]
    cp_wq = copy(wq_hbm, wq_v, 4)
    cp_mid = [copy(x_hbm.at[:, pl.ds(L, L)], x_v.at[1], 5), copy(wk_hbm, wk_v, 5)]
    cp_rest = [copy(x_hbm.at[:, pl.ds(s * L, L)], x_v.at[s], 6) for s in (2, 3)]
    cp_rest.append(copy(wo_hbm, wo_v, 6))
    cp_ffn = [copy(wg_hbm, wg_v, 7), copy(wu_hbm, wu_v, 7), copy(wd_hbm, wd_v, 7)]
    cp_out = [copy(out_v.at[s], out_hbm.at[:, pl.ds(s * L, L)], 8) for s in range(NSEG - 1)]
    cp_tail = [copy(out_v.at[NSEG - 1, pl.ds(r0, r1 - r0)],
                    out_hbm.at[pl.ds(r0, r1 - r0), pl.ds(S - L, L)], 8) for r0, r1 in TAIL]
    for cp in [cp_beta, cp_wr] + cp_x0 + cp_wv + [cp_wq] + cp_mid + cp_rest + cp_ffn:
        cp.start()

    col = _iota((T, T), 1)
    row = _iota((T, T), 0)
    for t in range(NWIN):
        same = None
        pick = None
        for n, h in enumerate(WIN_HEADS[t]):
            lo, hi = DH * h - WIN * t, DH * (h + 1) - WIN * t
            cin = (col >= lo) & (col < hi)
            blk = cin & (row >= lo) & (row < hi)
            same = blk if same is None else same | blk
            mine = cin[:8] & (row[:8] == n)
            pick = mine if pick is None else pick | mine
        mask_s[t, 0:T] = jnp.where(same, 1.0, 0.0)
        mask_s[t, T:T + 8] = jnp.where(pick, 1.0, 0.0)
    key = _iota((QB, T), 0)
    qry = _iota((QB, T), 1)
    qpos = [(qry - QB * c) % T for c in range(HG)]
    slot = qry // QB
    tiles = [qpos,
             [jnp.where(slot == c, qpos[3], qpos[c]) for c in range(3)] + [qry % QB + QB],
             [jnp.where(slot >= 2, qpos[0], qpos[2]),
              jnp.where((slot == 1) | (slot == 2), qpos[3], qpos[1])]]
    for b, tile_row in enumerate(tiles):
        for c, queries in enumerate(tile_row):
            bias_s[QB * b:QB * (b + 1), T * c:T * (c + 1)] = jnp.where(
                queries < key + QB * b, MASKVAL, 0.0)
    for j in range(S // T):
        xn_s[j, D // 2:DP // 2 - 8, :] = jnp.zeros(((DP - D) // 2 - 8, T), u32)

    def transpose_w(row0, w, j0=0, j1=NT):
        for j in range(j0, j1):
            for i in range(NT):
                _store_transposed(wt_s, row0, w, i, j)

    def layernorm(s, j):
        xe, xo = _halves(_pack(x_v[s, :, T * j:T * (j + 1)]))
        mean = jnp.sum(xe + xo, axis=0, keepdims=True) / D
        ce, co = xe - mean, xo - mean
        var = jnp.sum(ce * ce + co * co, axis=0, keepdims=True) / D
        inv = 1.0 / _round_bf16(jnp.sqrt(_round_bf16(_round_bf16(var) + LN_EPS)))
        mean = _round_bf16(mean)
        even, odd = [_round_bf16(_round_bf16(x - mean) * inv) for x in (xe, xo)]
        score = jnp.sum(even * wr_s[0] + odd * wr_s[1], axis=0, keepdims=True)
        score = jnp.broadcast_to(score, (8, T))
        r_s[NQT * s + j:NQT * s + j + 1, :] = score[:1]
        xn_s[NQT * s + j, 0:D // 2, :] = _join(even, odd)
        xn_s[NQT * s + j, DP // 2 - 8:DP // 2, :] = jnp.where(
            never, pltpu.bitcast(score, u32), jnp.zeros((), u32))

    def project(s, r0, r1):
        xn = _unpack(jnp.concatenate([xn_s[NQT * s + j] for j in range(NQT)], axis=1))
        return _dot(_unpack(wt_s[zero, r0 // 2:r1 // 2, :]), xn)

    def proj_q(s):
        q = project(s, RQ, RK)
        if s > 0:
            pq_s[s - 1] = _pack(_phi(q).astype(bf16))
        q = _pack((q * QSCALE).astype(bf16))
        for h in range(H):
            a = DH * h // 16
            lo = (DH * h - 16 * a) // 2
            pair = _iota((16, L), 0)
            qh = jnp.where((pair >= lo) & (pair < lo + DH // 2), q[8 * a:8 * a + 16],
                           jnp.zeros((), u32))
            for j in range(NQT):
                qt = qh[:, T * j:T * (j + 1)]
                q_s[s, h, j] = pltpu.roll(qt, QB * (h % HG), 1) if h % HG else qt

    def proj_k(s):
        k = project(s, RK, RV)
        if s < NSEG - 1:
            pk_s[s] = _pack(_phi(k).astype(bf16))
        for j in range(NQT):
            kb = k[:, T * j:T * (j + 1)].astype(bf16)
            for g in range(NG):
                kw = jnp.concatenate([kb[GWIN[g]:GWIN[g] + GK], jnp.zeros((T - GK, T), bf16)], axis=0)
                k_s[s, g, T // 2 * j:T // 2 * (j + 1), :] = _pack(kw.T)

    def proj_v(s, r0=0, r1=D):
        v_s[s, r0:r1, :] = _round_bf16(project(s, RV + r0, RV + r1))

    for cp in (cp_x0[0], cp_beta, cp_wr):
        cp.wait()
    gate = _round_bf16(_sigmoid(beta_v[...].astype(f32)))
    zero = jnp.where(jnp.max(gate) > 2.0, 1, 0)
    gate = jnp.concatenate([gate, jnp.zeros((1, T - H), f32)], axis=1)
    g_s[...] = jnp.broadcast_to(gate, (T, T)).T
    sub = _iota((8, T), 0)
    never = sub > zero + 8
    wr = jnp.concatenate([wr_v[...].reshape(1, D), jnp.zeros((1, DP - D), bf16)], axis=1)
    wr_s[0], wr_s[1] = _halves(_pack(jnp.broadcast_to(wr, (T, DP)).T)[:D // 2])
    layernorm(0, 0)
    layernorm(0, 1)
    cp_x0[1].wait()
    layernorm(0, 2)
    layernorm(0, 3)
    cp_wv[0].wait()
    transpose_w(RV, wv_v, 0, 2)
    proj_v(0, 0, VCUT[0])
    cp_wv[1].wait()
    transpose_w(RV, wv_v, 2, NT)
    proj_v(0, VCUT[0], 2 * T)
    proj_v(0, 2 * T, VCUT[1])
    cp_wq.wait()
    transpose_w(RQ, wq_v)
    proj_v(0, VCUT[1], VCUT[2])
    proj_q(0)
    proj_v(0, VCUT[2], VCUT[3])
    for cp in cp_mid:
        cp.wait()
    transpose_w(RK, wk_v)
    for j in range(NQT):
        layernorm(1, j)
    proj_v(0, VCUT[3], D)
    proj_k(0)
    proj_v(1)
    for cp in cp_rest:
        cp.wait()
    for s in (2, 3):
        for j in range(NQT):
            layernorm(s, j)
        proj_q(s - 1)
    proj_q(3)
    for j in range(NT):
        for i in range(NT - 1):
            _store_transposed(wot_s, 0, wo_v, i, j)

    r = _round_bf16(r_s[...])
    pos = (_iota((S // T, T), 0) * T + _iota((S // T, T), 1)).astype(f32)
    r1 = _all_max(r)
    i1 = -_all_max(jnp.where(r == r1, -pos, 1.0 - S))
    rest = pos != i1
    r2 = _all_max(jnp.where(rest, r, -jnp.inf))
    i2 = -_all_max(jnp.where(rest & (r == r2), -pos, 1.0 - S))
    i1, i2 = i1.astype(jnp.int32), i2.astype(jnp.int32)

    for s in range(1, NSEG):
        proj_k(s)
        if s > 1:
            proj_v(s)

    xsel = jnp.zeros((8, DP), f32)
    for c, idx in enumerate((i1, i2)):
        token = jnp.where(_iota((DP // 2, T), 1) == idx % T, xn_s[(idx // T)[0, 0]],
                          jnp.zeros((), u32))
        xsel = xsel + _dot_nt(jnp.where(sub == c, 1.0, 0.0), _unpack(token))

    ffn = {}

    def ffn_in(w, name, cg, i):
        k = min(T, D - T * i)
        part = _dot(xsel[:, T * i:T * i + k], w[T * i:T * i + k, L * cg:L * (cg + 1)])
        ffn[name] = part if i == 0 else ffn[name] + part
        if name == "up" and i == NT - 1:
            h_s[:, L * cg:L * (cg + 1)] = _round_bf16(
                ffn["gate"] * _sigmoid(ffn["gate"]) * ffn["up"])

    def ffn_out(cg, i):
        if i < 4:
            c0 = L * cg + T * i
            name, part = "y0", _dot_nt(h_s[:, c0:c0 + T], wd_v[0:4 * T, c0:c0 + T])
        else:
            cols = slice(L * cg, L * (cg + 1))
            name, part = "y1", _dot_nt(h_s[:, cols], wd_v[4 * T:D, cols])
        ffn[name] = ffn[name] + part if name in ffn else part

    def ffn_finish():
        y = jnp.concatenate([ffn["y0"], ffn["y1"], jnp.zeros((8, DP - D), f32)], axis=1)
        y = y * _sigmoid(jnp.where(_iota((8, DP), 0) == 0, r1, r2))
        y = jnp.concatenate([y, jnp.zeros((8, DP), f32)], axis=0)
        for j in range(NT):
            _store_transposed(wot_s, 0, wo_v, NT - 1, j, tail=y[:, T * j:T * (j + 1)].astype(bf16))

    rounds = []
    for cg in range(F // L):
        rounds += [(ffn_in, wg_v, "gate", cg, i) for i in range(NT)]
        rounds += [(ffn_in, wu_v, "up", cg, i) for i in range(NT)]
        if cg > 0:
            rounds += [(ffn_out, cg - 1, i) for i in range(NT)]
    rounds += [None] * 3
    rounds += [(ffn_out, F // L - 1, i) for i in range(NT)]

    steps = [(s, g, j, i) for s in range(NSEG) for g in range(NG) for j in range(NQT)
             for i in range(j + 1)]
    ns = len(steps)
    mx, tok, due = {}, {}, {}
    lane = _iota((8, T), 1)
    high = lane >= T // 2
    quarter = [lane // QB == c for c in range(HG)]
    mid = quarter[1] | quarter[2]
    first_row, last_row = sub == 0, sub == 7
    none, ones = jnp.zeros((8, T), u32), jnp.ones((8, T), f32)

    def q_tile(s, g, j, c):
        h = HG * g + c
        at = DH * h // 16 - GWIN[g] // 16
        return [none] * at + [q_s[s, h, j, 0:8], q_s[s, h, j, 8:16]] + [none] * (GK // 16 - 2 - at)

    def logits(s, g, k0, k1, q_tiles):
        keys = _unpack(k_s[s + zero, g, k0 // 2:k1 // 2, :])[:, :GK]
        return _dot(keys, _unpack(
            jnp.concatenate([jnp.concatenate(q, axis=0) for q in q_tiles], axis=1)))

    def stash(n, st, row0, col0, masked):
        m = None
        cols = slice(col0, col0 + st.shape[1])
        for r0 in range(0, st.shape[0], 8):
            rows = slice(row0 + r0, row0 + r0 + 8)
            x = st[r0:r0 + 8]
            if masked:
                x = x + bias_s[rows, cols]
            s_s[n % NB, rows, cols] = x
            m = x if m is None else jnp.maximum(m, x)
        return m

    def qk(n):
        s, g, j, i = steps[n]
        q = [q_tile(s, g, j, c) for c in range(HG)]
        k0 = T * i
        if i < j:
            ahead = QB if i == j - 1 else 0
            st = logits(s, g, k0, k0 + T + ahead, q)
            tok[n] = st[TOKROW:TOKROW + 8]
            m = stash(n, st[:T], 0, 0, False)
            if ahead:
                m = jnp.maximum(m, stash(n + 1, st[T:], 0, 0, True))
            mx[s, g, j] = m if i == 0 else jnp.maximum(mx[s, g, j], m)
            return
        m = stash(n, logits(s, g, k0, k0 + QB, q), 0, 0, True) if j == 0 else mx[s, g, j]
        x1 = logits(s, g, k0 + QB, k0 + 2 * QB, [_select(quarter[c], q[3], q[c]) for c in range(3)])
        x3 = logits(s, g, k0 + 3 * QB, k0 + T,
                    [_select(high, _select(mid, q[3], q[0]), _select(mid, q[2], q[1]))])
        tok[n] = jnp.concatenate([x1[QB - 8:], x3[QB - 8:]], axis=1)
        m1 = stash(n, x1, QB, 0, True)
        m1 = [m1[:, T * c:T * (c + 1)] for c in range(3)]
        m3 = stash(n, x3, QB, 3 * T, True)
        m2 = []
        for c, pair in enumerate((_select(high, q[0], q[2]), _select(mid, q[3], q[1]))):
            m2.append(jnp.maximum(*[
                stash(n, logits(s, g, k0 + r0, k0 + r0 + QB // 2, [pair]), r0, T * c, True)
                for r0 in (2 * QB, 2 * QB + QB // 2)]))
        ms = []
        for c in range(HG):
            x = m[:, T * c:T * (c + 1)]
            if c < 3:
                x = lax.select(quarter[c], x, jnp.maximum(x, m1[c]))
            else:
                for b in range(3):
                    x = lax.select(quarter[b], jnp.maximum(x, m1[b]), x)
            y = jnp.maximum(x, m2[c % 2])
            x = lax.select((high, mid)[c % 2], *((y, x) if c in (0, 3) else (x, y)))
            ms.append(lax.select(quarter[(c + 3) % HG], jnp.maximum(x, m3), x))
        mx[s, g, j] = jnp.max(jnp.concatenate(ms, axis=1), axis=0, keepdims=True)

    def pv(n):
        s, g, j, i = steps[n]
        ms = []
        for c in range(HG):
            m = jnp.broadcast_to(mx[s, g, j][:, T * c:T * (c + 1)], (8, T))
            first = tok[n + LAG - TOKBACK][:, T * c:T * (c + 1)]
            for x in due.pop((n, c), ()):
                first = jnp.maximum(first, x)
            ms.append(lax.select(never, first, m))

        def probs(r0, r1, c, m):
            return jnp.exp2(s_s[n % NB, r0:r1, T * c:T * (c + 1)].reshape(-1, 8, T) - m)

        if i == j:
            e1 = [probs(QB, 2 * QB, c, lax.select(quarter[c], ms[3], ms[c])) for c in range(3)]
            e3 = probs(QB, 2 * QB, 3, lax.select(high, lax.select(mid, ms[3], ms[0]),
                                                 lax.select(mid, ms[2], ms[1])))
            e2 = [probs(2 * QB, 3 * QB, 0, lax.select(high, ms[0], ms[2])),
                  probs(2 * QB, 3 * QB, 1, lax.select(mid, ms[3], ms[1]))]
        for c in range(HG):
            if i == j:
                if c < 3:
                    p1 = jnp.where(quarter[c], 0.0, e1[c])
                else:
                    p1 = jnp.where(quarter[0], e1[0], jnp.where(
                        quarter[1], e1[1], jnp.where(quarter[2], e1[2], 0.0)))
                p2 = jnp.where((high, mid)[c % 2],
                               *((e2[c % 2], 0.0) if c in (0, 3) else (0.0, e2[c % 2])))
                p3 = jnp.where(quarter[(c + 3) % HG], e3, 0.0)
                p = jnp.concatenate([probs(0, QB, c, ms[c]), p1, p2, p3], axis=0)
            else:
                p = probs(0, T, c, ms[c])
            h = HG * g + c
            a = DH * h // 8 * 8
            o = DH * h - a
            one = 23 if o == 0 else 0
            v = [v_s[s, a + r:a + r + 8, T * i:T * (i + 1)] for r in (0, 8, 16)]
            v[one // 8] = lax.select(last_row if one else first_row, ones, v[one // 8])
            acc = _dot(jnp.concatenate(v, axis=0), p.reshape(T, T).astype(bf16))
            if i > 0:
                acc = acc_s[c] + acc
            if i < j:
                acc_s[c] = acc
                continue
            den = acc[one:one + 1]
            inv = pltpu.reciprocal(den, approx=True)
            inv = inv * (2.0 - den * inv)
            val = acc * ((1.0 - g_s[h:h + 1, :]) * (inv * (2.0 - den * inv)))
            if c:
                val = pltpu.roll(val, T - QB * c, 1)
            due[n + DUE, c] = [val[r:r + 8] for r in (0, 8, 16)]
            o_s[s % 2, DH * h:DH * (h + 1), T * j:T * (j + 1)] = val[o:o + DH]

    def mem_update(s, t):
        w0 = WIN * t
        r0, r1_, one = _win_rows(t)
        v = [v_s[s, r:r + 8, :] for r in range(r0, r1_, 8)]
        v[(one - r0) // 8] = jnp.where(_iota((8, L), 0) == one % 8, 1.0, v[(one - r0) // 8])
        upd = _dot_nt(jnp.concatenate(v, axis=0), _unpack(pk_s[s, w0 // 2:(w0 + T) // 2, :]))
        rows = slice(r0 - w0, r1_ - w0)
        m_s[t, rows] = upd if s == 0 else m_s[t, rows] + upd

    def mem_read(s, t):
        heads = WIN_HEADS[t]
        w0 = WIN * t
        r0, r1_, one = _win_rows(t)
        rows = slice(r0 - w0, r1_ - w0)
        norm = jnp.where(mask_s[t, T:T + 8] > 0, m_s[t, one - w0:one - w0 + 1], 0.0)
        lhs = jnp.concatenate([norm, jnp.where(mask_s[t, rows] > 0, m_s[t, rows], 0.0)], axis=0)
        rd = _dot(_round_bf16(lhs), _unpack(pq_s[s - 1, w0 // 2:(w0 + T) // 2, :]))
        h0 = heads[0]
        coef = jnp.concatenate([g_s[h0:h0 + 8, :]] * NQT, axis=1) / (rd[:8] + 1e-6)
        for r in range(r0, r1_, 8):
            ha = max(r // DH, h0)
            hb = min((r + 7) // DH, heads[-1])
            cf = jnp.broadcast_to(coef[ha - h0:ha - h0 + 1], (8, L))
            if hb != ha:
                cf = jnp.where(_iota((8, L), 0) < DH * hb - r, cf,
                               jnp.broadcast_to(coef[hb - h0:hb - h0 + 1], (8, L)))
            val = rd[r - r0 + 8:r - r0 + 16] * cf
            lo, hi = max(r, DH * h0), min(r + 8, DH * (heads[-1] + 1))
            om_s[s - 1, lo:hi, :] = val[lo - r:hi - r]

    def pack_o(s, r0, r1_):
        o = o_s[s % 2, r0:r1_, :]
        if s > 0:
            o = o + om_s[s - 1, r0:r1_, :]
        ob_s[s, r0 // 2:r1_ // 2, :] = _pack(o.astype(bf16))

    def out_proj(s, r0, r1_, n=None):
        ob = ob_s[s]
        if n is not None:
            head = jnp.where(jnp.concatenate([never] * NQT, axis=1),
                             pltpu.bitcast(tok[n - TOKBACK], u32), ob[:8])
            ob = jnp.concatenate([head, ob[8:]], axis=0)
        res = _dot(_unpack(wot_s[zero, r0 // 2:r1_ // 2, :]), _unpack(ob))
        if n is not None:
            tok[n] = res[:8]
        xn = _unpack(jnp.concatenate(
            [xn_s[NQT * s + j, r0 // 2:r1_ // 2, :] for j in range(NQT)], axis=1))
        out_v[s, r0:r1_, :] = (res + x_v[s, r0:r1_, :].astype(f32) + xn.astype(f32)).astype(bf16)

    for s in range(NSEG):
        which = _iota((16, L), 0)
        routed = jnp.where(which == 0, i1, jnp.where(which == 1, i2, -1))
        ob_s[s, D // 2:D // 2 + 8, :] = _pack(
            jnp.where(_iota((16, L), 1) + s * L == routed, 1.0, 0.0).astype(bf16))
        ob_s[s, D // 2 + 8:DP // 2, :] = jnp.zeros(((DP - D) // 2 - 8, L), u32)

    extra = {}
    per = ns // NSEG
    full = [n for n, (_, _, j, i) in enumerate(steps) if i < j]

    def at(n, *task):
        extra.setdefault(n, []).append(task)

    def at_full(n, *task):
        n = next(m for m in full if m >= n)
        at(n, *task)
        return n

    for s in range(1, NSEG):
        for t in range(NWIN):
            at(MEM0 + 2 * s - 2, mem_update, s - 1, t)
            at(MEM0 + 2 * s - 1, mem_read, s, t)
    for cp in cp_ffn:
        at(FFN0, cp.wait)
    n = FFN0
    for task in rounds:
        n = n + 1 if task is None else at_full(n, *task) + 1
    at(n + 1, ffn_finish)
    for s in range(NSEG):
        for c in range(D // 48):
            group = (48 * (c + 1) - 1) // (HG * DH)
            n = per * s + per // NG * (group + 1) + LAG + c % 2 * 3 + 1
            at(min(n, ns + LAG), pack_o, s, 48 * c, 48 * (c + 1))
    for c in range(LAG):
        at(ns + c, out_proj, 0, FILL * c, FILL * (c + 1), ns + c)

    for n in range(ns + LAG + 1):
        if n < ns:
            qk(n)
        for fn, *args in extra.get(n, ()):
            if fn is not ffn_in:
                fn(*args)
        if LAG <= n < ns + LAG:
            pv(n - LAG)
        for fn, *args in extra.get(n, ()):
            if fn is ffn_in:
                fn(*args)
    out_proj(0, FILL * LAG, D, ns + LAG)
    cp_out[0].start()
    for s in range(1, NSEG - 1):
        out_proj(s, 0, D)
        cp_out[s].start()
    for (r0, r1_), cp in zip(TAIL, cp_tail):
        out_proj(NSEG - 1, r0, r1_)
        cp.start()
    for cp in cp_out + cp_tail:
        cp.wait()


@jax.jit
def pallas_parallel_sum__memory_aug_infini_attn__moe_arch_mod__prompt_kernel(
    A_x: jax.Array,
    A_wq: jax.Array,
    A_wk: jax.Array,
    A_wv: jax.Array,
    A_wo: jax.Array,
    A_beta: jax.Array,
    B_x: jax.Array,
    B_w_r: jax.Array,
    B_w_gate: jax.Array,
    B_w_up: jax.Array,
    B_w_down: jax.Array,
):
    del B_x
    out_t = pl.pallas_call(
        _kernel,
        out_shape=jax.ShapeDtypeStruct((D, S), bf16),
        in_specs=[pl.BlockSpec(memory_space=pl.ANY)] * 10,
        out_specs=pl.BlockSpec(memory_space=pl.ANY),
        scratch_shapes=[
            pltpu.VMEM((NSEG, D, L), bf16),
            pltpu.VMEM((D, D), bf16),
            pltpu.VMEM((D, D), bf16),
            pltpu.VMEM((D, D), bf16),
            pltpu.VMEM((D, D), bf16),
            pltpu.VMEM((D, F), bf16),
            pltpu.VMEM((D, F), bf16),
            pltpu.VMEM((D, F), bf16),
            pltpu.VMEM((1, H), bf16),
            pltpu.VMEM((D,), bf16),
            pltpu.VMEM((NSEG, D, L), bf16),
            pltpu.VMEM((1, 3 * D // 2, DP), u32),
            pltpu.VMEM((1, D // 2, DP), u32),
            pltpu.VMEM((S // T, DP // 2, T), u32),
            pltpu.VMEM((NSEG, H, NQT, 16, T), u32),
            pltpu.VMEM((NSEG, NG, L // 2, T), u32),
            pltpu.VMEM((NSEG, D, L), f32),
            pltpu.VMEM((NSEG - 1, D // 2, L), u32),
            pltpu.VMEM((NSEG - 1, D // 2, L), u32),
            pltpu.VMEM((2, D // 2, T), f32),
            pltpu.VMEM((S // T, T), f32),
            pltpu.VMEM((T, T), f32),
            pltpu.VMEM((3 * QB, HG * T), f32),
            pltpu.VMEM((NB, T, HG * T), f32),
            pltpu.VMEM((HG, 24, T), f32),
            pltpu.VMEM((2, D, L), f32),
            pltpu.VMEM((NSEG, DP // 2, L), u32),
            pltpu.VMEM((NWIN, T + 8, T), f32),
            pltpu.VMEM((NWIN, T, T), f32),
            pltpu.VMEM((NSEG - 1, D, L), f32),
            pltpu.VMEM((8, F), f32),
            pltpu.SemaphoreType.DMA((9,)),
        ],
        compiler_params=pltpu.CompilerParams(vmem_limit_bytes=100 * 1024 * 1024),
        name="infini_moe",
    )(A_x.reshape(S, D).T, A_wq, A_wk, A_wv, A_wo, A_beta.reshape(1, H), B_w_r,
      B_w_gate, B_w_up, B_w_down.T)
    return out_t.T.reshape(1, S, D)
```
